```python
import jax
import jax.numpy as jnp

def _softmax(x, axis=-1):
    return jax.nn.softmax(x, axis=axis)
def _gelu(x):
    return jax.nn.gelu(x, approximate=True)
def _silu(x):
    return jax.nn.silu(x)
def _sigmoid(x):
    return jax.nn.sigmoid(x)
def _layernorm(x, axis=-1, eps=1e-5):
    m = jnp.mean(x, axis=axis, keepdims=True)
    v = jnp.var(x, axis=axis, keepdims=True)
    return (x - m) / jnp.sqrt(v + eps)
def _scatter_add(tgt, idx, src, axis=0):
    return tgt.at[idx].add(src)
def _segment_sum(src, seg, n):
    return jax.ops.segment_sum(src, seg, n)
class _Rng:
    def __init__(self, key):
        self._k = key
    def _next(self):
        self._k, sub = jax.random.split(self._k)
        return sub
    def normal(self, shape):
        return jax.random.normal(self._next(), shape, dtype=jnp.bfloat16)
    def randint(self, lo, hi, shape):
        return jax.random.randint(self._next(), shape, lo, hi, dtype=jnp.int32)
    def uniform(self, shape, lo=0.0, hi=1.0):
        return jax.random.uniform(self._next(), shape, jnp.bfloat16, lo, hi)
    def permutation(self, n):
        return jax.random.permutation(self._next(), n)


kernel_name = 'interleave_layers__grouped_kv_mqa__sliding_local_dilated__prompt'

def setup_inputs():
    _rng = _Rng(jax.random.key(int.from_bytes(__import__("os").urandom(4), "little")))
    _w = (lambda a: (lambda t: t.astype(jnp.bfloat16) if jnp.issubdtype(t.dtype, jnp.floating) else t)(jnp.asarray(a)))
    def _A_setup():
        B, S, D, H = 1, 2048, 1024, 32
        Dh = D // H
        return {
            "x": _w((lambda *s: _rng.normal(s) * 0.05)(B, S, D)),
            "wq": _w((lambda *s: _rng.normal(s) * 0.05)(D, H * Dh)),
            "wk": _w((lambda *s: _rng.normal(s) * 0.05)(D, Dh)),
            "wv": _w((lambda *s: _rng.normal(s) * 0.05)(D, Dh)),
            "wo": _w((lambda *s: _rng.normal(s) * 0.05)(H * Dh, D)),
        }
    _A_in = _A_setup()

    def _B_setup():
        B, S, D = 1, 2048, 1024
        return {
            "x": _w((lambda *s: _rng.normal(s) * 0.05)(B, S, D)),
            "wqkv": _w((lambda *s: _rng.normal(s) * 0.05)(D, 3 * D)),
            "wo": _w((lambda *s: _rng.normal(s) * 0.05)(D, D)),
        }
    _B_in = _B_setup()

    return {
        "A_x": _A_in["x"],
        "A_wq": _A_in["wq"],
        "A_wk": _A_in["wk"],
        "A_wv": _A_in["wv"],
        "A_wo": _A_in["wo"],
        "B_x": _B_in["x"],
        "B_wqkv": _B_in["wqkv"],
        "B_wo": _B_in["wo"],
    }

def reference(A_x, A_wq, A_wk, A_wv, A_wo, B_x, B_wqkv, B_wo):
    def _A_ref(x, wq, wk, wv, wo):
        B, S, D = x.shape
        H = 32
        Dh = D // H
        q = (lambda x, *d: x.transpose(*d))((x @ wq).reshape(B, S, H, Dh), 0, 2, 1, 3)
        k = x @ wk
        v = x @ wv
        scores = jnp.einsum("bhqd,bkd->bhqk", q, k) * (Dh ** -0.5)
        p = _softmax(scores, axis=-1)
        o = jnp.einsum("bhqk,bkd->bhqd", p, v)
        return (lambda x, *d: x.transpose(*d))(o, 0, 2, 1, 3).reshape(B, S, H * Dh) @ wo

    def _B_ref(x, wqkv, wo):
        B, S, D = x.shape
        H = 32; Dh = D // H
        W, dil = 8, 2
        qkv = (lambda x, *d: x.transpose(*d))((x @ wqkv).reshape(B, S, 3, H, Dh), 2, 0, 3, 1, 4)
        q, k, v = qkv[0], qkv[1], qkv[2]
        scale = Dh ** -0.5
        pos = jnp.arange(S)
        off = jnp.arange(W) * dil
        idx = pos[:, None] - off[None, :]
        mask = idx >= 0
        idx_c = jnp.where(mask, idx, 0).reshape(-1)
        kg = k[:, :, idx_c, :].reshape(B, H, S, W, Dh)
        vg = v[:, :, idx_c, :].reshape(B, H, S, W, Dh)
        logits = jnp.einsum("bhsd,bhswd->bhsw", q, kg) * scale
        logits = jnp.where(mask[None, None, :, :], logits, -1e9)
        attn = _softmax(logits, axis=-1)
        o = jnp.einsum("bhsw,bhswd->bhsd", attn, vg)
        return (lambda x, *d: x.transpose(*d))(o, 0, 2, 1, 3).reshape(B, S, D) @ wo

    x = A_x
    x = x + _A_ref(_layernorm(x, axis=-1), A_wq, A_wk, A_wv, A_wo)
    x = x + _B_ref(_layernorm(x, axis=-1), B_wqkv, B_wo)
    x = x + _A_ref(_layernorm(x, axis=-1), A_wq, A_wk, A_wv, A_wo)
    x = x + _B_ref(_layernorm(x, axis=-1), B_wqkv, B_wo)
    return x
```

```python
import jax
import jax.numpy as jnp
import jax.experimental.pallas as pl
import jax.experimental.pallas.tpu as pltpu

F32, BF16, U32 = jnp.float32, jnp.bfloat16, jnp.uint32

S, D, H, DH = 2048, 1024, 32, 32
W, DIL = 8, 2
EPS = 1e-5
LOG2E = 1.4426950408889634
QSCALE = DH ** -0.5 * LOG2E
NEG = -1e9 * LOG2E

T = 256
NB = S // T
KA = 48
HALO = 16
U = 8
SHIFT = 20.0
L_LO, L_HI = 2.0 ** -40, 2.0 ** 33
UP = 1.0 + 2.0 ** -7


def _mm(a, b):
    return jnp.dot(a, b, preferred_element_type=F32)


def _ln(x):
    m = jnp.mean(x, axis=-1, keepdims=True)
    c = x - m
    v = jnp.mean(c * c, axis=-1, keepdims=True)
    return c * jax.lax.rsqrt(v + EPS)


def _iota(shape, dim):
    return jax.lax.broadcasted_iota(jnp.int32, shape, dim)


def _blk(i, n=T):
    if isinstance(i, int):
        return pl.ds(i * n, n)
    return pl.ds(pl.multiple_of(i * n, n), n)


def _kernel(x_hbm, wq_hbm, wk_hbm, wv_hbm, woa_hbm, wqkv_hbm, wob_hbm, out_hbm,
            xio, wq, wk, wv, woa, wqkv, wob, wp, wobp, wkvt, tmp,
            xr, xn, ob, qa, ka, vt, kmax, bad,
            q0, k0, v0, q1, k1, v1, sem_x, sem_w, sem_o):

    def x_copy(i):
        return pltpu.make_async_copy(x_hbm.at[_blk(i)], xio.at[_blk(i)], sem_x.at[i])

    def out_copy(i):
        return pltpu.make_async_copy(xio.at[_blk(i)], out_hbm.at[_blk(i)], sem_o.at[i])

    w_copies = [pltpu.make_async_copy(s, d, sem_w.at[n]) for n, (s, d) in enumerate(
        [(wk_hbm, wk), (wv_hbm, wv), (wq_hbm, wq), (wqkv_hbm, wqkv), (wob_hbm, wob), (woa_hbm, woa)])]
    x_copy(0).start()
    for c in w_copies[:3]:
        c.start()
    for i in range(1, NB):
        x_copy(i).start()
    for c in w_copies[3:]:
        c.start()

    def st_ln_in(i):
        x = xio[_blk(i), :].astype(F32)
        xr[_blk(i), :] = x
        xn[_blk(i), :] = _ln(x).astype(BF16)

    def st_ln(i):
        xn[_blk(i), :] = _ln(xr[_blk(i), :]).astype(BF16)

    def st_qkv_a(i):
        a = xn[_blk(i), :]
        kvt = jax.lax.dot_general(wkvt[...], a, (((1,), (1,)), ((), ())), preferred_element_type=F32)
        kt = (kvt[:DH] * QSCALE).astype(BF16).astype(F32)
        vt[:, _blk(i)] = kvt[DH:].astype(BF16)
        k2 = (kt * kt).reshape(DH // 8, 8, T).sum(0).sum(0, keepdims=True)
        km = kmax[...]
        for t in range(T // 128):
            km = jnp.maximum(km, k2[:, t * 128:(t + 1) * 128])
            kk = jnp.concatenate([kt[:, t * 128:(t + 1) * 128], jnp.zeros((128 - DH, 128), F32)], axis=0).T
            kk = jnp.where(_iota((128, 128), 1) == DH + 1, 1.0, kk)
            kk = jnp.concatenate([kk[g * 16:(g + 1) * 16] for g in reversed(range(8))], axis=0)
            ka[_blk(i * (T // 128) + t, 128), :] = kk.astype(BF16)
        kmax[...] = km
        r = _iota((KA - DH, 128), 0)
        for c in range(D // 256):
            q = _mm(a, wq[:, c * 256:(c + 1) * 256])
            for t in range(T // 128):
                for g2 in range(2):
                    qt = q[t * 128:(t + 1) * 128, g2 * 128:(g2 + 1) * 128].T
                    for h in range(4):
                        qh = qt[h * DH:(h + 1) * DH]
                        n2 = (qh * qh).reshape(DH // 8, 8, 128).sum(0).sum(0, keepdims=True)
                        nq = jnp.sqrt(n2) * (-UP * UP)
                        aug = jnp.where(r == 0, nq, jnp.where(r == 1, SHIFT, 0.0))
                        qa[i * (T // 128) + t, c * 2 + g2, :, h * 128:(h + 1) * 128] = (
                            jnp.concatenate([qh, aug], axis=0).astype(BF16))

    def st_fix_k():
        km = jnp.sqrt(jnp.max(kmax[...], axis=1, keepdims=True)) * (UP * UP)
        kk = ka[...].astype(F32)
        ka[...] = jnp.where(_iota(kk.shape, 1) == DH, km, kk).astype(BF16)

    def put_o(tb, g, ot):
        ot = jnp.concatenate([ot[:, h * 128:(h + 1) * 128] for h in range(4)], axis=0)
        ob[_blk(tb, 128), _blk(g, 128)] = ot.T.astype(BF16)

    def st_attn(tb):
        nt = S // 128
        steps = [(g, t) for g in range(U) for t in range(nt)]
        s, acc, l = {}, {}, {}
        flag = [bad[...]]

        def qk(n):
            g, t = steps[n]
            s[n] = _mm(ka[t * 128:(t + 1) * 128, :KA], qa[tb, g])

        def pv(n):
            g, t = steps[n]
            p = jnp.exp2(s.pop(n))
            ps = p.reshape(16, 8, 512).sum(0)
            p = jnp.concatenate([p[j * 16:(j + 1) * 16] for j in reversed(range(8))], axis=0)
            o = _mm(vt[:, t * 128:(t + 1) * 128], p.astype(BF16))
            acc[g], l[g] = (o, ps) if t == 0 else (acc[g] + o, l[g] + ps)
            if t == nt - 1:
                ll = l.pop(g).sum(0, keepdims=True)
                ok = jnp.logical_and(ll >= L_LO, ll <= L_HI)
                flag[0] = jnp.maximum(flag[0], jnp.where(ok, 0.0, 1.0))
                put_o(tb, g, acc.pop(g) * (1.0 / ll))

        for n in range(len(steps) + 1):
            if n < len(steps):
                qk(n)
            if n > 0:
                pv(n - 1)
        bad[...] = flag[0]

    def st_attn_exact(u):
        tb, g = u // U, u % U
        q = qa[tb, g, :DH, :]

        def scores(t):
            kk = jnp.concatenate(
                [ka[pl.ds(pl.multiple_of(t * 128 + j * 16, 16), 16), :DH] for j in reversed(range(8))], axis=0)
            return _mm(kk, q)

        m = jax.lax.fori_loop(
            0, S // 128, lambda t, m: jnp.maximum(m, jnp.max(scores(t), axis=0, keepdims=True)),
            jnp.full((1, 512), -jnp.inf, F32))

        def body(t, c):
            p = jnp.exp2(scores(t) - m)
            return c[0] + _mm(vt[:, _blk(t, 128)], p.astype(BF16)), c[1] + jnp.sum(p, axis=0, keepdims=True)

        acc, l = jax.lax.fori_loop(0, S // 128, body, (jnp.zeros((DH, 512), F32), jnp.zeros((1, 512), F32)))
        put_o(tb, g, acc * (1.0 / l))

    def st_out(i, w, emit):
        a = ob[_blk(i), :]
        for c in range(D // 256):
            cs = slice(c * 256, (c + 1) * 256)
            x = xr[_blk(i), cs] + _mm(a, w[:, cs])
            xr[_blk(i), cs] = x
            if emit:
                xio[_blk(i), cs] = x.astype(BF16)

    def st_qkv_b(i, bufs):
        a = xn[_blk(i), :]
        for j, buf in enumerate(bufs):
            off = 0 if j == 0 else HALO
            for c in range(D // 256):
                r = _mm(a, wp[:, j * D + c * 256:j * D + (c + 1) * 256])
                buf[2 * c, off:off + T, :] = r[:, :128]
                buf[2 * c + 1, off:off + T, :] = r[:, 128:]

    def st_halo(dst, src):
        for d, s in zip(dst[1:], src[1:]):
            d[:, :HALO, :] = s[:, T:T + HALO, :]

    def st_halo0(dst):
        for d in dst[1:]:
            d[:, :HALO, :] = jnp.broadcast_to(d[:, HALO:HALO + 1, :], (8, HALO, 128))

    def st_window(i, bufs, first=False):
        q, k, v = bufs
        even = (_iota((8, 128), 1) & 1) == 0

        def group(r):
            lg = [None] * W
            for j in range(8):
                qj = q[j, r:r + 8, :]
                for w in range(W):
                    pr = qj * k[j, pl.ds(HALO + r - DIL * w, 8), :]
                    lg[w] = pr if j == 0 else lg[w] + pr
            for w in range(W):
                y = lg[w] + pltpu.roll(lg[w], 64, 1)
                y = (y + jnp.where(even, pltpu.roll(y, 127, 1), pltpu.roll(y, 1, 1))) * QSCALE
                if first and r < DIL * w:
                    y = jnp.where(_iota((8, 128), 0) + r >= DIL * w, y, NEG)
                lg[w] = y
            m = lg[0]
            for w in range(1, W):
                m = jnp.maximum(m, lg[w])
            p = [jnp.exp2(y - m) for y in lg]
            den = p[0]
            for w in range(1, W):
                den = den + p[w]
            inv = 1.0 / den
            return [y * inv for y in p]

        for r in range(0, T, 16):
            ps = [group(r), group(r + 8)]
            for j in range(8):
                halves = []
                for hf in range(2):
                    o = None
                    for w in range(W):
                        pr = ps[hf][w] * v[j, pl.ds(HALO + r + 8 * hf - DIL * w, 8), :]
                        o = pr if w == 0 else o + pr
                    halves.append(o)
                row = i * T + r
                row = row if isinstance(row, int) else pl.multiple_of(row, 16)
                ob[pl.ds(row, 16), j * 128:(j + 1) * 128] = jnp.concatenate(halves, axis=0).astype(BF16)

    def st_permute(wt):
        for j in range(3):
            for t in range(8):
                cs = slice(j * D + t * 128, j * D + (t + 1) * 128)
                tmp[t * 128:(t + 1) * 128, :] = pltpu.bitcast(wqkv[_blk(wt, 256), cs], U32).T
            for u in range(8):
                cs = slice(j * D + u * 128, j * D + (u + 1) * 128)
                y = jnp.concatenate([tmp[pl.ds(4 * u + e, H, stride=DH), :] for e in range(4)], axis=0).T
                lane = _iota((128, 128), 1)
                src = (lane & 64) + (lane & 1) * 32 + ((lane & 63) >> 1)
                wp[_blk(wt, 256), cs] = pltpu.bitcast(jnp.take_along_axis(y, src, axis=1), BF16)

    def st_permute_o():
        for t in range(8):
            cs = slice(t * 128, (t + 1) * 128)
            tmp[:D // 2, :] = pltpu.bitcast(wob[:, cs], U32)
            for e in range(DH // 2):
                wobp[e * 64:(e + 1) * 64, cs] = pltpu.bitcast(tmp[pl.ds(e, H, stride=DH // 2), :], BF16)

    kmax[...] = jnp.zeros(kmax.shape, F32)
    x_copy(0).wait()
    st_ln_in(0)
    for c in w_copies[:2]:
        c.wait()
    wkvt[:DH, :] = wk[...].astype(F32).T.astype(BF16)
    wkvt[DH:, :] = wv[...].astype(F32).T.astype(BF16)
    w_copies[2].wait()

    @pl.loop(0, NB - 1)
    def _(i):
        x_copy(i + 1).wait()
        st_qkv_a(i)
        st_ln_in(i + 1)

    st_qkv_a(NB - 1)

    for c in w_copies[3:]:
        c.wait()

    @pl.loop(0, 4)
    def _(wt):
        st_permute(wt)

    st_permute_o()

    bufs = ((q0, k0, v0), (q1, k1, v1))

    @pl.loop(0, 2)
    def _(layer):
        st_fix_k()
        bad[...] = jnp.zeros(bad.shape, F32)

        @pl.loop(0, S // 128)
        def _(tb):
            st_attn(tb)

        @pl.when(jnp.max(bad[...]) > 0.0)
        def _():
            @pl.loop(0, (S // 128) * U)
            def _(u):
                st_attn_exact(u)

        st_out(0, woa, False)

        @pl.loop(1, NB)
        def _(i):
            st_ln(i - 1)
            st_out(i, woa, False)

        st_ln(NB - 1)
        st_qkv_b(0, bufs[0])
        st_halo0(bufs[0])
        st_window(0, bufs[0], first=True)
        st_qkv_b(1, bufs[1])

        @pl.loop(0, NB // 2 - 1)
        def _(j):
            st_halo(bufs[1], bufs[0])
            st_window(2 * j + 1, bufs[1])
            st_qkv_b(2 * j + 2, bufs[0])
            st_halo(bufs[0], bufs[1])
            st_window(2 * j + 2, bufs[0])
            st_qkv_b(2 * j + 3, bufs[1])

        st_halo(bufs[1], bufs[0])
        st_window(NB - 1, bufs[1])
        st_out(0, wobp, True)

        @pl.when(layer == 1)
        def _():
            out_copy(0).start()

        @pl.loop(1, NB)
        def _(i):
            st_ln(i - 1)
            st_out(i, wobp, True)

            @pl.when(layer == 1)
            def _():
                out_copy(i).start()

        @pl.when(layer == 0)
        def _():
            kmax[...] = jnp.zeros(kmax.shape, F32)
            st_qkv_a(0)
            st_ln(NB - 1)

            @pl.loop(1, NB)
            def _(i):
                st_qkv_a(i)

    for i in range(NB):
        out_copy(i).wait()


@jax.jit
def pallas_interleave_layers__grouped_kv_mqa__sliding_local_dilated__prompt_kernel(
    A_x: jax.Array,
    A_wq: jax.Array,
    A_wk: jax.Array,
    A_wv: jax.Array,
    A_wo: jax.Array,
    B_x: jax.Array,
    B_wqkv: jax.Array,
    B_wo: jax.Array,
):
    del B_x
    vm = pltpu.VMEM
    qkv = [vm((8, T, 128), F32), vm((8, T + HALO, 128), F32), vm((8, T + HALO, 128), F32)]
    out = pl.pallas_call(
        _kernel,
        out_shape=jax.ShapeDtypeStruct((S, D), BF16),
        in_specs=[pl.BlockSpec(memory_space=pl.ANY)] * 7,
        out_specs=pl.BlockSpec(memory_space=pl.ANY),
        scratch_shapes=[
            vm((S, D), BF16),
            vm((D, D), BF16), vm((D, DH), BF16), vm((D, DH), BF16), vm((D, D), BF16),
            vm((D, 3 * D), BF16), vm((D, D), BF16),
            vm((D, 3 * D), BF16), vm((D, D), BF16),
            vm((2 * DH, D), BF16),
            vm((D, 128), U32),
            vm((S, D), F32), vm((S, D), BF16), vm((S, D), BF16),
            vm((S // 128, U, KA, 512), BF16),
            vm((S, 128), BF16), vm((DH, S), BF16),
            vm((1, 128), F32), vm((1, 512), F32),
            *qkv, *qkv,
            pltpu.SemaphoreType.DMA((NB,)), pltpu.SemaphoreType.DMA((6,)), pltpu.SemaphoreType.DMA((NB,)),
        ],
        compiler_params=pltpu.CompilerParams(vmem_limit_bytes=110 * 1024 * 1024),
        name="interleave",
    )(A_x.reshape(S, D), A_wq, A_wk, A_wv, A_wo, B_wqkv, B_wo)
    return out.reshape(1, S, D)
```

```python
import functools

import jax
import jax.numpy as jnp
import jax.experimental.pallas as pl
import jax.experimental.pallas.tpu as pltpu

F32, BF16, U32 = jnp.float32, jnp.bfloat16, jnp.uint32

S, D, H, DH = 2048, 1024, 32, 32
W, DIL = 8, 2
EPS = 1e-5
LOG2E = 1.4426950408889634
QSCALE = DH ** -0.5 * LOG2E
NEG = -1e9 * LOG2E

T = 256
NB = S // T
KA = 48
HALO = 16
U = 8
SHIFT = 20.0
L_LO, L_HI = 2.0 ** -40, 2.0 ** 33
UP = 1.0 + 2.0 ** -7


def _mm(a, b):
    return jnp.dot(a, b, preferred_element_type=F32)


def _pack(x):
    return pltpu.bitcast(x.astype(BF16), U32)


def _bf(x):
    return pltpu.bitcast(x, BF16)


def _ln(x):
    m = jnp.mean(x, axis=-1, keepdims=True)
    c = x - m
    v = jnp.mean(c * c, axis=-1, keepdims=True)
    return c * jax.lax.rsqrt(v + EPS)


def _iota(shape, dim):
    return jax.lax.broadcasted_iota(jnp.int32, shape, dim)


def _ds(start, n):
    return pl.ds(start if isinstance(start, int) else pl.multiple_of(start, 8), n)


def _after(x, deps):
    for keep, d in deps:
        head = jnp.where(keep, x[:8, :128], pltpu.bitcast(d, x.dtype))
        if x.shape[1] > 128:
            head = jnp.concatenate([head, x[:8, 128:]], axis=1)
        x = jnp.concatenate([head, x[8:]], axis=0) if x.shape[0] > 8 else head
    return x


def _overlap(j, mms, *sides):
    keep = _iota((8, 128), 0) + j >= 0
    slots = [[] for _ in range(len(mms) - 1)]
    for side in sides:
        for n, f in enumerate(side):
            slots[n * len(slots) // len(side)].append(f)
    made, done = [], []
    for n, mm in enumerate(mms):
        made.append((keep, mm(done[n - 2] if n >= 2 else [])))
        if n < len(slots):
            done.append([(keep, f(made[n - 1:n])) for f in slots[n]])


def _kernel(x_hbm, wq_hbm, wkt_hbm, wvt_hbm, woa_hbm, wqkv_hbm, wob_hbm, out_hbm,
            xio, wq, woa, wqkv, wob, wp, wobp, wkvt, tmp,
            xe, xo, oe, oo, xn0, xn1, qa, ka, vt, kmax, bad,
            b0, b1, sem_x, sem_w, sem_o):
    xr, ob, xn = (xe, xo), (oe, oo), (xn0, xn1)
    bufs = (b0, b1)
    TP = T // 2

    def x_copy(i):
        return pltpu.make_async_copy(x_hbm.bitcast(U32).at[_ds(i * TP, TP)], xio.at[_ds(i * TP, TP)], sem_x.at[i])

    def out_copy(i):
        return pltpu.make_async_copy(xio.at[_ds(i * TP, TP)], out_hbm.bitcast(U32).at[_ds(i * TP, TP)], sem_o.at[i])

    w_copies = [pltpu.make_async_copy(s.bitcast(U32), d, sem_w.at[n]) for n, (s, d) in enumerate(
        [(wkt_hbm, wkvt.at[:DH // 2]), (wvt_hbm, wkvt.at[DH // 2:]), (wq_hbm, wq),
         (wqkv_hbm, wqkv), (wob_hbm, wob), (woa_hbm, woa)])]
    x_copy(0).start()
    for c in w_copies[:3]:
        c.start()

    def st_ln(j, par, dst, from_input=False):
        def step(r, deps):
            if from_input:
                x = _bf(xio[_ds((2 * j + par) * TP + r // 2, 8), :]).astype(F32)
                xr[par][_ds(j * T + r, 16), :] = x
            else:
                x = xr[par][_ds(j * T + r, 16), :]
            x = jnp.concatenate([_after(x[:8], deps), _after(x[8:], deps)], axis=0)
            y = _pack(_ln(x))
            dst[r // 2:r // 2 + 8, :] = y
            return y[:, :128]
        return [functools.partial(step, r) for r in range(0, T, 16)]

    def st_qkv_a(i, src):
        def kv(deps):
            kvt = jax.lax.dot_general(_bf(_after(wkvt[...], deps)), _bf(src[...]), (((1,), (1,)), ((), ())),
                                      preferred_element_type=F32)
            kt = (kvt[:DH] * QSCALE).astype(BF16).astype(F32)
            k2 = (kt * kt).reshape(DH // 8, 8, T).sum(0).sum(0, keepdims=True)
            km = kmax[...]
            for t in range(T // 128):
                ts = slice(t * 128, (t + 1) * 128)
                vt[i * (T // 128) + t] = _pack(kvt[DH:, ts])
                km = jnp.maximum(km, k2[:, ts])
                kk = jnp.concatenate([kt[:, ts], jnp.zeros((128 - DH, 128), F32)], axis=0).T
                kk = jnp.where(_iota((128, 128), 1) == DH + 1, 1.0, kk)
                kk = jnp.concatenate([kk[g * 16:(g + 1) * 16] for g in reversed(range(8))], axis=0)
                ka[_ds((i * (T // 128) + t) * 64, 64), :] = _pack(kk)
            kmax[...] = km
            return k2[:, :128]

        def q(c, deps):
            r = _iota((16, 128), 0)
            y = _mm(_bf(_after(src[...], deps)), _bf(wq[:, c * 256:(c + 1) * 256]))
            for t in range(T // 128):
                for g2 in range(2):
                    qt = y[t * 128:(t + 1) * 128, g2 * 128:(g2 + 1) * 128].T
                    qh = [qt[h * DH:(h + 1) * DH] for h in range(4)]
                    n2 = [(a * a).reshape(DH // 8, 8, 128).sum(0).sum(0, keepdims=True) for a in qh]
                    for h in range(4):
                        nq = jnp.sqrt(n2[h]) * (-UP * UP)
                        aug = jnp.where(r == 0, nq, jnp.where(r == 1, SHIFT, 0.0))
                        qa[i * (T // 128) + t, c * 2 + g2, :, h * 128:(h + 1) * 128] = (
                            jnp.concatenate([_pack(qh[h]), _pack(aug)], axis=0))
            return y[:8, :128]

        return [functools.partial(q, c) for c in range(D // 256)], kv

    def st_fix_k():
        km = jnp.sqrt(jnp.max(kmax[...], axis=1, keepdims=True)) * (UP * UP)
        kk = _bf(ka[...]).astype(F32)
        ka[...] = _pack(jnp.where(_iota(kk.shape, 1) == DH, km, kk))

    def put_o(tb, g, ot):
        ot = jnp.concatenate([ot[:, h * 128:(h + 1) * 128] for h in range(4)], axis=0)
        oe[_ds(tb * 64, 64), _ds(g * 128, 128)] = _pack(ot.T)

    def st_attn(tb):
        nt = S // 128
        steps = [(g, t) for g in range(U) for t in range(nt)]
        s, acc, l = {}, {}, {}
        flag = [bad[...]]

        def qk(n):
            g, t = steps[n]
            s[n] = _mm(_bf(ka[t * 64:(t + 1) * 64, :])[:, :KA], _bf(qa[tb, g]))

        def pv(n):
            g, t = steps[n]
            p = jnp.exp2(s.pop(n))
            ps = p.reshape(16, 8, 512).sum(0)
            p = jnp.concatenate([p[j * 16:(j + 1) * 16] for j in reversed(range(8))], axis=0)
            o = _mm(_bf(vt[t]), p.astype(BF16))
            acc[g], l[g] = (o, ps) if t == 0 else (acc[g] + o, l[g] + ps)
            if t == nt - 1:
                ll = l.pop(g).sum(0, keepdims=True)
                ok = jnp.logical_and(ll >= L_LO, ll <= L_HI)
                flag[0] = jnp.maximum(flag[0], jnp.where(ok, 0.0, 1.0))
                put_o(tb, g, acc.pop(g) * (1.0 / ll))

        for n in range(len(steps) + 1):
            if n < len(steps):
                qk(n)
            if n > 0:
                pv(n - 1)
        bad[...] = flag[0]

    def st_attn_exact(u):
        tb, g = u // U, u % U
        q = _bf(qa[tb, g, :DH // 2, :])

        def scores(t):
            kk = jnp.concatenate([ka[_ds(t * 64 + j * 8, 8), :] for j in reversed(range(8))], axis=0)
            return _mm(_bf(kk)[:, :DH], q)

        m = jax.lax.fori_loop(
            0, S // 128, lambda t, m: jnp.maximum(m, jnp.max(scores(t), axis=0, keepdims=True)),
            jnp.full((1, 512), -jnp.inf, F32))

        def body(t, c):
            p = jnp.exp2(scores(t) - m)
            return c[0] + _mm(_bf(vt[t]), p.astype(BF16)), c[1] + jnp.sum(p, axis=0, keepdims=True)

        acc, l = jax.lax.fori_loop(0, S // 128, body, (jnp.zeros((DH, 512), F32), jnp.zeros((1, 512), F32)))
        put_o(tb, g, acc * (1.0 / l))

    def st_out(j, par, w, o_ref):
        def step(c, deps):
            cs = slice(c * 256, (c + 1) * 256)
            rows = _ds((2 * j + par) * TP, TP)
            y = _mm(_bf(_after(o_ref[rows, :], deps)), _bf(w[:, cs]))
            x = xr[par][_ds(j * T, T), cs] + y
            xr[par][_ds(j * T, T), cs] = x
            if w is wobp:
                xio[rows, cs] = _pack(x)
            return y[:8, :128]
        return [functools.partial(step, c) for c in range(D // 256)]

    def st_qkv_b(par):
        def step(c, deps):
            y = _mm(_bf(_after(xn[par][...], deps)), _bf(wp[:, c * 256:(c + 1) * 256]))
            bufs[par][2 * c, HALO:, :] = y[:, :128]
            bufs[par][2 * c + 1, HALO:, :] = y[:, 128:]
            return y[:8, :128]
        return [functools.partial(step, c) for c in range(3 * D // 256)]

    def halo(par, is_first=None):
        h = bufs[1 - par][8:24, T:T + HALO, :]
        if is_first is not None:
            h = jnp.where(is_first, jnp.broadcast_to(bufs[par][8:24, HALO:HALO + 1, :], h.shape), h)
        bufs[par][8:24, :HALO, :] = h

    def st_window(j, par):
        buf = bufs[par]

        def probs(lg, r):
            even = (_iota((8, 128), 1) & 1) == 0
            for w in range(W):
                y = lg[w] + pltpu.roll(lg[w], 64, 1)
                y = (y + jnp.where(even, pltpu.roll(y, 127, 1), pltpu.roll(y, 1, 1))) * QSCALE
                if par == 0 and r < DIL * w:
                    y = jnp.where(_iota((8, 128), 0) + (j * 2 * T + r) >= DIL * w, y, NEG)
                lg[w] = y
            m = lg[0]
            for w in range(1, W):
                m = jnp.maximum(m, lg[w])
            p = [jnp.exp2(y - m) for y in lg]
            den = p[0]
            for w in range(1, W):
                den = den + p[w]
            inv = 1.0 / den
            return [y * inv for y in p]

        def windows(c, r):
            rows = {e: buf[c, pl.ds(HALO + r + e, 8), :] for e in range(8, -DIL * W, -DIL)}
            return [[rows[8 * hf - DIL * w] for w in range(W)] for hf in range(2)]

        def step(r, deps):
            lg = [[None] * W, [None] * W]
            for c in range(8):
                kk = windows(8 + c, r)
                for hf in range(2):
                    qc = _after(buf[c, HALO + r + 8 * hf:HALO + r + 8 * hf + 8, :], deps)
                    for w in range(W):
                        pr = qc * kk[hf][w]
                        lg[hf][w] = pr if c == 0 else lg[hf][w] + pr
            ps = [probs(lg[hf], r + 8 * hf) for hf in range(2)]
            for c in range(8):
                vv = windows(16 + c, r)
                halves = []
                for hf in range(2):
                    o = ps[hf][0] * vv[hf][0]
                    for w in range(1, W):
                        o = o + ps[hf][w] * vv[hf][w]
                    halves.append(o)
                y = _pack(jnp.concatenate(halves, axis=0))
                ob[par][_ds((2 * j + par) * TP + r // 2, 8), c * 128:(c + 1) * 128] = y
            return y

        return [functools.partial(step, r) for r in range(0, T, 16)]

    def st_permute(n, wt):
        lane = _iota((128, 128), 1)
        src = (lane & 64) + (lane & 1) * 32 + ((lane & 63) >> 1)
        for t in range(8):
            y = wqkv[_ds(wt * 128, 128), _ds(n * D + t * 128, 128)].T
            for h in range(4):
                tmp[pl.ds((4 * t + h) * (DH + 1), DH), :] = y[h * DH:(h + 1) * DH]
        for u in range(8):
            y = jnp.concatenate([tmp[pl.ds(4 * u + e, H, stride=DH + 1), :] for e in range(4)], axis=0).T
            wp[_ds(wt * 128, 128), _ds(n * D + u * 128, 128)] = jnp.take_along_axis(y, src, axis=1)

    def st_permute_o(t):
        cs = _ds(t * 128, 128)
        for h in range(H):
            tmp[pl.ds(h * (DH // 2 + 1), DH // 2), :] = wob[h * DH // 2:(h + 1) * DH // 2, cs]
        for e in range(DH // 2):
            wobp[e * H:(e + 1) * H, cs] = tmp[pl.ds(e, H, stride=DH // 2 + 1), :]

    NP = NB // 2

    def qkv_a(j, from_input):
        for par, jn in ((0, j), (1, jnp.minimum(j + 1, NP - 1))):
            qs, kv = st_qkv_a(2 * j + par, xn[par])
            _overlap(j, [kv] + qs, st_ln(jn, 1 - par, xn[1 - par], from_input))

    kmax[...] = jnp.zeros(kmax.shape, F32)
    b1[...] = jnp.zeros(b1.shape, F32)
    x_copy(1).start()
    x_copy(2).start()
    x_copy(0).wait()
    for f in st_ln(0, 0, xn0, True):
        f([])
    for c in w_copies[:3]:
        c.wait()

    @pl.loop(0, NP)
    def _(j):
        x_copy(2 * j + 1).wait()

        @pl.when(j + 1 < NP)
        def _():
            x_copy(2 * j + 2).wait()
            x_copy(2 * j + 3).start()

        @pl.when(j + 2 < NP)
        def _():
            x_copy(2 * j + 4).start()

        @pl.when(j == 1)
        def _():
            for c in w_copies[3:]:
                c.start()

        qkv_a(j, True)

    for c in w_copies[3:]:
        c.wait()

    @pl.loop(0, 12)
    def _(u):
        st_permute(u // 4, u % 4)

    @pl.loop(0, 8)
    def _(t):
        st_permute_o(t)

    @pl.loop(0, 2)
    def _(layer):
        st_fix_k()
        bad[...] = jnp.zeros(bad.shape, F32)

        @pl.loop(0, S // 128)
        def _(tb):
            st_attn(tb)

        @pl.when(jnp.max(bad[...]) > 0.0)
        def _():
            @pl.loop(0, (S // 128) * U)
            def _(u):
                st_attn_exact(u)

        @pl.loop(0, NP)
        def _(j):
            _overlap(j, st_out(j, 0, woa, oe))
            _overlap(j, st_out(j, 1, woa, oe), st_ln(0, 0, xn0))

        @pl.loop(0, NP)
        def _(j):
            _overlap(j, st_qkv_b(0), st_ln(j, 1, xn1), st_window(jnp.maximum(j - 1, 0), 1))
            halo(0, j == 0)
            _overlap(j, st_qkv_b(1), st_ln(jnp.minimum(j + 1, NP - 1), 0, xn0), st_window(j, 0))
            halo(1)

        def out_b(j, first=False):
            _overlap(layer, st_out(j, 0, wobp, oe), st_window(NP - 1, 1) if first else [])
            _overlap(layer, st_out(j, 1, wobp, oo), st_ln(0, 0, xn0) if first else [])

            @pl.when(layer == 1)
            def _():
                out_copy(2 * j).start()
                out_copy(2 * j + 1).start()

        out_b(0, True)
        pl.loop(1, NP)(out_b)

        @pl.when(layer == 0)
        def _():
            kmax[...] = jnp.zeros(kmax.shape, F32)

            @pl.loop(0, NP)
            def _(j):
                qkv_a(j, False)

    for i in range(NB):
        out_copy(i).wait()


@jax.jit
def pallas_interleave_layers__grouped_kv_mqa__sliding_local_dilated__prompt_kernel(
    A_x: jax.Array,
    A_wq: jax.Array,
    A_wk: jax.Array,
    A_wv: jax.Array,
    A_wo: jax.Array,
    B_x: jax.Array,
    B_wqkv: jax.Array,
    B_wo: jax.Array,
):
    del B_x
    vm = pltpu.VMEM
    out = pl.pallas_call(
        _kernel,
        out_shape=jax.ShapeDtypeStruct((S, D), BF16),
        in_specs=[pl.BlockSpec(memory_space=pl.ANY)] * 7,
        out_specs=pl.BlockSpec(memory_space=pl.ANY),
        scratch_shapes=[
            vm((S // 2, D), U32),
            vm((D // 2, D), U32), vm((D // 2, D), U32),
            vm((D // 2, 3 * D), U32), vm((D // 2, D), U32),
            vm((D // 2, 3 * D), U32), vm((D // 2, D), U32),
            vm((DH, D), U32),
            vm((D + H, 128), U32),
            vm((S // 2, D), F32), vm((S // 2, D), F32),
            vm((S // 2, D), U32), vm((S // 2, D), U32),
            vm((T // 2, D), U32), vm((T // 2, D), U32),
            vm((S // 128, U, KA // 2, 512), U32),
            vm((S // 2, 128), U32), vm((S // 128, DH // 2, 128), U32),
            vm((1, 128), F32), vm((1, 512), F32),
            vm((24, T + HALO, 128), F32), vm((24, T + HALO, 128), F32),
            pltpu.SemaphoreType.DMA((NB,)), pltpu.SemaphoreType.DMA((6,)), pltpu.SemaphoreType.DMA((NB,)),
        ],
        compiler_params=pltpu.CompilerParams(vmem_limit_bytes=110 * 1024 * 1024),
        name="four_layers",
    )(A_x.reshape(S, D), A_wq, A_wk.T, A_wv.T, A_wo, B_wqkv, B_wo)
    return out.reshape(1, S, D)
```

```python
import functools

import jax
import jax.numpy as jnp
import jax.experimental.pallas as pl
import jax.experimental.pallas.tpu as pltpu

F32, BF16, U32 = jnp.float32, jnp.bfloat16, jnp.uint32

S, D, H, DH = 2048, 1024, 32, 32
W, DIL = 8, 2
EPS = 1e-5
LOG2E = 1.4426950408889634
QSCALE = DH ** -0.5 * LOG2E
NEG = -1e9 * LOG2E

T = 256
NB = S // T
KA = 48
HALO = 16
U = 8
TU = 1
SHIFT = 20.0
L_LO, L_HI = 2.0 ** -40, 2.0 ** 33


def _mm(a, b):
    return jnp.dot(a, b, preferred_element_type=F32)


def _pack(x):
    return pltpu.bitcast(x.astype(BF16), U32)


def _bf(x):
    return pltpu.bitcast(x, BF16)


def _ln(x):
    m = jnp.mean(x, axis=-1, keepdims=True)
    c = x - m
    v = jnp.mean(c * c, axis=-1, keepdims=True)
    return c * jax.lax.rsqrt(v + EPS)


def _total(xs):
    return functools.reduce(jnp.add, xs)


def _norm(sq):
    return sq * jax.lax.rsqrt(sq + 1e-30)


def _iota(shape, dim):
    return jax.lax.broadcasted_iota(jnp.int32, shape, dim)


def _ds(start, n):
    return pl.ds(start if isinstance(start, int) else pl.multiple_of(start, 8), n)


def _after(x, deps, rows=(0,)):
    for r, ds in zip(rows, deps):
        for keep, d in ds:
            parts = [jnp.where(keep, x[r:r + 8, :128], pltpu.bitcast(d, x.dtype))]
            if x.shape[1] > 128:
                parts = [jnp.concatenate(parts + [x[r:r + 8, 128:]], axis=1)]
            parts = ([x[:r]] if r else []) + parts + ([x[r + 8:]] if r + 8 < x.shape[0] else [])
            x = jnp.concatenate(parts, axis=0)
    return x


def _overlap(j, mms, *sides, gates=2):
    keep = _iota((8, 128), 0) + j >= 0
    done = [[] for _ in range(len(mms) * gates + 1)]
    todo = [[] for _ in done]
    for steps, lo, hi in sides:
        for m, f in enumerate(steps):
            todo[lo + m * (hi + 1 - lo) // len(steps)].append(f)
    for n, mm in enumerate(mms):
        gs = range(n * gates, (n + 1) * gates)
        for g in gs:
            done[g] = [(keep, f()) for f in todo[g]]
        mm([done[g] for g in gs])
    for f in todo[-1]:
        f()


def _kernel(x_hbm, wq_hbm, wkt_hbm, wvt_hbm, woa_hbm, wqkv_hbm, wob_hbm, out_hbm,
            xio, wq, woa, wqkv, wob, wp, wobp, wkvt, tmp, tmpo,
            xe, xo, oe, oo, xn0, xn1, qa, ka, vt, kmax, bad,
            qkv, pw, sem_x, sem_w, sem_o):
    xr, ob, xn = (xe, xo), (oe, oo), (xn0, xn1)
    TP = T // 2

    def x_copy(i):
        return pltpu.make_async_copy(x_hbm.bitcast(U32).at[_ds(i * TP, TP)], xio.at[_ds(i * TP, TP)], sem_x.at[i])

    def out_copy(i):
        return pltpu.make_async_copy(xio.at[_ds(i * TP, TP)], out_hbm.bitcast(U32).at[_ds(i * TP, TP)], sem_o.at[i])

    w_copies = [pltpu.make_async_copy(s.bitcast(U32), d, sem_w.at[n]) for n, (s, d) in enumerate(
        [(wkt_hbm, wkvt.at[:DH // 2]), (wvt_hbm, wkvt.at[DH // 2:]), (wq_hbm, wq),
         (wqkv_hbm, wqkv), (wob_hbm, wob), (woa_hbm, woa)])]
    x_copy(0).start()
    for c in w_copies[:3]:
        c.start()

    def st_ln(j, par, dst, from_input=False):
        def step(r):
            if from_input:
                x = _bf(xio[_ds((2 * j + par) * TP + r // 2, 8), :]).astype(F32)
                xr[par][_ds(j * T + r, 16), :] = x
            else:
                x = xr[par][_ds(j * T + r, 16), :]
            y = _ln(x)
            dst[r // 2:r // 2 + 8, :] = _pack(y)
            return _total([y[a:a + 8, b:b + 128] for a in (0, 8) for b in range(0, D, 128)])
        return [functools.partial(step, r) for r in range(0, T, 16)]

    def st_qkv_a(i, src):
        def kv(deps):
            kvt = jax.lax.dot_general(_bf(_after(wkvt[...], deps)), _bf(src[...]), (((1,), (1,)), ((), ())),
                                      preferred_element_type=F32)
            kt = (kvt[:DH] * QSCALE).astype(BF16).astype(F32)
            k2 = (kt * kt).reshape(DH // 8, 8, T).sum(0).sum(0, keepdims=True)
            km = kmax[...]
            for t in range(T // 128):
                ts = slice(t * 128, (t + 1) * 128)
                vt[i * (T // 128) + t] = _pack(kvt[DH:, ts])
                km = jnp.maximum(km, k2[:, ts])
                kk = jnp.concatenate([kt[:, ts], jnp.zeros((128 - DH, 128), F32)], axis=0).T
                kk = jnp.where(_iota((128, 128), 1) == DH + 1, 1.0, kk)
                kk = jnp.concatenate([kk[g * 16:(g + 1) * 16] for g in reversed(range(8))], axis=0)
                ka[_ds((i * (T // 128) + t) * 64, 64), :] = _pack(kk)
            kmax[...] = km

        def q(c, deps):
            r = _iota((16, 128), 0)
            y = _mm(_bf(src[...]), _bf(_after(wq[:, c * 256:(c + 1) * 256], deps, (0, D // 4))))
            for t in range(T // 128):
                for g2 in range(2):
                    qt = y[t * 128:(t + 1) * 128, g2 * 128:(g2 + 1) * 128].T
                    qh = [qt[h * DH:(h + 1) * DH] for h in range(4)]
                    n2 = [(a * a).reshape(DH // 8, 8, 128).sum(0).sum(0, keepdims=True) for a in qh]
                    aug = _pack(jnp.concatenate(
                        [jnp.where(r == 0, -_norm(a), jnp.where(r == 1, SHIFT, 0.0)) for a in n2], axis=0))
                    qp = _pack(qt)
                    for h in range(4):
                        dst = qa.at[i * (T // 128) + t, c * 2 + g2]
                        dst[:DH // 2, h * 128:(h + 1) * 128] = qp[h * 16:(h + 1) * 16]
                        dst[DH // 2:, h * 128:(h + 1) * 128] = aug[h * 8:(h + 1) * 8]

        return [functools.partial(q, c) for c in range(D // 256)], kv

    def st_fix_k():
        km = _norm(jnp.max(kmax[...], axis=1, keepdims=True))
        kk = _bf(ka[...]).astype(F32)
        ka[...] = _pack(jnp.where(_iota(kk.shape, 1) == DH, km, kk))

    def put_o(tb, g, ot):
        ot = jnp.concatenate([ot[:, h * 128:(h + 1) * 128] for h in range(4)], axis=0)
        oe[_ds(tb * 64, 64), _ds(g * 128, 128)] = _pack(ot.T)

    def st_attn(j):
        nt = S // 128
        steps = [(j * TU + i, g, t) for i in range(TU) for g in range(U) for t in range(nt)]
        s, acc, l = {}, {}, {}
        flag = [bad[...]]

        def qk(n, deps):
            tb, g, t = steps[n]
            s[n] = (_mm(_bf(_after(ka[t * 64:(t + 1) * 64, :], deps))[:, :KA], _bf(qa[tb, g])))

        def pv(n):
            tb, g, t = steps[n]
            p = jnp.exp2(s.pop(n))
            ps = p.reshape(16, 8, 512).sum(0)
            p = jnp.concatenate([p[j * 16:(j + 1) * 16] for j in reversed(range(8))], axis=0)
            o = _mm(_bf(vt[t]), p.astype(BF16))
            acc[0], l[0] = (o, ps) if t == 0 else (acc[0] + o, l[0] + ps)
            if t == nt - 1:
                ll = l.pop(0).sum(0, keepdims=True)
                ok = jnp.logical_and(ll >= L_LO, ll <= L_HI)
                flag[0] = jnp.maximum(flag[0], jnp.where(ok, 0.0, 1.0))
                put_o(tb, g, acc.pop(0) * (1.0 / ll))

        def step(n, deps):
            if n < len(steps):
                qk(n, deps)
            if n > 0:
                pv(n - 1)

        side = [f for i in range(TU) for f in st_permute(j * TU + i)]
        _overlap(j, [functools.partial(step, n) for n in range(len(steps) + 1)],
                 (side, 4, len(steps) - 2), gates=1)
        bad[...] = flag[0]

    def st_attn_exact(u):
        tb, g = u // U, u % U
        q = _bf(qa[tb, g, :DH // 2, :])

        def scores(t):
            kk = jnp.concatenate([ka[_ds(t * 64 + j * 8, 8), :] for j in reversed(range(8))], axis=0)
            return _mm(_bf(kk)[:, :DH], q)

        m = jax.lax.fori_loop(
            0, S // 128, lambda t, m: jnp.maximum(m, jnp.max(scores(t), axis=0, keepdims=True)),
            jnp.full((1, 512), -jnp.inf, F32))

        def body(t, c):
            p = jnp.exp2(scores(t) - m)
            return c[0] + _mm(_bf(vt[t]), p.astype(BF16)), c[1] + jnp.sum(p, axis=0, keepdims=True)

        acc, l = jax.lax.fori_loop(0, S // 128, body, (jnp.zeros((DH, 512), F32), jnp.zeros((1, 512), F32)))
        put_o(tb, g, acc * (1.0 / l))

    def st_out(j, par, w, o_ref):
        def step(c, deps):
            cs = slice(c * 256, (c + 1) * 256)
            rows = _ds((2 * j + par) * TP, TP)
            y = _mm(_bf(o_ref[rows, :]), _bf(_after(w[:, cs], deps, (0, D // 4))))
            x = xr[par][_ds(j * T, T), cs] + y
            xr[par][_ds(j * T, T), cs] = x
            if w is wobp:
                xio[rows, cs] = _pack(x)
        return [functools.partial(step, c) for c in range(D // 256)]

    def st_qkv_b(j, par):
        def step(c, deps):
            if c % 4 == 0 and c:
                cs = slice(2 * c, 2 * c + 8)
                qkv[cs, :HALO, :] = qkv[cs, T:, :]
            y = _mm(_bf(xn[par][...]), _bf(_after(wp[:, c * 256:(c + 1) * 256], deps, (0, D // 4))))
            qkv[2 * c, HALO:, :] = y[:, :128]
            qkv[2 * c + 1, HALO:, :] = y[:, 128:]
            if c == 11 and par == 0:
                first = jnp.broadcast_to(qkv[16:, HALO:HALO + 1, :], (8, HALO, 128))
                qkv[16:, :HALO, :] = jnp.where(j == 0, first, qkv[16:, :HALO, :])
        return [functools.partial(step, c) for c in range(3 * D // 256)]

    def windows(c, r):
        rows = {e: qkv[c, pl.ds(HALO + r + e, 8), :] for e in range(8, -DIL * W, -DIL)}
        return [[rows[8 * hf - DIL * w] for w in range(W)] for hf in range(2)]

    def st_probs(j, par):
        def softmax(lg, r):
            even = (_iota((8, 128), 1) & 1) == 0
            for w in range(W):
                y = lg[w] + pltpu.roll(lg[w], 64, 1)
                y = (y + jnp.where(even, pltpu.roll(y, 127, 1), pltpu.roll(y, 1, 1))) * QSCALE
                if par == 0 and r < DIL * w:
                    y = jnp.where(_iota((8, 128), 0) + (j * 2 * T + r) >= DIL * w, y, NEG)
                lg[w] = y
            m = lg[0]
            for w in range(1, W):
                m = jnp.maximum(m, lg[w])
            p = [jnp.exp2(y - m) for y in lg]
            den = p[0]
            for w in range(1, W):
                den = den + p[w]
            inv = 1.0 / den
            p = [y * inv for y in p]
            for w in range(W):
                pw[w, r:r + 8, :] = p[w]
            return p

        def step(r):
            lg = [[None] * W, [None] * W]
            for c in range(8):
                kk = windows(8 + c, r)
                for hf in range(2):
                    qc = qkv[c, HALO + r + 8 * hf:HALO + r + 8 * hf + 8, :]
                    for w in range(W):
                        pr = qc * kk[hf][w]
                        lg[hf][w] = pr if c == 0 else lg[hf][w] + pr
            return _total(softmax(lg[0], r) + softmax(lg[1], r + 8))

        return [functools.partial(step, r) for r in range(0, T, 16)]

    def st_mix(j, par):
        def step(r):
            ps = [[pw[w, r + 8 * hf:r + 8 * hf + 8, :] for w in range(W)] for hf in range(2)]
            ys = []
            for c in range(8):
                vv = windows(16 + c, r)
                halves = []
                for hf in range(2):
                    o = ps[hf][0] * vv[hf][0]
                    for w in range(1, W):
                        o = o + ps[hf][w] * vv[hf][w]
                    halves.append(o)
                ys += halves
                ob[par][_ds((2 * j + par) * TP + r // 2, 8), c * 128:(c + 1) * 128] = (
                    _pack(jnp.concatenate(halves, axis=0)))
            return _total(ys)

        return [functools.partial(step, r) for r in range(0, T, 16)]

    def st_permute(u):
        n, rows = jnp.minimum(u // 4, 2), _ds(u % 4 * 128, 128)
        cs = _ds(u % 8 * 128, 128)

        def gather(t):
            y = wqkv[rows, _ds(n * D + t * 128, 128)].T
            for h in range(4):
                tmp[pl.ds((4 * t + h) * (DH + 1), DH), :] = y[h * DH:(h + 1) * DH]
                h = 4 * t + h
                tmpo[pl.ds(h * (DH // 2 + 1), DH // 2), :] = wob[h * DH // 2:(h + 1) * DH // 2, cs]
            return y[-8:]

        def scatter(t):
            lane = _iota((128, 128), 1)
            src = (lane & 64) + (lane & 1) * 32 + ((lane & 63) >> 1)
            y = jnp.concatenate([tmp[pl.ds(4 * t + e, H, stride=DH + 1), :] for e in range(4)], axis=0)
            y = jnp.take_along_axis(y.T, src, axis=1)
            wp[rows, _ds(n * D + t * 128, 128)] = y
            for e in (2 * t, 2 * t + 1):
                wobp[e * H:(e + 1) * H, cs] = tmpo[pl.ds(e, H, stride=DH // 2 + 1), :]
            return y[-8:]

        return [functools.partial(f, t) for f in (gather, scatter) for t in range(8)]

    NP = NB // 2

    def qkv_a(j, from_input):
        for par, jn in ((0, j), (1, jnp.minimum(j + 1, NP - 1))):
            qs, kv = st_qkv_a(2 * j + par, xn[par])
            _overlap(j, qs + [kv], (st_ln(jn, 1 - par, xn[1 - par], from_input), 2, 8))

    kmax[...] = jnp.zeros(kmax.shape, F32)
    qkv[8:] = jnp.zeros((16, T + HALO, 128), F32)
    pw[...] = jnp.zeros(pw.shape, F32)
    x_copy(1).start()
    x_copy(2).start()
    x_copy(0).wait()
    for f in st_ln(0, 0, xn0, True):
        f()
    for c in w_copies[:3]:
        c.wait()

    @pl.loop(0, NP)
    def _(j):
        x_copy(2 * j + 1).wait()

        @pl.when(j + 1 < NP)
        def _():
            x_copy(2 * j + 2).wait()
            x_copy(2 * j + 3).start()

        @pl.when(j + 2 < NP)
        def _():
            x_copy(2 * j + 4).start()

        @pl.when(j == 1)
        def _():
            for c in w_copies[3:]:
                c.start()

        qkv_a(j, True)

    for c in w_copies[3:]:
        c.wait()

    @pl.loop(0, 2)
    def _(layer):
        st_fix_k()
        bad[...] = jnp.zeros(bad.shape, F32)

        @pl.loop(0, S // 128 // TU)
        def _(j):
            st_attn(j)

        @pl.when(jnp.max(bad[...]) > 0.0)
        def _():
            @pl.loop(0, (S // 128) * U)
            def _(u):
                st_attn_exact(u)

        @pl.loop(0, NP)
        def _(j):
            _overlap(j, st_out(j, 0, woa, oe) + st_out(j, 1, woa, oe), (st_ln(0, 0, xn0), 11, 15))

        @pl.loop(0, NP)
        def _(j):
            _overlap(j, st_qkv_b(j, 0) + st_qkv_b(j, 1),
                     (st_mix(jnp.maximum(j - 1, 0), 1), 2, 9), (st_ln(j, 1, xn1), 10, 17), (st_probs(j, 0), 19, 24),
                     (st_mix(j, 0), 28, 40), (st_ln(jnp.minimum(j + 1, NP - 1), 0, xn0), 36, 41),
                     (st_probs(j, 1), 42, 48))

        def out_b(j, first=False):
            sides = [(st_mix(NP - 1, 1), 2, 7), (st_ln(0, 0, xn0), 11, 15)] if first else []
            _overlap(layer, st_out(j, 0, wobp, oe) + st_out(j, 1, wobp, oo), *sides)

            @pl.when(layer == 1)
            def _():
                out_copy(2 * j).start()
                out_copy(2 * j + 1).start()

        out_b(0, True)
        pl.loop(1, NP)(out_b)

        @pl.when(layer == 0)
        def _():
            kmax[...] = jnp.zeros(kmax.shape, F32)

            @pl.loop(0, NP)
            def _(j):
                qkv_a(j, False)

    for i in range(NB):
        out_copy(i).wait()


@jax.jit
def pallas_interleave_layers__grouped_kv_mqa__sliding_local_dilated__prompt_kernel(
    A_x: jax.Array,
    A_wq: jax.Array,
    A_wk: jax.Array,
    A_wv: jax.Array,
    A_wo: jax.Array,
    B_x: jax.Array,
    B_wqkv: jax.Array,
    B_wo: jax.Array,
):
    del B_x
    vm = pltpu.VMEM
    out = pl.pallas_call(
        _kernel,
        out_shape=jax.ShapeDtypeStruct((S, D), BF16),
        in_specs=[pl.BlockSpec(memory_space=pl.ANY)] * 7,
        out_specs=pl.BlockSpec(memory_space=pl.ANY),
        scratch_shapes=[
            vm((S // 2, D), U32),
            vm((D // 2, D), U32), vm((D // 2, D), U32),
            vm((D // 2, 3 * D), U32), vm((D // 2, D), U32),
            vm((D // 2, 3 * D), U32), vm((D // 2, D), U32),
            vm((DH, D), U32),
            vm((D + H, 128), U32), vm((D // 2 + H, 128), U32),
            vm((S // 2, D), F32), vm((S // 2, D), F32),
            vm((S // 2, D), U32), vm((S // 2, D), U32),
            vm((T // 2, D), U32), vm((T // 2, D), U32),
            vm((S // 128, U, KA // 2, 512), U32),
            vm((S // 2, 128), U32), vm((S // 128, DH // 2, 128), U32),
            vm((1, 128), F32), vm((1, 512), F32),
            vm((24, T + HALO, 128), F32), vm((W, T, 128), F32),
            pltpu.SemaphoreType.DMA((NB,)), pltpu.SemaphoreType.DMA((6,)), pltpu.SemaphoreType.DMA((NB,)),
        ],
        compiler_params=pltpu.CompilerParams(vmem_limit_bytes=110 * 1024 * 1024),
        name="four_layers",
    )(A_x.reshape(S, D), A_wq, A_wk.T, A_wv.T, A_wo, B_wqkv, B_wo)
    return out.reshape(1, S, D)
```

```python
import functools

import jax
import jax.numpy as jnp
import numpy as np
import jax.experimental.pallas as pl
import jax.experimental.pallas.tpu as pltpu

F32, BF16, U32 = jnp.float32, jnp.bfloat16, jnp.uint32

S, D, H, DH = 2048, 1024, 32, 32
W, DIL = 8, 2
EPS = 1e-5
LOG2E = 1.4426950408889634
QSCALE = DH ** -0.5 * LOG2E
NEG = -1e9 * LOG2E

T = 256
NB = S // T
KA = 48
HALO = 16
LEAD = 4
U = 8
TU = 1
SHIFT_BITS = 0x41A00000
L_LO, L_HI = 2.0 ** -40, 2.0 ** 33


def _mm(a, b):
    return jnp.dot(a, b, preferred_element_type=F32)


def _pack(x):
    return pltpu.bitcast(x.astype(BF16), U32)


def _bf(x):
    return pltpu.bitcast(x, BF16)


def _ln(x):
    m = jnp.mean(x, axis=-1, keepdims=True)
    c = x - m
    v = jnp.mean(c * c, axis=-1, keepdims=True)
    return c * jax.lax.rsqrt(v + EPS)


def _total(xs):
    return functools.reduce(jnp.add, xs)


def _norm(sq):
    return sq * jax.lax.rsqrt(sq + 1e-30)


def _iota(shape, dim):
    return jax.lax.broadcasted_iota(jnp.int32, shape, dim)


def _ds(start, n):
    return pl.ds(start if isinstance(start, int) else pl.multiple_of(start, 8), n)


def _after(x, deps, rows=(0,)):
    for r, ds in zip(rows, deps):
        for keep, d in ds:
            parts = [jnp.where(keep, x[r:r + 8, :128], pltpu.bitcast(d, x.dtype))]
            if x.shape[1] > 128:
                parts = [jnp.concatenate(parts + [x[r:r + 8, 128:]], axis=1)]
            parts = ([x[:r]] if r else []) + parts + ([x[r + 8:]] if r + 8 < x.shape[0] else [])
            x = jnp.concatenate(parts, axis=0)
    return x


def _overlap(j, mms, *sides, gates=2):
    keep = _iota((8, 128), 0) + j >= 0
    done = [[] for _ in range(len(mms) * gates + 1)]
    todo = [[] for _ in done]
    for steps, lo, hi, limit in sides:
        for m, f in enumerate(steps):
            g = lo + m * (hi + 1 - lo) // len(steps)
            todo[min(g + LEAD, limit)].append((g, f))
    made = [[]]

    def run(g):
        return [f(lambda x: _after(x, [made[start]])) for start, f in todo[g]]

    for n, mm in enumerate(mms):
        gs = range(n * gates, (n + 1) * gates)
        for g in gs:
            if todo[g]:
                done[g] = [(keep, _total(run(g)))]
        made += [[] if y is None else [(keep, y)] for y in mm([done[g] for g in gs])]
    run(len(done) - 1)


def _ends(y):
    return y[:8, :128], y[-8:, -128:]


def _now(x):
    return x


def _kernel(x_hbm, wq_hbm, wkt_hbm, wvt_hbm, woa_hbm, wqkv_hbm, wob_hbm, out_hbm,
            xio, wq, woa, wqkv, wob, wp, wobp, wkvt, tmp, tmpo,
            xe, xo, oe, oo, xn0, xn1, qa, ka, vt, kmax, bad,
            b0, b1, pw, sem_x, sem_w, sem_o):
    xr, ob, xn = (xe, xo), (oe, oo), (xn0, xn1)
    bufs = (b0, b1)
    TP = T // 2

    def x_copy(i):
        return pltpu.make_async_copy(x_hbm.bitcast(U32).at[_ds(i * TP, TP)], xio.at[_ds(i * TP, TP)], sem_x.at[i])

    def out_copy(i):
        return pltpu.make_async_copy(xio.at[_ds(i * TP, TP)], out_hbm.bitcast(U32).at[_ds(i * TP, TP)], sem_o.at[i])

    w_copies = [pltpu.make_async_copy(s.bitcast(U32), d, sem_w.at[n]) for n, (s, d) in enumerate(
        [(wkt_hbm, wkvt.at[:DH // 2]), (wvt_hbm, wkvt.at[DH // 2:]), (wq_hbm, wq),
         (wqkv_hbm, wqkv), (wob_hbm, wob), (woa_hbm, woa)])]
    x_copy(0).start()
    for c in w_copies[:3]:
        c.start()

    def st_ln(j, par, dst, from_input=False):
        def step(r, start):
            if from_input:
                x = _bf(xio[_ds((2 * j + par) * TP + r // 2, 8), :]).astype(F32)
                xr[par][_ds(j * T + r, 16), :] = x
            else:
                x = xr[par][_ds(j * T + r, 16), :]
            y = _ln(jnp.concatenate([start(x[:8]), start(x[8:])], axis=0))
            dst[r // 2:r // 2 + 8, :] = _pack(y)
            return _total([y[a:a + 8, b:b + 128] for a in (0, 8) for b in range(0, D, 128)])
        return [functools.partial(step, r) for r in range(0, T, 16)]

    def st_qkv_a(i, src):
        def kv(deps):
            kvt = jax.lax.dot_general(_bf(_after(wkvt[...], deps)), _bf(src[...]), (((1,), (1,)), ((), ())),
                                      preferred_element_type=F32)
            kt = (kvt[:DH] * QSCALE).astype(BF16).astype(F32)
            k2 = (kt * kt).reshape(DH // 8, 8, T).sum(0).sum(0, keepdims=True)
            km = kmax[...]
            for t in range(T // 128):
                ts = slice(t * 128, (t + 1) * 128)
                vt[i * (T // 128) + t] = _pack(kvt[DH:, ts])
                km = jnp.maximum(km, k2[:, ts])
                kk = jnp.concatenate([kt[:, ts], jnp.zeros((128 - DH, 128), F32)], axis=0).T
                kk = jnp.where(_iota((128, 128), 1) == DH + 1, 1.0, kk)
                kk = jnp.concatenate([kk[g * 16:(g + 1) * 16] for g in reversed(range(8))], axis=0)
                ka[_ds((i * (T // 128) + t) * 64, 64), :] = _pack(kk)
            kmax[...] = km
            return _ends(kvt)

        def q(c, deps):
            r = _iota((8, 128), 0)
            y = _mm(_bf(src[...]), _bf(_after(wq[:, c * 256:(c + 1) * 256], deps, (0, D // 4))))
            for t in range(T // 128):
                for g2 in range(2):
                    qt = y[t * 128:(t + 1) * 128, g2 * 128:(g2 + 1) * 128].T
                    qh = [qt[h * DH:(h + 1) * DH] for h in range(4)]
                    n2 = [(a * a).reshape(DH // 8, 8, 128).sum(0).sum(0, keepdims=True) for a in qh]
                    for h in range(4):
                        aug = (pltpu.bitcast(-_norm(n2[h]), U32) >> 16) | np.uint32(SHIFT_BITS)
                        dst = qa.at[i * (T // 128) + t, c * 2 + g2]
                        dst[:DH // 2, h * 128:(h + 1) * 128] = _pack(qh[h])
                        dst[DH // 2:, h * 128:(h + 1) * 128] = jnp.where(r == 0, aug, np.uint32(0))
            return _ends(y)

        return [functools.partial(q, c) for c in range(D // 256)], kv

    def st_fix_k():
        km = _norm(jnp.max(kmax[...], axis=1, keepdims=True))
        kk = _bf(ka[...]).astype(F32)
        ka[...] = _pack(jnp.where(_iota(kk.shape, 1) == DH, km, kk))

    def put_o(tb, g, ot):
        ot = jnp.concatenate([ot[:, h * 128:(h + 1) * 128] for h in range(4)], axis=0)
        oe[_ds(tb * 64, 64), _ds(g * 128, 128)] = _pack(ot.T)

    def st_attn(j):
        nt = S // 128
        steps = [(j * TU + i, g, t) for i in range(TU) for g in range(U) for t in range(nt)]
        s, acc, l = {}, {}, {}
        flag = [bad[...]]

        def qk(n, deps):
            tb, g, t = steps[n]
            s[n] = (_mm(_bf(_after(ka[t * 64:(t + 1) * 64, :], deps))[:, :KA], _bf(qa[tb, g])))

        def pv(n):
            tb, g, t = steps[n]
            p = jnp.exp2(s.pop(n))
            ps = p.reshape(16, 8, 512).sum(0)
            p = jnp.concatenate([p[j * 16:(j + 1) * 16] for j in reversed(range(8))], axis=0)
            o = _mm(_bf(vt[t]), p.astype(BF16))
            acc[0], l[0] = (o, ps) if t == 0 else (acc[0] + o, l[0] + ps)
            if t == nt - 1:
                ll = l.pop(0).sum(0, keepdims=True)
                ok = jnp.logical_and(ll >= L_LO, ll <= L_HI)
                flag[0] = jnp.maximum(flag[0], jnp.where(ok, 0.0, 1.0))
                put_o(tb, g, acc.pop(0) * (1.0 / ll))

        def step(n, deps):
            if n < len(steps):
                qk(n, deps)
            if n > 0:
                pv(n - 1)
            return [None]

        side = [f for i in range(TU) for f in st_permute(j * TU + i)]
        _overlap(j, [functools.partial(step, n) for n in range(len(steps) + 1)],
                 (side, 0, len(steps) - 8, len(steps)), gates=1)
        bad[...] = flag[0]

    def st_attn_exact(u):
        tb, g = u // U, u % U
        q = _bf(qa[tb, g, :DH // 2, :])

        def scores(t):
            kk = jnp.concatenate([ka[_ds(t * 64 + j * 8, 8), :] for j in reversed(range(8))], axis=0)
            return _mm(_bf(kk)[:, :DH], q)

        m = jax.lax.fori_loop(
            0, S // 128, lambda t, m: jnp.maximum(m, jnp.max(scores(t), axis=0, keepdims=True)),
            jnp.full((1, 512), -jnp.inf, F32))

        def body(t, c):
            p = jnp.exp2(scores(t) - m)
            return c[0] + _mm(_bf(vt[t]), p.astype(BF16)), c[1] + jnp.sum(p, axis=0, keepdims=True)

        acc, l = jax.lax.fori_loop(0, S // 128, body, (jnp.zeros((DH, 512), F32), jnp.zeros((1, 512), F32)))
        put_o(tb, g, acc * (1.0 / l))

    def st_out(j, par, w, o_ref):
        def step(c, deps):
            cs = slice(c * 256, (c + 1) * 256)
            rows = _ds((2 * j + par) * TP, TP)
            y = _mm(_bf(o_ref[rows, :]), _bf(_after(w[:, cs], deps, (0, D // 4))))
            x = xr[par][_ds(j * T, T), cs] + y
            xr[par][_ds(j * T, T), cs] = x
            if w is wobp:
                xio[rows, cs] = _pack(x)
            return _ends(y)
        return [functools.partial(step, c) for c in range(D // 256)]

    def st_qkv_b(j, par):
        qkv = bufs[par]

        def step(c, deps):
            y = _mm(_bf(xn[par][...]), _bf(_after(wp[:, c * 256:(c + 1) * 256], deps, (0, D // 4))))
            qkv[2 * c, HALO:, :] = y[:, :128]
            qkv[2 * c + 1, HALO:, :] = y[:, 128:]
            if c == 7 or c == 11:
                cs = slice(2 * c - 6, 2 * c + 2)
                h = bufs[1 - par][cs, T:, :]
                if c == 11 and par == 0:
                    h = jnp.where(j == 0, jnp.broadcast_to(qkv[cs, HALO:HALO + 1, :], h.shape), h)
                qkv[cs, :HALO, :] = h
            return _ends(y)
        return [functools.partial(step, c) for c in range(3 * D // 256)]

    def st_probs(j, par):
        buf = bufs[par]

        def softmax(lg, r):
            for w in range(W):
                y = lg[w] * QSCALE
                if par == 0 and r < DIL * w:
                    y = jnp.where(_iota((8, 128), 0) + (j * 2 * T + r) >= DIL * w, y, NEG)
                lg[w] = y
            m = lg[0]
            for w in range(1, W):
                m = jnp.maximum(m, lg[w])
            p = [jnp.exp2(y - m) for y in lg]
            inv = 1.0 / _total(p)
            p = [y * inv for y in p]
            for w in range(W):
                pw[w, r:r + 8, :] = p[w]
            return p

        def step(r, start):
            lg = [[None] * W, [None] * W]
            for c in range(8):
                k = {e: buf[8 + c, pl.ds(HALO + r + e, 8), :] for e in range(-DIL * (W - 1), 9, DIL)}
                for hf in range(2):
                    qc = start(buf[c, HALO + r + 8 * hf:HALO + r + 8 * hf + 8, :])
                    for w in range(W):
                        pr = qc * k[8 * hf - DIL * w]
                        lg[hf][w] = pr if c == 0 else lg[hf][w] + pr
            for shift in (64, 32):
                lg = [[y + pltpu.roll(y, shift, 1) for y in ys] for ys in lg]
            return _total(softmax(lg[0], r) + softmax(lg[1], r + 8))

        return [functools.partial(step, r) for r in range(0, T, 16)]

    def st_mix(j, par):
        buf = bufs[par]

        def step(r, start):
            ps = [[start(pw[w, r + 8 * hf:r + 8 * hf + 8, :]) for w in range(W)] for hf in range(2)]
            ys = []
            for c in range(8):
                v = {e: buf[16 + c, pl.ds(HALO + r + e, 8), :] for e in range(-DIL * (W - 1), 9, DIL)}
                halves = [_total([ps[hf][w] * v[8 * hf - DIL * w] for w in range(W)]) for hf in range(2)]
                ob[par][_ds((2 * j + par) * TP + r // 2, 8), c * 128:(c + 1) * 128] = (
                    _pack(jnp.concatenate(halves, axis=0)))
                ys += halves
            return _total(ys)

        return [functools.partial(step, r) for r in range(0, T, 16)]

    def st_permute(u):
        n, rows = jnp.minimum(u // 4, 2), _ds(u % 4 * 128, 128)
        cs = _ds(u % 8 * 128, 128)

        def gather(t, start):
            y = wqkv[rows, _ds(n * D + t * 128, 128)].T
            for h in range(4 * t, 4 * t + 4):
                tmp[pl.ds(h * (DH + 1), DH), :] = y[h % 4 * DH:(h % 4 + 1) * DH]
                tmpo[h % 2, pl.ds(h // 2 * (DH // 2 + 1), DH // 2), :] = wob[h * DH // 2:(h + 1) * DH // 2, cs]
            return pltpu.bitcast(y[-8:], F32)

        def scatter(t, start):
            y = jnp.concatenate([tmp[pl.ds(4 * t + e, H, stride=DH + 1), :] for e in range(4)], axis=0).T
            wp[rows, _ds(n * D + t * 128, 128)] = y
            for e in (2 * t, 2 * t + 1):
                a, b = [tmpo[k, pl.ds(e, H // 2, stride=DH // 2 + 1), :] for k in range(2)]
                wobp[e * H:e * H + H // 2, cs] = (a & np.uint32(0xFFFF)) | (b << 16)
                wobp[e * H + H // 2:(e + 1) * H, cs] = (a >> 16) | (b & np.uint32(0xFFFF0000))
            return pltpu.bitcast(y[-8:], F32)

        return [functools.partial(f, t) for f in (gather, scatter) for t in range(8)]

    NP = NB // 2

    def qkv_a(j, from_input):
        for par, jn in ((0, j), (1, jnp.minimum(j + 1, NP - 1))):
            qs, kv = st_qkv_a(2 * j + par, xn[par])
            _overlap(j, qs + [kv], (st_ln(jn, 1 - par, xn[1 - par], from_input), 0, 5, 9))

    kmax[...] = jnp.zeros(kmax.shape, F32)
    b1[...] = jnp.zeros(b1.shape, F32)
    pw[...] = jnp.zeros(pw.shape, F32)
    x_copy(0).wait()
    x_copy(1).start()
    for f in st_ln(0, 0, xn0, True):
        f(_now)
    for c in w_copies[:3]:
        c.wait()
    for i in range(2, NB):
        x_copy(i).start()

    @pl.loop(0, NP)
    def _(j):
        x_copy(2 * j + 1).wait()

        @pl.when(j + 1 < NP)
        def _():
            x_copy(2 * j + 2).wait()

        @pl.when(j == 1)
        def _():
            for c in w_copies[3:]:
                c.start()

        qkv_a(j, True)

    for c in w_copies[3:]:
        c.wait()

    @pl.loop(0, 2)
    def _(layer):
        st_fix_k()
        bad[...] = jnp.zeros(bad.shape, F32)

        @pl.loop(0, S // 128 // TU)
        def _(j):
            st_attn(j)

        @pl.when(jnp.max(bad[...]) > 0.0)
        def _():
            @pl.loop(0, (S // 128) * U)
            def _(u):
                st_attn_exact(u)

        @pl.loop(0, NP)
        def _(j):
            _overlap(j, st_out(j, 0, woa, oe) + st_out(j, 1, woa, oe), (st_ln(0, 0, xn0), 9, 12, 15))

        @pl.loop(0, NP)
        def _(j):
            jp, jn = jnp.maximum(j - 1, 0), jnp.minimum(j + 1, NP - 1)
            pr = st_probs(j, 0)
            _overlap(j, st_qkv_b(j, 0) + st_qkv_b(j, 1),
                     (st_probs(jp, 1)[8:], 0, 6, 9), (st_mix(jp, 1), 7, 16, 19), (st_ln(j, 1, xn1), 9, 18, 23),
                     (pr, 17, 28, 31), (st_mix(j, 0), 29, 38, 41), (st_ln(jn, 0, xn0), 33, 42, 48),
                     (st_probs(j, 1)[:8], 39, 44, 48))

        def out_b(j, first=False):
            sides = [(st_probs(NP - 1, 1)[8:], 0, 4, 7),
                     (st_mix(NP - 1, 1), 5, 12, 16), (st_ln(0, 0, xn0), 9, 12, 15)] if first else []
            _overlap(layer, st_out(j, 0, wobp, oe) + st_out(j, 1, wobp, oo), *sides)

            @pl.when(layer == 1)
            def _():
                out_copy(2 * j).start()
                out_copy(2 * j + 1).start()

        out_b(0, True)
        pl.loop(1, NP)(out_b)

        @pl.when(layer == 0)
        def _():
            kmax[...] = jnp.zeros(kmax.shape, F32)

            @pl.loop(0, NP)
            def _(j):
                qkv_a(j, False)

    for i in range(NB):
        out_copy(i).wait()


@jax.jit
def pallas_interleave_layers__grouped_kv_mqa__sliding_local_dilated__prompt_kernel(
    A_x: jax.Array,
    A_wq: jax.Array,
    A_wk: jax.Array,
    A_wv: jax.Array,
    A_wo: jax.Array,
    B_x: jax.Array,
    B_wqkv: jax.Array,
    B_wo: jax.Array,
):
    del B_x
    vm = pltpu.VMEM
    out = pl.pallas_call(
        _kernel,
        out_shape=jax.ShapeDtypeStruct((S, D), BF16),
        in_specs=[pl.BlockSpec(memory_space=pl.ANY)] * 7,
        out_specs=pl.BlockSpec(memory_space=pl.ANY),
        scratch_shapes=[
            vm((S // 2, D), U32),
            vm((D // 2, D), U32), vm((D // 2, D), U32),
            vm((D // 2, 3 * D), U32), vm((D // 2, D), U32),
            vm((D // 2, 3 * D), U32), vm((D // 2, D), U32),
            vm((DH, D), U32),
            vm((D + H, 128), U32), vm((2, D // 4 + H // 2, 128), U32),
            vm((S // 2, D), F32), vm((S // 2, D), F32),
            vm((S // 2, D), U32), vm((S // 2, D), U32),
            vm((T // 2, D), U32), vm((T // 2, D), U32),
            vm((S // 128, U, KA // 2, 512), U32),
            vm((S // 2, 128), U32), vm((S // 128, DH // 2, 128), U32),
            vm((1, 128), F32), vm((1, 512), F32),
            vm((24, T + HALO, 128), F32), vm((24, T + HALO, 128), F32), vm((W, T, 128), F32),
            pltpu.SemaphoreType.DMA((NB,)), pltpu.SemaphoreType.DMA((6,)), pltpu.SemaphoreType.DMA((NB,)),
        ],
        compiler_params=pltpu.CompilerParams(vmem_limit_bytes=110 * 1024 * 1024),
        name="four_layers",
    )(A_x.reshape(S, D), A_wq, A_wk.T, A_wv.T, A_wo, B_wqkv, B_wo)
    return out.reshape(1, S, D)
```

```python
import functools

import jax
import jax.numpy as jnp
import numpy as np
import jax.experimental.pallas as pl
import jax.experimental.pallas.tpu as pltpu

F32, BF16, U32 = jnp.float32, jnp.bfloat16, jnp.uint32

S, D, H, DH = 2048, 1024, 32, 32
W, DIL = 8, 2
EPS = 1e-5
LOG2E = 1.4426950408889634
QSCALE = DH ** -0.5 * LOG2E
NEG = -1e9 * LOG2E

T = 256
NB = S // T
KA = 48
HALO = 16
LEAD = 4
U = 8
TU = 2
NV = 8
VTILES = [(2 * n + 1) * (S // 128) // (2 * NV) for n in range(NV)]
VB = 4
VLO, VHI = 2, 16
SHIFT_BITS = 0x41A00000
L_LO, L_HI = 2.0 ** -40, 2.0 ** 33


def _mm(a, b):
    return jnp.dot(a, b, preferred_element_type=F32)


def _pack(x):
    return pltpu.bitcast(x.astype(BF16), U32)


def _bf(x):
    return pltpu.bitcast(x, BF16)


def _ln(x):
    m = jnp.mean(x, axis=-1, keepdims=True)
    c = x - m
    v = jnp.mean(c * c, axis=-1, keepdims=True)
    return c * jax.lax.rsqrt(v + EPS)


def _total(xs):
    return functools.reduce(jnp.add, xs)


def _norm(sq):
    return sq * jax.lax.rsqrt(sq + 1e-30)


def _iota(shape, dim):
    return jax.lax.broadcasted_iota(jnp.int32, shape, dim)


def _ds(start, n):
    return pl.ds(start if isinstance(start, int) else pl.multiple_of(start, 8), n)


def _after(x, deps, rows=(0,)):
    for r, ds in zip(rows, deps):
        for keep, d in ds:
            parts = [jnp.where(keep, x[r:r + 8, :128], pltpu.bitcast(d, x.dtype))]
            if x.shape[1] > 128:
                parts = [jnp.concatenate(parts + [x[r:r + 8, 128:]], axis=1)]
            parts = ([x[:r]] if r else []) + parts + ([x[r + 8:]] if r + 8 < x.shape[0] else [])
            x = jnp.concatenate(parts, axis=0)
    return x


def _overlap(j, mms, *sides, gates=2):
    keep = _iota((8, 128), 0) + j >= 0
    done = [[] for _ in range(len(mms) * gates + 1)]
    todo = [[] for _ in done]
    for steps, lo, hi, limit in sides:
        for m, f in enumerate(steps):
            g = lo + m * (hi + 1 - lo) // len(steps)
            todo[min(g + LEAD, limit)].append((g, f))
    made = [[]]

    def run(g):
        return [f(lambda x: _after(x, [made[start]])) for start, f in todo[g]]

    for n, mm in enumerate(mms):
        gs = range(n * gates, (n + 1) * gates)
        for g in gs:
            if todo[g]:
                done[g] = [(keep, _total(run(g)))]
        made += [[] if y is None else [(keep, y)] for y in mm([done[g] for g in gs])]
    run(len(done) - 1)


def _ends(y):
    return y[:8, :128], y[-8:, -128:]


def _now(x):
    return x


def _kernel(x_hbm, wq_hbm, wkt_hbm, wvt_hbm, woa_hbm, wqkv_hbm, wob_hbm, out_hbm,
            xio, wq, woa, wqkv, wob, wp, wobp, wkvt, tmp, tmpo,
            xe, xo, oe, oo, xn0, xn1, qa, ka, vt, kb, sp0, sp1, kmax, bad,
            b0, b1, pw, sem_x, sem_w, sem_o):
    xr, ob, xn = (xe, xo), (oe, oo), (xn0, xn1)
    bufs, side_p = (b0, b1), (sp0, sp1)
    TP = T // 2

    def x_copy(i):
        return pltpu.make_async_copy(x_hbm.bitcast(U32).at[_ds(i * TP, TP)], xio.at[_ds(i * TP, TP)], sem_x.at[i])

    def out_copy(i):
        return pltpu.make_async_copy(xio.at[_ds(i * TP, TP)], out_hbm.bitcast(U32).at[_ds(i * TP, TP)], sem_o.at[i])

    w_copies = [pltpu.make_async_copy(s.bitcast(U32), d, sem_w.at[n]) for n, (s, d) in enumerate(
        [(wkt_hbm, wkvt.at[:DH // 2]), (wvt_hbm, wkvt.at[DH // 2:]), (wq_hbm, wq),
         (wqkv_hbm, wqkv), (wob_hbm, wob), (woa_hbm, woa)])]
    x_copy(0).start()
    for c in w_copies[:3]:
        c.start()

    def st_ln(j, par, dst, from_input=False):
        def step(r, start):
            if from_input:
                x = _bf(xio[_ds((2 * j + par) * TP + r // 2, 8), :]).astype(F32)
                xr[par][_ds(j * T + r, 16), :] = x
            else:
                x = xr[par][_ds(j * T + r, 16), :]
            y = _ln(jnp.concatenate([start(x[:8]), start(x[8:])], axis=0))
            dst[r // 2:r // 2 + 8, :] = _pack(y)
            return _total([y[a:a + 8, b:b + 128] for a in (0, 8) for b in range(0, D, 128)])
        return [functools.partial(step, r) for r in range(0, T, 16)]

    def st_qkv_a(i, src):
        def kv(deps):
            kvt = jax.lax.dot_general(_bf(_after(wkvt[...], deps)), _bf(src[...]), (((1,), (1,)), ((), ())),
                                      preferred_element_type=F32)
            kt = (kvt[:DH] * QSCALE).astype(BF16).astype(F32)
            k2 = (kt * kt).reshape(DH // 8, 8, T).sum(0).sum(0, keepdims=True)
            km = kmax[:1]
            for t in range(T // 128):
                ts = slice(t * 128, (t + 1) * 128)
                vt[i * (T // 128) + t] = _pack(kvt[DH:, ts])
                km = jnp.maximum(km, k2[:, ts])
                kk = jnp.concatenate([kt[:, ts], jnp.zeros((128 - DH, 128), F32)], axis=0).T
                kk = jnp.where(_iota((128, 128), 1) == DH + 1, 1.0, kk)
                kk = jnp.concatenate([kk[g * 16:(g + 1) * 16] for g in reversed(range(8))], axis=0)
                ka[_ds((i * (T // 128) + t) * 64, 64), :] = _pack(kk)
            kmax[:1] = km
            return _ends(kvt)

        def q(c, deps):
            r = _iota((8, 128), 0)
            y = _mm(_bf(src[...]), _bf(_after(wq[:, c * 256:(c + 1) * 256], deps, (0, D // 4))))
            for t in range(T // 128):
                for g2 in range(2):
                    qt = y[t * 128:(t + 1) * 128, g2 * 128:(g2 + 1) * 128].T
                    qh = [qt[h * DH:(h + 1) * DH] for h in range(4)]
                    n2 = [(a * a).reshape(DH // 8, 8, 128).sum(0).sum(0, keepdims=True) for a in qh]
                    for h in range(4):
                        aug = (pltpu.bitcast(-_norm(n2[h]), U32) >> 16) | np.uint32(SHIFT_BITS)
                        dst = qa.at[i * (T // 128) + t, c * 2 + g2]
                        dst[:DH // 2, h * 128:(h + 1) * 128] = _pack(qh[h])
                        dst[DH // 2:, h * 128:(h + 1) * 128] = jnp.where(r == 0, aug, np.uint32(0))
            return _ends(y)

        return [functools.partial(q, c) for c in range(D // 256)], kv

    def st_fix_k():
        km = _norm(jnp.max(kmax[:1], axis=1, keepdims=True))
        kk = _bf(ka[...]).astype(F32)
        km = km.astype(BF16).astype(F32)
        ka[...] = _pack(jnp.where(_iota(kk.shape, 1) == DH, km, kk))
        kmax[...] = jnp.broadcast_to(km, kmax.shape)
        for n, t in enumerate(VTILES):
            k = _bf(ka[t * 64 + 56:(t + 1) * 64, :])
            sp0[n * 16:n * 16 + 16, :] = jnp.exp2(_mm(k[:, :KA], _bf(qa[0, 0])))
            k = k.astype(F32)
            for d in range(DH):
                for a in range(2):
                    kb[2 * n + a, d] = jnp.broadcast_to(k[8 * a:8 * a + 8, d:d + 1], (8, 128))

    def put_o(tb, g, ot):
        ot = jnp.concatenate([ot[:, h * 128:(h + 1) * 128] for h in range(4)], axis=0)
        oe[_ds(tb * 64, 64), _ds(g * 128, 128)] = _pack(ot.T)

    def st_attn(j):
        nt = S // 128
        steps = [(j * TU + i, g, t) for i in range(TU) for g in range(U) for t in range(nt)]
        s, acc, l = {}, {}, {}
        flag = [bad[...]]

        keep = _iota((8, 128), 0) + j >= 0
        part = {}

        def qk_vpu(tb, g, h, b, i, start):
            def row(i):
                w = jnp.broadcast_to(qa[tb, g, i:i + 1, h * 128:(h + 1) * 128], (8, 128))
                w = _after(w, [[(keep, start)]])
                return pltpu.bitcast(w << 16, F32), pltpu.bitcast(w & np.uint32(0xFFFF0000), F32)

            if i == 0:
                lo, hi = row(DH // 2)
                part[0] = [lo * kmax[...] + hi] * VB
            lo, hi = row(i)
            part[0] = [y + (kb[b * VB + a, 2 * i] * lo + kb[b * VB + a, 2 * i + 1] * hi)
                       for a, y in enumerate(part[0])]
            if i == DH // 2 - 1:
                side_p[g % 2][b * VB * 8:(b + 1) * VB * 8, h * 128:(h + 1) * 128] = (
                    jnp.exp2(jnp.concatenate(part.pop(0), axis=0)))

        items = [(h, b, i) for h in range(4) for b in range(2 * NV // VB) for i in range(DH // 2)]

        def qk(n, deps):
            tb, g, t = steps[n]
            rows = 56 if t in VTILES else 64
            s[n] = _mm(_bf(_after(ka[t * 64:t * 64 + rows, :], deps))[:, :KA], _bf(qa[tb, g]))
            if g == U - 1:
                tb = jnp.minimum(tb + 1, nt - 1)
            for m, item in enumerate(items):
                at = int(14 * (VLO + m * (VHI - VLO) / len(items)))
                if at // 14 == t:
                    qk_vpu(tb, (g + 1) % U, *item, s[n][8 * (at % 14):8 * (at % 14) + 8, :128])

        def pv(n):
            tb, g, t = steps[n]
            p = jnp.exp2(s.pop(n))
            if t in VTILES:
                r = VTILES.index(t) * 16
                p = jnp.concatenate([p, side_p[g % 2][r:r + 16, :]], axis=0)
            ps = p.reshape(16, 8, 512).sum(0)
            p = jnp.concatenate([p[j * 16:(j + 1) * 16] for j in reversed(range(8))], axis=0)
            o = _mm(_bf(vt[t]), p.astype(BF16))
            acc[0], l[0] = (o, ps) if t == 0 else (acc[0] + o, l[0] + ps)
            if t == nt - 1:
                ll = l.pop(0).sum(0, keepdims=True)
                ok = jnp.logical_and(ll >= L_LO, ll <= L_HI)
                flag[0] = jnp.maximum(flag[0], jnp.where(ok, 0.0, 1.0))
                put_o(tb, g, acc.pop(0) * (1.0 / ll))

        def step(n, deps):
            if n < len(steps):
                qk(n, deps)
            if n > 0:
                pv(n - 1)
            return [None]

        side = [f for i in range(TU) for f in st_permute(j * TU + i)]
        _overlap(j, [functools.partial(step, n) for n in range(len(steps) + 1)],
                 (side, 0, len(steps) - 8, len(steps)), gates=1)
        bad[...] = flag[0]

    def st_attn_exact(u):
        tb, g = u // U, u % U
        q = _bf(qa[tb, g, :DH // 2, :])

        def scores(t):
            kk = jnp.concatenate([ka[_ds(t * 64 + j * 8, 8), :] for j in reversed(range(8))], axis=0)
            return _mm(_bf(kk)[:, :DH], q)

        m = jax.lax.fori_loop(
            0, S // 128, lambda t, m: jnp.maximum(m, jnp.max(scores(t), axis=0, keepdims=True)),
            jnp.full((1, 512), -jnp.inf, F32))

        def body(t, c):
            p = jnp.exp2(scores(t) - m)
            return c[0] + _mm(_bf(vt[t]), p.astype(BF16)), c[1] + jnp.sum(p, axis=0, keepdims=True)

        acc, l = jax.lax.fori_loop(0, S // 128, body, (jnp.zeros((DH, 512), F32), jnp.zeros((1, 512), F32)))
        put_o(tb, g, acc * (1.0 / l))

    def st_out(j, par, w, o_ref):
        def step(c, deps):
            cs = slice(c * 256, (c + 1) * 256)
            rows = _ds((2 * j + par) * TP, TP)
            y = _mm(_bf(o_ref[rows, :]), _bf(_after(w[:, cs], deps, (0, D // 4))))
            x = xr[par][_ds(j * T, T), cs] + y
            xr[par][_ds(j * T, T), cs] = x
            if w is wobp:
                xio[rows, cs] = _pack(x)
            return _ends(y)
        return [functools.partial(step, c) for c in range(D // 256)]

    def st_qkv_b(j, par):
        qkv = bufs[par]

        def step(c, deps):
            y = _mm(_bf(xn[par][...]), _bf(_after(wp[:, c * 256:(c + 1) * 256], deps, (0, D // 4))))
            qkv[2 * c, HALO:, :] = y[:, :128]
            qkv[2 * c + 1, HALO:, :] = y[:, 128:]
            if c == 7 or c == 11:
                cs = slice(2 * c - 6, 2 * c + 2)
                h = bufs[1 - par][cs, T:, :]
                if c == 11 and par == 0:
                    h = jnp.where(j == 0, jnp.broadcast_to(qkv[cs, HALO:HALO + 1, :], h.shape), h)
                qkv[cs, :HALO, :] = h
            return _ends(y)
        return [functools.partial(step, c) for c in range(3 * D // 256)]

    def st_probs(j, par):
        buf = bufs[par]

        def softmax(lg, r):
            for w in range(W):
                y = lg[w] * QSCALE
                if par == 0 and r < DIL * w:
                    y = jnp.where(_iota((8, 128), 0) + (j * 2 * T + r) >= DIL * w, y, NEG)
                lg[w] = y
            m = lg[0]
            for w in range(1, W):
                m = jnp.maximum(m, lg[w])
            p = [jnp.exp2(y - m) for y in lg]
            inv = 1.0 / _total(p)
            p = [y * inv for y in p]
            for w in range(W):
                pw[w, r:r + 8, :] = p[w]
            return p

        def step(r, start):
            lg = [[None] * W, [None] * W]
            for c in range(8):
                k = {e: buf[8 + c, pl.ds(HALO + r + e, 8), :] for e in range(-DIL * (W - 1), 9, DIL)}
                for hf in range(2):
                    qc = start(buf[c, HALO + r + 8 * hf:HALO + r + 8 * hf + 8, :])
                    for w in range(W):
                        pr = qc * k[8 * hf - DIL * w]
                        lg[hf][w] = pr if c == 0 else lg[hf][w] + pr
            for shift in (64, 32):
                lg = [[y + pltpu.roll(y, shift, 1) for y in ys] for ys in lg]
            return _total(softmax(lg[0], r) + softmax(lg[1], r + 8))

        return [functools.partial(step, r) for r in range(0, T, 16)]

    def st_mix(j, par):
        buf = bufs[par]

        def step(r, start):
            ps = [[start(pw[w, r + 8 * hf:r + 8 * hf + 8, :]) for w in range(W)] for hf in range(2)]
            ys = []
            for c in range(8):
                v = {e: buf[16 + c, pl.ds(HALO + r + e, 8), :] for e in range(-DIL * (W - 1), 9, DIL)}
                halves = [_total([ps[hf][w] * v[8 * hf - DIL * w] for w in range(W)]) for hf in range(2)]
                ob[par][_ds((2 * j + par) * TP + r // 2, 8), c * 128:(c + 1) * 128] = (
                    _pack(jnp.concatenate(halves, axis=0)))
                ys += halves
            return _total(ys)

        return [functools.partial(step, r) for r in range(0, T, 16)]

    def st_permute(u):
        n, rows = jnp.minimum(u // 4, 2), _ds(u % 4 * 128, 128)
        cs = _ds(u % 8 * 128, 128)

        def gather(t, start):
            y = wqkv[rows, _ds(n * D + t * 128, 128)].T
            for h in range(4 * t, 4 * t + 4):
                tmp[pl.ds(h * (DH + 1), DH), :] = y[h % 4 * DH:(h % 4 + 1) * DH]
                tmpo[h % 2, pl.ds(h // 2 * (DH // 2 + 1), DH // 2), :] = wob[h * DH // 2:(h + 1) * DH // 2, cs]
            return pltpu.bitcast(y[-8:], F32)

        def scatter(t, start):
            y = jnp.concatenate([tmp[pl.ds(4 * t + e, H, stride=DH + 1), :] for e in range(4)], axis=0).T
            wp[rows, _ds(n * D + t * 128, 128)] = y
            for e in (2 * t, 2 * t + 1):
                a, b = [tmpo[k, pl.ds(e, H // 2, stride=DH // 2 + 1), :] for k in range(2)]
                wobp[e * H:e * H + H // 2, cs] = (a & np.uint32(0xFFFF)) | (b << 16)
                wobp[e * H + H // 2:(e + 1) * H, cs] = (a >> 16) | (b & np.uint32(0xFFFF0000))
            return pltpu.bitcast(y[-8:], F32)

        return [functools.partial(f, t) for f in (gather, scatter) for t in range(8)]

    NP = NB // 2

    def qkv_a(j, from_input):
        for par, jn in ((0, j), (1, jnp.minimum(j + 1, NP - 1))):
            qs, kv = st_qkv_a(2 * j + par, xn[par])
            _overlap(j, qs + [kv], (st_ln(jn, 1 - par, xn[1 - par], from_input), 0, 5, 9))

    kmax[...] = jnp.zeros(kmax.shape, F32)
    b1[...] = jnp.zeros(b1.shape, F32)
    pw[...] = jnp.zeros(pw.shape, F32)
    x_copy(0).wait()
    x_copy(1).start()
    for f in st_ln(0, 0, xn0, True):
        f(_now)
    for c in w_copies[:3]:
        c.wait()
    for i in range(2, NB):
        x_copy(i).start()

    @pl.loop(0, NP)
    def _(j):
        x_copy(2 * j + 1).wait()

        @pl.when(j + 1 < NP)
        def _():
            x_copy(2 * j + 2).wait()

        @pl.when(j == 1)
        def _():
            for c in w_copies[3:]:
                c.start()

        qkv_a(j, True)

    for c in w_copies[3:]:
        c.wait()

    @pl.loop(0, 2)
    def _(layer):
        st_fix_k()
        bad[...] = jnp.zeros(bad.shape, F32)

        @pl.loop(0, S // 128 // TU)
        def _(j):
            st_attn(j)

        @pl.when(jnp.max(bad[...]) > 0.0)
        def _():
            @pl.loop(0, (S // 128) * U)
            def _(u):
                st_attn_exact(u)

        @pl.loop(0, NP)
        def _(j):
            _overlap(j, st_out(j, 0, woa, oe) + st_out(j, 1, woa, oe), (st_ln(0, 0, xn0), 9, 12, 15))

        @pl.loop(0, NP)
        def _(j):
            jp, jn = jnp.maximum(j - 1, 0), jnp.minimum(j + 1, NP - 1)
            pr = st_probs(j, 0)
            _overlap(j, st_qkv_b(j, 0) + st_qkv_b(j, 1),
                     (st_probs(jp, 1)[8:], 0, 6, 9), (st_mix(jp, 1), 7, 16, 19), (st_ln(j, 1, xn1), 9, 18, 23),
                     (pr, 17, 28, 31), (st_mix(j, 0), 29, 38, 41), (st_ln(jn, 0, xn0), 33, 42, 48),
                     (st_probs(j, 1)[:8], 39, 44, 48))

        def out_b(j, first=False):
            sides = [(st_probs(NP - 1, 1)[8:], 0, 4, 7),
                     (st_mix(NP - 1, 1), 5, 12, 16), (st_ln(0, 0, xn0), 9, 12, 15)] if first else []
            _overlap(layer, st_out(j, 0, wobp, oe) + st_out(j, 1, wobp, oo), *sides)

            @pl.when(layer == 1)
            def _():
                out_copy(2 * j).start()
                out_copy(2 * j + 1).start()

        out_b(0, True)
        pl.loop(1, NP)(out_b)

        @pl.when(layer == 0)
        def _():
            kmax[...] = jnp.zeros(kmax.shape, F32)

            @pl.loop(0, NP)
            def _(j):
                qkv_a(j, False)

    for i in range(NB):
        out_copy(i).wait()


@jax.jit
def pallas_interleave_layers__grouped_kv_mqa__sliding_local_dilated__prompt_kernel(
    A_x: jax.Array,
    A_wq: jax.Array,
    A_wk: jax.Array,
    A_wv: jax.Array,
    A_wo: jax.Array,
    B_x: jax.Array,
    B_wqkv: jax.Array,
    B_wo: jax.Array,
):
    del B_x
    vm = pltpu.VMEM
    out = pl.pallas_call(
        _kernel,
        out_shape=jax.ShapeDtypeStruct((S, D), BF16),
        in_specs=[pl.BlockSpec(memory_space=pl.ANY)] * 7,
        out_specs=pl.BlockSpec(memory_space=pl.ANY),
        scratch_shapes=[
            vm((S // 2, D), U32),
            vm((D // 2, D), U32), vm((D // 2, D), U32),
            vm((D // 2, 3 * D), U32), vm((D // 2, D), U32),
            vm((D // 2, 3 * D), U32), vm((D // 2, D), U32),
            vm((DH, D), U32),
            vm((D + H, 128), U32), vm((2, D // 4 + H // 2, 128), U32),
            vm((S // 2, D), F32), vm((S // 2, D), F32),
            vm((S // 2, D), U32), vm((S // 2, D), U32),
            vm((T // 2, D), U32), vm((T // 2, D), U32),
            vm((S // 128, U, KA // 2, 512), U32),
            vm((S // 2, 128), U32), vm((S // 128, DH // 2, 128), U32),
            vm((2 * NV, DH, 8, 128), F32),
            vm((16 * NV, 512), F32), vm((16 * NV, 512), F32),
            vm((8, 128), F32), vm((1, 512), F32),
            vm((24, T + HALO, 128), F32), vm((24, T + HALO, 128), F32), vm((W, T, 128), F32),
            pltpu.SemaphoreType.DMA((NB,)), pltpu.SemaphoreType.DMA((6,)), pltpu.SemaphoreType.DMA((NB,)),
        ],
        compiler_params=pltpu.CompilerParams(vmem_limit_bytes=110 * 1024 * 1024),
        name="four_layers",
    )(A_x.reshape(S, D), A_wq, A_wk.T, A_wv.T, A_wo, B_wqkv, B_wo)
    return out.reshape(1, S, D)
```

```python
import functools

import jax
import jax.numpy as jnp
import numpy as np
import jax.experimental.pallas as pl
import jax.experimental.pallas.tpu as pltpu

F32, BF16, U32 = jnp.float32, jnp.bfloat16, jnp.uint32

S, D, H, DH = 2048, 1024, 32, 32
W, DIL = 8, 2
EPS = 1e-5
LOG2E = 1.4426950408889634
QSCALE = DH ** -0.5 * LOG2E
NEG = -1e9 * LOG2E

T = 256
NB = S // T
KA = 48
HALO = 16
LEAD = 3
U = 8
TU = 2
NV = 8
VTILES = list(range(1, S // 128, 2))
VB = 4
VLO, VHI = 2, 16
SHIFT_BITS = 0x41A00000
L_LO, L_HI = 2.0 ** -40, 2.0 ** 33


def _mm(a, b):
    return jnp.dot(a, b, preferred_element_type=F32)


def _pack(x):
    return pltpu.bitcast(x.astype(BF16), U32)


def _bf(x):
    return pltpu.bitcast(x, BF16)


def _ln(x):
    m = jnp.mean(x, axis=-1, keepdims=True)
    c = x - m
    v = jnp.mean(c * c, axis=-1, keepdims=True)
    return c * jax.lax.rsqrt(v + EPS)


def _total(xs):
    return functools.reduce(jnp.add, xs)


def _norm(sq):
    return sq * jax.lax.rsqrt(sq + 1e-30)


def _iota(shape, dim):
    return jax.lax.broadcasted_iota(jnp.int32, shape, dim)


def _ds(start, n):
    return pl.ds(start if isinstance(start, int) else pl.multiple_of(start, 8), n)


def _after(x, deps, rows=(0,)):
    for r, ds in zip(rows, deps):
        for keep, d in ds:
            parts = [jnp.where(keep, x[r:r + 8, :128], pltpu.bitcast(d, x.dtype))]
            if x.shape[1] > 128:
                parts = [jnp.concatenate(parts + [x[r:r + 8, 128:]], axis=1)]
            parts = ([x[:r]] if r else []) + parts + ([x[r + 8:]] if r + 8 < x.shape[0] else [])
            x = jnp.concatenate(parts, axis=0)
    return x


def _overlap(j, mms, *sides, gates=2):
    keep = _iota((8, 128), 0) + j >= 0
    done = [[] for _ in range(len(mms) * gates + 1)]
    todo = [[] for _ in done]
    for steps, lo, hi, limit in sides:
        dt = (hi - lo) / len(steps)
        for m, f in enumerate(steps):
            todo[min(int(lo + (m + 1) * dt) + LEAD, limit)].append((f, lo + m * dt, dt))
    made = []

    def release(t, dt, x, frac=0.0):
        if not made or made[-1] is None:
            return x
        n = min(int((t + frac * dt) * len(made) / (g // gates * gates)), len(made) - 1)
        return _after(x, [[(keep, made[n])]])

    for g in range(len(done)):
        if todo[g]:
            done[g] = [(keep, _total([f(functools.partial(release, t, dt)) for f, t, dt in todo[g]]))]
        if g % gates == gates - 1 and g < len(mms) * gates:
            made += mms[g // gates](done[g + 1 - gates:g + 1])


def _mm_halves(a, b):
    k = a.shape[1] // 2
    ys = [_mm(a[:, :k], b[:k]), _mm(a[:, k:], b[k:])]
    return ys[0] + ys[1], [y[r:r + 8, :128] for y in ys for r in range(0, y.shape[0], 8)]


def _now(x, frac=0.0):
    return x


def _kernel(x_hbm, wq_hbm, wkt_hbm, wvt_hbm, woa_hbm, wqkv_hbm, wob_hbm, out_hbm,
            xio, wq, woa, wqkv, wob, wp, wobp, wkvt, tmp, tmpo,
            xe, xo, oe, oo, xn0, xn1, qa, ka, vt, kb, sp0, sp1, kmax, bad,
            b0, b1, pw, sem_x, sem_w, sem_o):
    xr, ob, xn = (xe, xo), (oe, oo), (xn0, xn1)
    bufs, side_p = (b0, b1), (sp0, sp1)
    TP = T // 2

    def x_copy(i):
        return pltpu.make_async_copy(x_hbm.bitcast(U32).at[_ds(i * TP, TP)], xio.at[_ds(i * TP, TP)], sem_x.at[i])

    def out_copy(i):
        return pltpu.make_async_copy(xio.at[_ds(i * TP, TP)], out_hbm.bitcast(U32).at[_ds(i * TP, TP)], sem_o.at[i])

    w_copies = [pltpu.make_async_copy(s.bitcast(U32), d, sem_w.at[n]) for n, (s, d) in enumerate(
        [(wkt_hbm, wkvt.at[:DH // 2]), (wvt_hbm, wkvt.at[DH // 2:]), (wq_hbm, wq),
         (wqkv_hbm, wqkv), (wob_hbm, wob), (woa_hbm, woa)])]
    x_copy(0).start()
    for c in w_copies[:3]:
        c.start()

    def st_ln(j, par, dst, from_input=False):
        def step(r, start):
            if from_input:
                x = _bf(xio[_ds((2 * j + par) * TP + r // 2, 8), :]).astype(F32)
                xr[par][_ds(j * T + r, 16), :] = x
            else:
                x = xr[par][_ds(j * T + r, 16), :]
            y = _ln(jnp.concatenate([start(x[:8]), start(x[8:], 0.5)], axis=0))
            dst[r // 2:r // 2 + 8, :] = _pack(y)
            return _total([y[a:a + 8, b:b + 128] for a in (0, 8) for b in range(0, D, 128)])
        return [functools.partial(step, r) for r in range(0, T, 16)]

    def st_qkv_a(i, src):
        def kv(deps):
            kvt = jax.lax.dot_general(_bf(_after(wkvt[...], deps[:1])), _bf(src[...]), (((1,), (1,)), ((), ())),
                                      preferred_element_type=F32)
            kt = (kvt[:DH] * QSCALE).astype(BF16).astype(F32)
            k2 = (kt * kt).reshape(DH // 8, 8, T).sum(0).sum(0, keepdims=True)
            km = kmax[:1]
            for t in range(T // 128):
                ts = slice(t * 128, (t + 1) * 128)
                vt[i * (T // 128) + t] = _pack(kvt[DH:, ts])
                km = jnp.maximum(km, k2[:, ts])
                kk = jnp.concatenate([kt[:, ts], jnp.zeros((128 - DH, 128), F32)], axis=0).T
                kk = jnp.where(_iota((128, 128), 1) == DH + 1, 1.0, kk)
                kk = jnp.concatenate([kk[g * 16:(g + 1) * 16] for g in reversed(range(8))], axis=0)
                ka[_ds((i * (T // 128) + t) * 64, 64), :] = _pack(kk)
                if t == 1:
                    for d in range(DH):
                        for a in range(2):
                            kb[2 * i + a, d] = jnp.broadcast_to(kk[112 + 8 * a:120 + 8 * a, d:d + 1], (8, 128))
            kmax[:1] = km
            return [kvt[:8, :128]] * (T // 4)

        def q(c, deps):
            r = _iota((8, 128), 0)
            y, tiles = _mm_halves(_bf(src[...]), _bf(_after(wq[:, c * 256:(c + 1) * 256], deps, (0, D // 4))))
            for t in range(T // 128):
                for g2 in range(2):
                    qt = y[t * 128:(t + 1) * 128, g2 * 128:(g2 + 1) * 128].T
                    qh = [qt[h * DH:(h + 1) * DH] for h in range(4)]
                    n2 = [(a * a).reshape(DH // 8, 8, 128).sum(0).sum(0, keepdims=True) for a in qh]
                    for h in range(4):
                        aug = (pltpu.bitcast(-_norm(n2[h]), U32) >> 16) | np.uint32(SHIFT_BITS)
                        dst = qa.at[i * (T // 128) + t, c * 2 + g2]
                        dst[:DH // 2, h * 128:(h + 1) * 128] = _pack(qh[h])
                        dst[DH // 2:, h * 128:(h + 1) * 128] = jnp.where(r == 0, aug, np.uint32(0))
            return tiles

        return [functools.partial(q, c) for c in range(D // 256)], kv

    def st_fix_k():
        km = _norm(jnp.max(kmax[:1], axis=1, keepdims=True)).astype(BF16).astype(F32)
        kmax[...] = jnp.broadcast_to(km, kmax.shape)
        km = pltpu.bitcast(kmax[:1], U32)
        ka[...] = jnp.where(_iota(ka.shape, 1) == DH, km | (km >> 16), ka[...])
        for n, t in enumerate(VTILES):
            k = _bf(ka[t * 64 + 56:(t + 1) * 64, :])
            sp0[n * 16:n * 16 + 16, :] = jnp.exp2(_mm(k[:, :KA], _bf(qa[0, 0])))

    def put_o(tb, g, ot):
        ot = jnp.concatenate([ot[:, h * 128:(h + 1) * 128] for h in range(4)], axis=0)
        oe[_ds(tb * 64, 64), _ds(g * 128, 128)] = _pack(ot.T)

    def st_attn(j):
        nt = S // 128
        steps = [(j * TU + i, g, t) for i in range(TU) for g in range(U) for t in range(nt)]
        s, acc, l = {}, {}, {}
        flag = [bad[...]]

        keep = _iota((8, 128), 0) + j >= 0
        part = {}

        def qk_vpu(tb, g, h, b, i, start):
            def row(i):
                w = jnp.broadcast_to(qa[tb, g, i:i + 1, h * 128:(h + 1) * 128], (8, 128))
                w = _after(w, [[(keep, start)]])
                return pltpu.bitcast(w << 16, F32), pltpu.bitcast(w & np.uint32(0xFFFF0000), F32)

            if i == 0:
                lo, hi = row(DH // 2)
                part[0] = [lo * kmax[...] + hi] * VB
            lo, hi = row(i)
            part[0] = [y + (kb[b * VB + a, 2 * i] * lo + kb[b * VB + a, 2 * i + 1] * hi)
                       for a, y in enumerate(part[0])]
            if i == DH // 2 - 1:
                side_p[g % 2][b * VB * 8:(b + 1) * VB * 8, h * 128:(h + 1) * 128] = (
                    jnp.exp2(jnp.concatenate(part.pop(0), axis=0)))

        items = [(h, b, i) for h in range(4) for b in range(2 * NV // VB) for i in range(DH // 2)]

        def qk(n, deps):
            tb, g, t = steps[n]
            rows = 56 if t in VTILES else 64
            s[n] = _mm(_bf(_after(ka[t * 64:t * 64 + rows, :], deps))[:, :KA], _bf(qa[tb, g]))
            if g == U - 1:
                tb = jnp.minimum(tb + 1, nt - 1)
            for m, item in enumerate(items):
                at = int(14 * (VLO + m * (VHI - VLO) / len(items)))
                if at // 14 == t:
                    qk_vpu(tb, (g + 1) % U, *item, s[n][8 * (at % 14):8 * (at % 14) + 8, :128])

        def pv(n):
            tb, g, t = steps[n]
            p = jnp.exp2(s.pop(n))
            if t in VTILES:
                r = VTILES.index(t) * 16
                p = jnp.concatenate([p, side_p[g % 2][r:r + 16, :]], axis=0)
            ps = p.reshape(16, 8, 512).sum(0)
            p = jnp.concatenate([p[j * 16:(j + 1) * 16] for j in reversed(range(8))], axis=0)
            o = _mm(_bf(vt[t]), p.astype(BF16))
            acc[0], l[0] = (o, ps) if t == 0 else (acc[0] + o, l[0] + ps)
            if t == nt - 1:
                ll = l.pop(0).sum(0, keepdims=True)
                ok = jnp.logical_and(ll >= L_LO, ll <= L_HI)
                flag[0] = jnp.maximum(flag[0], jnp.where(ok, 0.0, 1.0))
                put_o(tb, g, acc.pop(0) * (1.0 / ll))

        def step(n, deps):
            if n < len(steps):
                qk(n, deps)
            if n > 0:
                pv(n - 1)
            return [None]

        side = [f for i in range(TU) for f in st_permute(j * TU + i)]
        _overlap(j, [functools.partial(step, n) for n in range(len(steps) + 1)],
                 (side, 0, len(steps) - 8, len(steps)), gates=1)
        bad[...] = flag[0]

    def st_attn_exact(u):
        tb, g = u // U, u % U
        q = _bf(qa[tb, g, :DH // 2, :])

        def scores(t):
            kk = jnp.concatenate([ka[_ds(t * 64 + j * 8, 8), :] for j in reversed(range(8))], axis=0)
            return _mm(_bf(kk)[:, :DH], q)

        m = jax.lax.fori_loop(
            0, S // 128, lambda t, m: jnp.maximum(m, jnp.max(scores(t), axis=0, keepdims=True)),
            jnp.full((1, 512), -jnp.inf, F32))

        def body(t, c):
            p = jnp.exp2(scores(t) - m)
            return c[0] + _mm(_bf(vt[t]), p.astype(BF16)), c[1] + jnp.sum(p, axis=0, keepdims=True)

        acc, l = jax.lax.fori_loop(0, S // 128, body, (jnp.zeros((DH, 512), F32), jnp.zeros((1, 512), F32)))
        put_o(tb, g, acc * (1.0 / l))

    def st_out(j, par, w, o_ref):
        def step(c, deps):
            cs = slice(c * 256, (c + 1) * 256)
            rows = _ds((2 * j + par) * TP, TP)
            y, tiles = _mm_halves(_bf(o_ref[rows, :]), _bf(_after(w[:, cs], deps, (0, D // 4))))
            x = xr[par][_ds(j * T, T), cs] + y
            xr[par][_ds(j * T, T), cs] = x
            if w is wobp:
                xio[rows, cs] = _pack(x)
            return tiles
        return [functools.partial(step, c) for c in range(D // 256)]

    def st_qkv_b(j, par):
        qkv = bufs[par]

        def step(c, deps):
            y, tiles = _mm_halves(_bf(xn[par][...]), _bf(_after(wp[:, c * 256:(c + 1) * 256], deps, (0, D // 4))))
            qkv[2 * c, HALO:, :] = y[:, :128]
            qkv[2 * c + 1, HALO:, :] = y[:, 128:]
            if c == 7 or c == 11:
                cs = slice(2 * c - 6, 2 * c + 2)
                h = bufs[1 - par][cs, T:, :]
                if c == 11 and par == 0:
                    h = jnp.where(j == 0, jnp.broadcast_to(qkv[cs, HALO:HALO + 1, :], h.shape), h)
                qkv[cs, :HALO, :] = h
            return tiles
        return [functools.partial(step, c) for c in range(3 * D // 256)]

    def st_probs(j, par):
        buf = bufs[par]

        def softmax(lg, r):
            for w in range(W):
                y = lg[w] * QSCALE
                if par == 0 and r < DIL * w:
                    y = jnp.where(_iota((8, 128), 0) + (j * 2 * T + r) >= DIL * w, y, NEG)
                lg[w] = y
            m = lg[0]
            for w in range(1, W):
                m = jnp.maximum(m, lg[w])
            p = [jnp.exp2(y - m) for y in lg]
            inv = 1.0 / _total(p)
            p = [y * inv for y in p]
            for w in range(W):
                pw[w, r:r + 8, :] = p[w]
            return p

        def step(r, start):
            lg = [[None] * W, [None] * W]
            for c in range(8):
                k = {e: buf[8 + c, pl.ds(HALO + r + e, 8), :] for e in range(-DIL * (W - 1), 9, DIL)}
                for hf in range(2):
                    qc = start(buf[c, HALO + r + 8 * hf:HALO + r + 8 * hf + 8, :], c / 8)
                    for w in range(W):
                        pr = qc * k[8 * hf - DIL * w]
                        lg[hf][w] = pr if c == 0 else lg[hf][w] + pr
            for shift in (64, 32):
                lg = [[y + pltpu.roll(y, shift, 1) for y in ys] for ys in lg]
            return _total(softmax(lg[0], r) + softmax(lg[1], r + 8))

        return [functools.partial(step, r) for r in range(0, T, 16)]

    def st_mix(j, par):
        buf = bufs[par]

        def step(r, start):
            o = [[None] * 8, [None] * 8]
            for n, e in enumerate(range(-DIL * (W - 1), 9, DIL)):
                v = [buf[16 + c, pl.ds(HALO + r + e, 8), :] for c in range(8)]
                for hf in range(2):
                    w = (8 * hf - e) // DIL
                    if 0 <= w < W:
                        p = start(pw[w, r + 8 * hf:r + 8 * hf + 8, :], n / 12)
                        o[hf] = [p * a if b is None else b + p * a for a, b in zip(v, o[hf])]
            for c in range(8):
                ob[par][_ds((2 * j + par) * TP + r // 2, 8), c * 128:(c + 1) * 128] = (
                    _pack(jnp.concatenate([o[0][c], o[1][c]], axis=0)))
            return _total(o[0] + o[1])

        return [functools.partial(step, r) for r in range(0, T, 16)]

    def st_permute(u):
        n, rows = jnp.minimum(u // 4, 2), _ds(u % 4 * 128, 128)
        cs = _ds(u % 8 * 128, 128)

        def gather(t, start):
            y = wqkv[rows, _ds(n * D + t * 128, 128)].T
            for h in range(4 * t, 4 * t + 4):
                tmp[pl.ds(h * (DH + 1), DH), :] = y[h % 4 * DH:(h % 4 + 1) * DH]
                tmpo[h % 2, pl.ds(h // 2 * (DH // 2 + 1), DH // 2), :] = wob[h * DH // 2:(h + 1) * DH // 2, cs]
            return pltpu.bitcast(y[-8:], F32)

        def scatter(t, start):
            y = jnp.concatenate([tmp[pl.ds(4 * t + e, H, stride=DH + 1), :] for e in range(4)], axis=0).T
            wp[rows, _ds(n * D + t * 128, 128)] = y
            for e in (2 * t, 2 * t + 1):
                a, b = [tmpo[k, pl.ds(e, H // 2, stride=DH // 2 + 1), :] for k in range(2)]
                wobp[e * H:e * H + H // 2, cs] = (a & np.uint32(0xFFFF)) | (b << 16)
                wobp[e * H + H // 2:(e + 1) * H, cs] = (a >> 16) | (b & np.uint32(0xFFFF0000))
            return pltpu.bitcast(y[-8:], F32)

        return [functools.partial(f, t) for f in (gather, scatter) for t in range(8)]

    NP = NB // 2

    def qkv_a(j, from_input):
        for par, jn in ((0, j), (1, jnp.minimum(j + 1, NP - 1))):
            qs, kv = st_qkv_a(2 * j + par, xn[par])
            _overlap(j, [kv] + qs, (st_ln(jn, 1 - par, xn[1 - par], from_input), 2, 7, 10))

    kmax[...] = jnp.zeros(kmax.shape, F32)
    b1[...] = jnp.zeros(b1.shape, F32)
    pw[...] = jnp.zeros(pw.shape, F32)
    x_copy(0).wait()
    x_copy(1).start()
    for f in st_ln(0, 0, xn0, True):
        f(_now)
    for c in w_copies[:3]:
        c.wait()
    for i in range(2, NB):
        x_copy(i).start()

    @pl.loop(0, NP)
    def _(j):
        x_copy(2 * j + 1).wait()

        @pl.when(j + 1 < NP)
        def _():
            x_copy(2 * j + 2).wait()

        @pl.when(j == 1)
        def _():
            for c in w_copies[3:]:
                c.start()

        qkv_a(j, True)

    for c in w_copies[3:]:
        c.wait()

    @pl.loop(0, 2)
    def _(layer):
        st_fix_k()
        bad[...] = jnp.zeros(bad.shape, F32)

        @pl.loop(0, S // 128 // TU)
        def _(j):
            st_attn(j)

        @pl.when(jnp.max(bad[...]) > 0.0)
        def _():
            @pl.loop(0, (S // 128) * U)
            def _(u):
                st_attn_exact(u)

        @pl.loop(0, NP)
        def _(j):
            _overlap(j, st_out(j, 0, woa, oe) + st_out(j, 1, woa, oe), (st_ln(0, 0, xn0), 9, 13, 15))

        @pl.loop(0, NP)
        def _(j):
            jp, jn = jnp.maximum(j - 1, 0), jnp.minimum(j + 1, NP - 1)
            pr = st_probs(j, 0)
            _overlap(j, st_qkv_b(j, 0) + st_qkv_b(j, 1),
                     (st_probs(jp, 1)[8:], 0, 7, 9), (st_mix(jp, 1), 7, 17, 19), (st_ln(j, 1, xn1), 9, 19, 23),
                     (st_probs(j, 0), 17, 29, 31), (st_mix(j, 0), 29, 39, 41), (st_ln(jn, 0, xn0), 33, 43, 48),
                     (st_probs(j, 1)[:8], 39, 46, 48))

        def out_b(j, first=False):
            sides = [(st_probs(NP - 1, 1)[8:], 0, 5, 7),
                     (st_mix(NP - 1, 1), 5, 14, 16), (st_ln(0, 0, xn0), 9, 13, 15)] if first else []
            _overlap(layer, st_out(j, 0, wobp, oe) + st_out(j, 1, wobp, oo), *sides)

            @pl.when(layer == 1)
            def _():
                out_copy(2 * j).start()
                out_copy(2 * j + 1).start()

        out_b(0, True)
        pl.loop(1, NP)(out_b)

        @pl.when(layer == 0)
        def _():
            kmax[...] = jnp.zeros(kmax.shape, F32)

            @pl.loop(0, NP)
            def _(j):
                qkv_a(j, False)

    for i in range(NB):
        out_copy(i).wait()


@jax.jit
def pallas_interleave_layers__grouped_kv_mqa__sliding_local_dilated__prompt_kernel(
    A_x: jax.Array,
    A_wq: jax.Array,
    A_wk: jax.Array,
    A_wv: jax.Array,
    A_wo: jax.Array,
    B_x: jax.Array,
    B_wqkv: jax.Array,
    B_wo: jax.Array,
):
    del B_x
    vm = pltpu.VMEM
    out = pl.pallas_call(
        _kernel,
        out_shape=jax.ShapeDtypeStruct((S, D), BF16),
        in_specs=[pl.BlockSpec(memory_space=pl.ANY)] * 7,
        out_specs=pl.BlockSpec(memory_space=pl.ANY),
        scratch_shapes=[
            vm((S // 2, D), U32),
            vm((D // 2, D), U32), vm((D // 2, D), U32),
            vm((D // 2, 3 * D), U32), vm((D // 2, D), U32),
            vm((D // 2, 3 * D), U32), vm((D // 2, D), U32),
            vm((DH, D), U32),
            vm((D + H, 128), U32), vm((2, D // 4 + H // 2, 128), U32),
            vm((S // 2, D), F32), vm((S // 2, D), F32),
            vm((S // 2, D), U32), vm((S // 2, D), U32),
            vm((T // 2, D), U32), vm((T // 2, D), U32),
            vm((S // 128, U, KA // 2, 512), U32),
            vm((S // 2, 128), U32), vm((S // 128, DH // 2, 128), U32),
            vm((2 * NV, DH, 8, 128), F32),
            vm((16 * NV, 512), F32), vm((16 * NV, 512), F32),
            vm((8, 128), F32), vm((1, 512), F32),
            vm((24, T + HALO, 128), F32), vm((24, T + HALO, 128), F32), vm((W, T, 128), F32),
            pltpu.SemaphoreType.DMA((NB,)), pltpu.SemaphoreType.DMA((6,)), pltpu.SemaphoreType.DMA((NB,)),
        ],
        compiler_params=pltpu.CompilerParams(vmem_limit_bytes=110 * 1024 * 1024),
        name="four_layers",
    )(A_x.reshape(S, D), A_wq, A_wk.T, A_wv.T, A_wo, B_wqkv, B_wo)
    return out.reshape(1, S, D)
```

```python
import functools

import jax
import jax.numpy as jnp
import numpy as np
import jax.experimental.pallas as pl
import jax.experimental.pallas.tpu as pltpu

F32, BF16, U32 = jnp.float32, jnp.bfloat16, jnp.uint32

S, D, H, DH = 2048, 1024, 32, 32
W, DIL = 8, 2
EPS = 1e-5
LOG2E = 1.4426950408889634
QSCALE = DH ** -0.5 * LOG2E
NEG = -1e9 * LOG2E

T = 256
NB = S // T
KA = 48
HALO = 16
LEAD = 3
U = 8
TU = 1
NV = 8
VTILES = list(range(1, S // 128, 2))
VB = 4
VLO, VHI = 2, 16
SHIFT_BITS = 0x41A00000
L_LO, L_HI = 2.0 ** -40, 2.0 ** 33


def _mm(a, b):
    return jnp.dot(a, b, preferred_element_type=F32)


def _pack(x):
    return pltpu.bitcast(x.astype(BF16), U32)


def _bf(x):
    return pltpu.bitcast(x, BF16)


def _ln(x):
    m = jnp.mean(x, axis=-1, keepdims=True)
    c = x - m
    v = jnp.mean(c * c, axis=-1, keepdims=True)
    return c * jax.lax.rsqrt(v + EPS)


def _total(xs):
    return functools.reduce(jnp.add, xs)


def _norm(sq):
    return sq * jax.lax.rsqrt(sq + 1e-30)


def _iota(shape, dim):
    return jax.lax.broadcasted_iota(jnp.int32, shape, dim)


def _ds(start, n):
    return pl.ds(start if isinstance(start, int) else pl.multiple_of(start, 8), n)


def _after(x, deps, rows=(0,)):
    for r, ds in zip(rows, deps):
        for keep, d in ds:
            parts = [jnp.where(keep, x[r:r + 8, :128], pltpu.bitcast(d, x.dtype))]
            if x.shape[1] > 128:
                parts = [jnp.concatenate(parts + [x[r:r + 8, 128:]], axis=1)]
            parts = ([x[:r]] if r else []) + parts + ([x[r + 8:]] if r + 8 < x.shape[0] else [])
            x = jnp.concatenate(parts, axis=0)
    return x


def _overlap(j, mms, *sides, gates=2):
    keep = _iota((8, 128), 0) + j >= 0
    done = [[] for _ in range(len(mms) * gates + 1)]
    todo = [[] for _ in done]
    for steps, lo, hi, limit in sides:
        dt = (hi - lo) / len(steps)
        for m, f in enumerate(steps):
            todo[min(int(lo + (m + 1) * dt) + LEAD, limit)].append((f, lo + m * dt, dt))
    made = []

    def release(t, dt, x, frac=0.0):
        if not made:
            return x
        n = min(int((t + frac * dt) * len(made) / (g // gates * gates)), len(made) - 1)
        return _after(x, [[(keep, made[n])]])

    for g in range(len(done)):
        if todo[g]:
            done[g] = [(keep, _total([f(functools.partial(release, t, dt)) for f, t, dt in todo[g]]))]
        if g % gates == gates - 1 and g < len(mms) * gates:
            made += mms[g // gates](done[g + 1 - gates:g + 1])


def _mm_halves(a, b):
    k = a.shape[1] // 2
    ys = [_mm(a[:, :k], b[:k]), _mm(a[:, k:], b[k:])]
    return ys[0] + ys[1], [y[r:r + 8, :128] for y in ys for r in range(0, y.shape[0], 8)]


def _now(x, frac=0.0):
    return x


def _kernel(x_hbm, wq_hbm, wkt_hbm, wvt_hbm, woa_hbm, wqkv_hbm, wob_hbm, out_hbm,
            xio, wq, woa, wqkv, wob, wp, wobp, wkvt, tmp, tmpo,
            xe, xo, oe, oo, xn0, xn1, qa, ka, vt, kb, sp0, sp1, cs, ca, cl, kmax, bad,
            b0, b1, pw, sem_x, sem_w, sem_o):
    xr, ob, xn = (xe, xo), (oe, oo), (xn0, xn1)
    bufs, side_p = (b0, b1), (sp0, sp1)
    TP = T // 2

    def x_copy(i):
        return pltpu.make_async_copy(x_hbm.bitcast(U32).at[_ds(i * TP, TP)], xio.at[_ds(i * TP, TP)], sem_x.at[i])

    def out_copy(i):
        return pltpu.make_async_copy(xio.at[_ds(i * TP, TP)], out_hbm.bitcast(U32).at[_ds(i * TP, TP)], sem_o.at[i])

    w_copies = [pltpu.make_async_copy(s.bitcast(U32), d, sem_w.at[n]) for n, (s, d) in enumerate(
        [(wkt_hbm, wkvt.at[:DH // 2]), (wvt_hbm, wkvt.at[DH // 2:]), (wq_hbm, wq),
         (wqkv_hbm, wqkv), (wob_hbm, wob), (woa_hbm, woa)])]
    x_copy(0).start()
    for c in w_copies[:3]:
        c.start()

    def st_ln(j, par, dst, from_input=False):
        def step(r, start):
            if from_input:
                x = _bf(xio[_ds((2 * j + par) * TP + r // 2, 8), :]).astype(F32)
                xr[par][_ds(j * T + r, 16), :] = x
            else:
                x = xr[par][_ds(j * T + r, 16), :]
            y = _ln(jnp.concatenate([start(x[:8]), start(x[8:], 0.5)], axis=0))
            dst[r // 2:r // 2 + 8, :] = _pack(y)
            return _total([y[a:a + 8, b:b + 128] for a in (0, 8) for b in range(0, D, 128)])
        return [functools.partial(step, r) for r in range(0, T, 16)]

    def st_qkv_a(i, src):
        def kv(deps):
            kvt = jax.lax.dot_general(_bf(_after(wkvt[...], deps[:1])), _bf(src[...]), (((1,), (1,)), ((), ())),
                                      preferred_element_type=F32)
            kt = (kvt[:DH] * QSCALE).astype(BF16).astype(F32)
            k2 = (kt * kt).reshape(DH // 8, 8, T).sum(0).sum(0, keepdims=True)
            km = kmax[:1]
            for t in range(T // 128):
                ts = slice(t * 128, (t + 1) * 128)
                vt[i * (T // 128) + t] = _pack(kvt[DH:, ts])
                km = jnp.maximum(km, k2[:, ts])
                kk = jnp.concatenate([kt[:, ts], jnp.zeros((128 - DH, 128), F32)], axis=0).T
                kk = jnp.where(_iota((128, 128), 1) == DH + 1, 1.0, kk)
                kk = jnp.concatenate([kk[g * 16:(g + 1) * 16] for g in reversed(range(8))], axis=0)
                ka[_ds((i * (T // 128) + t) * 64, 64), :] = _pack(kk)
                if t == 1:
                    for d in range(DH):
                        for a in range(2):
                            kb[2 * i + a, d] = jnp.broadcast_to(kk[112 + 8 * a:120 + 8 * a, d:d + 1], (8, 128))
            kmax[:1] = km
            return [kvt[:8, :128]] * (T // 4)

        def q(c, deps):
            r = _iota((8, 128), 0)
            y, tiles = _mm_halves(_bf(src[...]), _bf(_after(wq[:, c * 256:(c + 1) * 256], deps, (0, D // 4))))
            for t in range(T // 128):
                for g2 in range(2):
                    qt = y[t * 128:(t + 1) * 128, g2 * 128:(g2 + 1) * 128].T
                    qh = [qt[h * DH:(h + 1) * DH] for h in range(4)]
                    n2 = [(a * a).reshape(DH // 8, 8, 128).sum(0).sum(0, keepdims=True) for a in qh]
                    for h in range(4):
                        aug = (pltpu.bitcast(-_norm(n2[h]), U32) >> 16) | np.uint32(SHIFT_BITS)
                        dst = qa.at[i * (T // 128) + t, c * 2 + g2]
                        dst[:DH // 2, h * 128:(h + 1) * 128] = _pack(qh[h])
                        dst[DH // 2:, h * 128:(h + 1) * 128] = jnp.where(r == 0, aug, np.uint32(0))
            return tiles

        return [functools.partial(q, c) for c in range(D // 256)], kv

    def st_fix_k():
        km = _norm(jnp.max(kmax[:1], axis=1, keepdims=True)).astype(BF16).astype(F32)
        kmax[...] = jnp.broadcast_to(km, kmax.shape)
        km = pltpu.bitcast(kmax[:1], U32)
        ka[...] = jnp.where(_iota(ka.shape, 1) == DH, km | (km >> 16), ka[...])
        bad[...] = jnp.zeros(bad.shape, F32)
        for ref in (cs, ca, cl, sp1):
            ref[...] = jnp.zeros(ref.shape, F32)
        for n, t in enumerate(VTILES):
            k = _bf(ka[t * 64 + 56:(t + 1) * 64, :])
            sp0[n * 16:n * 16 + 16, :] = jnp.exp2(_mm(k[:, :KA], _bf(qa[0, 0])))

    def put_o(tb, g, ot):
        ot = jnp.concatenate([ot[:, h * 128:(h + 1) * 128] for h in range(4)], axis=0)
        oe[_ds(tb * 64, 64), _ds(g * 128, 128)] = _pack(ot.T)

    def pv(tb, g, t, s, state):
        p = jnp.exp2(s)
        if t in VTILES:
            r = VTILES.index(t) * 16
            p = jnp.concatenate([p, side_p[g % 2][r:r + 16, :]], axis=0)
        l = p.reshape(16, 8, 512).sum(0)
        p = jnp.concatenate([p[k * 16:(k + 1) * 16] for k in reversed(range(8))], axis=0)
        o = _mm(_bf(vt[t]), p.astype(BF16))
        if t:
            o, l = state[0] + o, state[1] + l
        if t == S // 128 - 1:
            l = l.sum(0, keepdims=True)
            ok = jnp.logical_and(l >= L_LO, l <= L_HI)
            bad[...] = jnp.maximum(bad[...], jnp.where(ok, 0.0, 1.0))
            put_o(tb, g, o * (1.0 / l))
        return o, l

    def pv_carried(tb):
        pv(tb, U - 1, S // 128 - 1, cs[...], (ca[...], cl[...]))

    def st_attn(j):
        nt = S // 128
        steps = [(j * TU + i, g, t) for i in range(TU) for g in range(U) for t in range(nt)]
        s = {}
        side = [f for i in range(TU) for f in st_permute(j * TU + i)]
        side = [(f, 4 + k * (len(steps) - 8) // len(side)) for k, f in enumerate(side)]

        keep = _iota((8, 128), 0) + j >= 0
        part = {}

        def qk_vpu(tb, g, h, b, i, start):
            def row(i):
                w = jnp.broadcast_to(qa[tb, g, i:i + 1, h * 128:(h + 1) * 128], (8, 128))
                w = _after(w, [[(keep, start)]])
                return pltpu.bitcast(w << 16, F32), pltpu.bitcast(w & np.uint32(0xFFFF0000), F32)

            if i == 0:
                lo, hi = row(DH // 2)
                part[0] = [lo * kmax[...] + hi] * VB
            lo, hi = row(i)
            part[0] = [y + (kb[b * VB + a, 2 * i] * lo + kb[b * VB + a, 2 * i + 1] * hi)
                       for a, y in enumerate(part[0])]
            if i == DH // 2 - 1:
                side_p[g % 2][b * VB * 8:(b + 1) * VB * 8, h * 128:(h + 1) * 128] = (
                    jnp.exp2(jnp.concatenate(part.pop(0), axis=0)))

        items = [(h, b, i) for h in range(4) for b in range(2 * NV // VB) for i in range(DH // 2)]

        def qk(n):
            tb, g, t = steps[n]
            rows = 56 if t in VTILES else 64
            s[n] = _mm(_bf(ka[t * 64:t * 64 + rows, :])[:, :KA], _bf(qa[tb, g]))
            if g == U - 1:
                tb = jnp.minimum(tb + 1, nt - 1)
            for m, item in enumerate(items):
                at = int(14 * (VLO + m * (VHI - VLO) / len(items)))
                if at // 14 == t:
                    qk_vpu(tb, (g + 1) % U, *item, s[n][8 * (at % 14):8 * (at % 14) + 8, :128])

        state = None
        for n, step in enumerate(steps):
            qk(n)
            state = pv(prev[0], *steps[n - 1][1:], prev[1], state) if n else pv_carried(jnp.maximum(j * TU - 1, 0))
            prev = step[0], s.pop(n)
            for f, at in side:
                if at == n:
                    f(lambda x: _after(x, [[(keep, prev[1][:8, :128])]]))
        cs[...], ca[...], cl[...] = prev[1], *state

    def st_attn_exact(u):
        tb, g = u // U, u % U
        q = _bf(qa[tb, g, :DH // 2, :])

        def scores(t):
            kk = jnp.concatenate([ka[_ds(t * 64 + j * 8, 8), :] for j in reversed(range(8))], axis=0)
            return _mm(_bf(kk)[:, :DH], q)

        m = jax.lax.fori_loop(
            0, S // 128, lambda t, m: jnp.maximum(m, jnp.max(scores(t), axis=0, keepdims=True)),
            jnp.full((1, 512), -jnp.inf, F32))

        def body(t, c):
            p = jnp.exp2(scores(t) - m)
            return c[0] + _mm(_bf(vt[t]), p.astype(BF16)), c[1] + jnp.sum(p, axis=0, keepdims=True)

        acc, l = jax.lax.fori_loop(0, S // 128, body, (jnp.zeros((DH, 512), F32), jnp.zeros((1, 512), F32)))
        put_o(tb, g, acc * (1.0 / l))

    def st_out(j, par, w, o_ref):
        def step(c, deps):
            cs = slice(c * 256, (c + 1) * 256)
            rows = _ds((2 * j + par) * TP, TP)
            y, tiles = _mm_halves(_bf(o_ref[rows, :]), _bf(_after(w[:, cs], deps, (0, D // 4))))
            x = xr[par][_ds(j * T, T), cs] + y
            xr[par][_ds(j * T, T), cs] = x
            if w is wobp:
                xio[rows, cs] = _pack(x)
            return tiles
        return [functools.partial(step, c) for c in range(D // 256)]

    def st_qkv_b(j, par):
        qkv = bufs[par]

        def step(c, deps):
            y, tiles = _mm_halves(_bf(xn[par][...]), _bf(_after(wp[:, c * 256:(c + 1) * 256], deps, (0, D // 4))))
            qkv[2 * c, HALO:, :] = y[:, :128]
            qkv[2 * c + 1, HALO:, :] = y[:, 128:]
            if c == 7 or c == 11:
                cs = slice(2 * c - 6, 2 * c + 2)
                h = bufs[1 - par][cs, T:, :]
                if c == 11 and par == 0:
                    h = jnp.where(j == 0, jnp.broadcast_to(qkv[cs, HALO:HALO + 1, :], h.shape), h)
                qkv[cs, :HALO, :] = h
            return tiles
        return [functools.partial(step, c) for c in range(3 * D // 256)]

    def st_probs(j, par):
        buf = bufs[par]

        def softmax(lg, r):
            for w in range(W):
                y = lg[w] * QSCALE
                if par == 0 and r < DIL * w:
                    y = jnp.where(_iota((8, 128), 0) + (j * 2 * T + r) >= DIL * w, y, NEG)
                lg[w] = y
            m = lg[0]
            for w in range(1, W):
                m = jnp.maximum(m, lg[w])
            p = [jnp.exp2(y - m) for y in lg]
            inv = 1.0 / _total(p)
            p = [y * inv for y in p]
            for w in range(W):
                pw[w, r:r + 8, :] = p[w]
            return p

        def step(r, start):
            lg = [[None] * W, [None] * W]
            for c in range(8):
                k = {e: buf[8 + c, pl.ds(HALO + r + e, 8), :] for e in range(-DIL * (W - 1), 9, DIL)}
                for hf in range(2):
                    qc = start(buf[c, HALO + r + 8 * hf:HALO + r + 8 * hf + 8, :], c / 8)
                    for w in range(W):
                        pr = qc * k[8 * hf - DIL * w]
                        lg[hf][w] = pr if c == 0 else lg[hf][w] + pr
            for shift in (64, 32):
                lg = [[y + pltpu.roll(y, shift, 1) for y in ys] for ys in lg]
            return _total(softmax(lg[0], r) + softmax(lg[1], r + 8))

        return [functools.partial(step, r) for r in range(0, T, 16)]

    def st_mix(j, par):
        buf = bufs[par]

        def step(r, start):
            o = [[None] * 8, [None] * 8]
            for n, e in enumerate(range(-DIL * (W - 1), 9, DIL)):
                v = [buf[16 + c, pl.ds(HALO + r + e, 8), :] for c in range(8)]
                for hf in range(2):
                    w = (8 * hf - e) // DIL
                    if 0 <= w < W:
                        p = start(pw[w, r + 8 * hf:r + 8 * hf + 8, :], n / 12)
                        o[hf] = [p * a if b is None else b + p * a for a, b in zip(v, o[hf])]
            for c in range(8):
                ob[par][_ds((2 * j + par) * TP + r // 2, 8), c * 128:(c + 1) * 128] = (
                    _pack(jnp.concatenate([o[0][c], o[1][c]], axis=0)))
            return _total(o[0] + o[1])

        return [functools.partial(step, r) for r in range(0, T, 16)]

    def st_permute(u):
        n, rows = jnp.minimum(u // 4, 2), _ds(u % 4 * 128, 128)
        cs = _ds(u % 8 * 128, 128)

        def gather(t, start):
            y = wqkv[rows, _ds(n * D + t * 128, 128)].T
            for h in range(4 * t, 4 * t + 4):
                tmp[pl.ds(h * (DH + 1), DH), :] = y[h % 4 * DH:(h % 4 + 1) * DH]
                tmpo[h % 2, pl.ds(h // 2 * (DH // 2 + 1), DH // 2), :] = wob[h * DH // 2:(h + 1) * DH // 2, cs]
            return pltpu.bitcast(y[-8:], F32)

        def scatter(t, start):
            y = jnp.concatenate([tmp[pl.ds(4 * t + e, H, stride=DH + 1), :] for e in range(4)], axis=0).T
            wp[rows, _ds(n * D + t * 128, 128)] = y
            for e in (2 * t, 2 * t + 1):
                a, b = [tmpo[k, pl.ds(e, H // 2, stride=DH // 2 + 1), :] for k in range(2)]
                wobp[e * H:e * H + H // 2, cs] = (a & np.uint32(0xFFFF)) | (b << 16)
                wobp[e * H + H // 2:(e + 1) * H, cs] = (a >> 16) | (b & np.uint32(0xFFFF0000))
            return pltpu.bitcast(y[-8:], F32)

        return [functools.partial(f, t) for f in (gather, scatter) for t in range(8)]

    NP = NB // 2

    def qkv_a(j, from_input):
        for par, jn in ((0, j), (1, jnp.minimum(j + 1, NP - 1))):
            qs, kv = st_qkv_a(2 * j + par, xn[par])
            _overlap(j, [kv] + qs, (st_ln(jn, 1 - par, xn[1 - par], from_input), 2, 7, 10))

    kmax[...] = jnp.zeros(kmax.shape, F32)
    b1[...] = jnp.zeros(b1.shape, F32)
    pw[...] = jnp.zeros(pw.shape, F32)
    x_copy(0).wait()
    x_copy(1).start()
    for f in st_ln(0, 0, xn0, True):
        f(_now)
    for c in w_copies[:3]:
        c.wait()
    for i in range(2, NB):
        x_copy(i).start()

    @pl.loop(0, NP)
    def _(j):
        x_copy(2 * j + 1).wait()

        @pl.when(j + 1 < NP)
        def _():
            x_copy(2 * j + 2).wait()

        @pl.when(j == 1)
        def _():
            for c in w_copies[3:]:
                c.start()

        qkv_a(j, True)

    for c in w_copies[3:]:
        c.wait()

    @pl.loop(0, 2)
    def _(layer):
        st_fix_k()

        @pl.loop(0, S // 128 // TU)
        def _(j):
            st_attn(j)

        pv_carried(S // 128 - 1)

        @pl.when(jnp.max(bad[...]) > 0.0)
        def _():
            @pl.loop(0, (S // 128) * U)
            def _(u):
                st_attn_exact(u)

        @pl.loop(0, NP)
        def _(j):
            _overlap(j, st_out(j, 0, woa, oe) + st_out(j, 1, woa, oe), (st_ln(0, 0, xn0), 9, 13, 15))

        @pl.loop(0, NP)
        def _(j):
            jp, jn = jnp.maximum(j - 1, 0), jnp.minimum(j + 1, NP - 1)
            pr = st_probs(j, 0)
            _overlap(j, st_qkv_b(j, 0) + st_qkv_b(j, 1),
                     (st_probs(jp, 1)[8:], 0, 7, 9), (st_mix(jp, 1), 7, 17, 19), (st_ln(j, 1, xn1), 9, 19, 23),
                     (st_probs(j, 0), 17, 29, 31), (st_mix(j, 0), 29, 39, 41), (st_ln(jn, 0, xn0), 33, 43, 48),
                     (st_probs(j, 1)[:8], 39, 46, 48))

        def out_b(j, first=False):
            sides = [(st_probs(NP - 1, 1)[8:], 0, 5, 7),
                     (st_mix(NP - 1, 1), 5, 14, 16), (st_ln(0, 0, xn0), 9, 13, 15)] if first else []
            _overlap(layer, st_out(j, 0, wobp, oe) + st_out(j, 1, wobp, oo), *sides)

            @pl.when(layer == 1)
            def _():
                out_copy(2 * j).start()
                out_copy(2 * j + 1).start()

        out_b(0, True)
        pl.loop(1, NP)(out_b)

        @pl.when(layer == 0)
        def _():
            kmax[...] = jnp.zeros(kmax.shape, F32)

            @pl.loop(0, NP)
            def _(j):
                qkv_a(j, False)

    for i in range(NB):
        out_copy(i).wait()


@jax.jit
def pallas_interleave_layers__grouped_kv_mqa__sliding_local_dilated__prompt_kernel(
    A_x: jax.Array,
    A_wq: jax.Array,
    A_wk: jax.Array,
    A_wv: jax.Array,
    A_wo: jax.Array,
    B_x: jax.Array,
    B_wqkv: jax.Array,
    B_wo: jax.Array,
):
    del B_x
    vm = pltpu.VMEM
    out = pl.pallas_call(
        _kernel,
        out_shape=jax.ShapeDtypeStruct((S, D), BF16),
        in_specs=[pl.BlockSpec(memory_space=pl.ANY)] * 7,
        out_specs=pl.BlockSpec(memory_space=pl.ANY),
        scratch_shapes=[
            vm((S // 2, D), U32),
            vm((D // 2, D), U32), vm((D // 2, D), U32),
            vm((D // 2, 3 * D), U32), vm((D // 2, D), U32),
            vm((D // 2, 3 * D), U32), vm((D // 2, D), U32),
            vm((DH, D), U32),
            vm((D + H, 128), U32), vm((2, D // 4 + H // 2, 128), U32),
            vm((S // 2, D), F32), vm((S // 2, D), F32),
            vm((S // 2, D), U32), vm((S // 2, D), U32),
            vm((T // 2, D), U32), vm((T // 2, D), U32),
            vm((S // 128, U, KA // 2, 512), U32),
            vm((S // 2, 128), U32), vm((S // 128, DH // 2, 128), U32),
            vm((2 * NV, DH, 8, 128), F32),
            vm((16 * NV, 512), F32), vm((16 * NV, 512), F32),
            vm((112, 512), F32), vm((DH, 512), F32), vm((8, 512), F32),
            vm((8, 128), F32), vm((1, 512), F32),
            vm((24, T + HALO, 128), F32), vm((24, T + HALO, 128), F32), vm((W, T, 128), F32),
            pltpu.SemaphoreType.DMA((NB,)), pltpu.SemaphoreType.DMA((6,)), pltpu.SemaphoreType.DMA((NB,)),
        ],
        compiler_params=pltpu.CompilerParams(vmem_limit_bytes=110 * 1024 * 1024),
        name="four_layers",
    )(A_x.reshape(S, D), A_wq, A_wk.T, A_wv.T, A_wo, B_wqkv, B_wo)
    return out.reshape(1, S, D)
```

```python
import functools

import jax
import jax.numpy as jnp
import numpy as np
import jax.experimental.pallas as pl
import jax.experimental.pallas.tpu as pltpu

F32, BF16, U32 = jnp.float32, jnp.bfloat16, jnp.uint32

S, D, H, DH = 2048, 1024, 32, 32
W, DIL = 8, 2
EPS = 1e-5
LOG2E = 1.4426950408889634
QSCALE = DH ** -0.5 * LOG2E
NEG = -1e9 * LOG2E

T = 256
NB = S // T
KA = 48
HALO = 16
LEAD = 12
U = 8
TU = 1
NV = 8
VTILES = list(range(1, S // 128, 2))
VB = 4
VLO, VHI = 2, 16
SHIFT_BITS = 0x41A00000
L_LO, L_HI = 2.0 ** -40, 2.0 ** 33


def _mm(a, b):
    return jnp.dot(a, b, preferred_element_type=F32)


def _pack(x):
    return pltpu.bitcast(x.astype(BF16), U32)


def _bf(x):
    return pltpu.bitcast(x, BF16)


def _ln(x):
    m = jnp.mean(x, axis=-1, keepdims=True)
    c = x - m
    v = jnp.mean(c * c, axis=-1, keepdims=True)
    return c * jax.lax.rsqrt(v + EPS)


def _total(xs):
    return functools.reduce(jnp.add, xs)


def _norm(sq):
    return sq * jax.lax.rsqrt(sq + 1e-30)


def _iota(shape, dim):
    return jax.lax.broadcasted_iota(jnp.int32, shape, dim)


def _ds(start, n):
    return pl.ds(start if isinstance(start, int) else pl.multiple_of(start, 8), n)


def _cols(start, n=128):
    return pl.ds(start if isinstance(start, int) else pl.multiple_of(start, 128), n)


def _after(x, deps):
    for keep, d in deps:
        head = jnp.where(keep, x[:8, :128], pltpu.bitcast(d, x.dtype))
        if x.shape[1] > 128:
            head = jnp.concatenate([head, x[:8, 128:]], axis=1)
        x = jnp.concatenate([head, x[8:]], axis=0) if x.shape[0] > 8 else head
    return x


def _overlap(j, mms, *sides):
    keep = _iota((8, 128), 0) + j >= 0
    todo = [[] for _ in range(len(mms) + 1)]
    for steps, lo, hi, limit in sides:
        dt = (hi - lo) / len(steps)
        for m, f in enumerate(steps):
            todo[min(int(lo + (m + 1) * dt) + LEAD, limit)].append((f, lo + m * dt, dt))
    made = []

    def release(t, dt, x, frac=0.0):
        if not made:
            return x
        return _after(x, [(keep, made[min(int((t + frac * dt) * len(made) / n), len(made) - 1)])])

    for n, steps in enumerate(todo):
        done = [f(functools.partial(release, t, dt)) for f, t, dt in steps]
        if n < len(mms):
            made += mms[n]([(keep, _total(done))] if done else [])


def _left_factors(a11, a12, a21, a22):
    return a11 + a22, a21 + a22, a11, a22, a11 + a12, a21 - a11, a12 - a22


def _right_factors(b11, b12, b21, b22):
    return b11 + b22, b11, b12 - b22, b21 - b11, b22, b11 + b12, b21 + b22


def _strassen(a, b, c, emit):
    v = {}

    def step(m, deps):
        y = _mm(_bf(a.at[m][...]), _bf(_after(b.at[m][:, c * 128:(c + 1) * 128], deps)))
        if m == 5:
            v[1, 1] = y
        elif m == 0:
            v[1, 1] += y
            v[0, 0] = y
        elif m == 1:
            v[1, 1] -= y
            v[1, 0] = y
        elif m == 3:
            v[0, 0] += y
            emit(1, 0, v.pop((1, 0)) + y)
        elif m == 6:
            v[0, 0] += y
        elif m == 4:
            emit(0, 0, v.pop((0, 0)) - y)
            v[0, 1] = y
        else:
            emit(0, 1, v.pop((0, 1)) + y)
            emit(1, 1, v.pop((1, 1)) + y)
        return [y[r:r + 8] for r in range(0, y.shape[0], 8)]

    return [functools.partial(step, m) for m in (5, 0, 1, 3, 6, 4, 2)]


def _now(x, frac=0.0):
    return x


def _kernel(x_hbm, wq_hbm, wkt_hbm, wvt_hbm, woa_hbm, wqkv_hbm, wob_hbm, out_hbm,
            xio, wq, woa, wqkv, wob, wp, wobp, sq, soa, sp, sob, wkvt, tmp, tmpo,
            xe, xo, ob, xn0, xn1, on0, on1, qa, ka, vt, kb, sp0, sp1, cs, ca, cl, kmax, bad,
            b0, b1, pw, sem_x, sem_w, sem_o):
    xr, xn, on = (xe, xo), (xn0, xn1), (on0, on1)
    bufs, side_p = (b0, b1), (sp0, sp1)
    TP = T // 2

    def x_copy(i):
        return pltpu.make_async_copy(x_hbm.bitcast(U32).at[_ds(i * TP, TP)], xio.at[_ds(i * TP, TP)], sem_x.at[i])

    def out_copy(i):
        return pltpu.make_async_copy(xio.at[_ds(i * TP, TP)], out_hbm.bitcast(U32).at[_ds(i * TP, TP)], sem_o.at[i])

    w_copies = [pltpu.make_async_copy(s.bitcast(U32), d, sem_w.at[n]) for n, (s, d) in enumerate(
        [(wkt_hbm, wkvt.at[:DH // 2]), (wvt_hbm, wkvt.at[DH // 2:]), (wq_hbm, wq),
         (wqkv_hbm, wqkv), (wob_hbm, wob), (woa_hbm, woa)])]
    x_copy(0).start()
    for c in w_copies[:3]:
        c.start()

    def put_left(dst, r, top, bottom):
        quarters = top[:, :D // 2], top[:, D // 2:], bottom[:, :D // 2], bottom[:, D // 2:]
        fs = _left_factors(*quarters) + quarters[1:3]
        for m in range(dst.shape[0]):
            dst.at[m][r // 2:r // 2 + 8, :] = _pack(fs[m])
        return _total([f[a:a + 8, b:b + 128] for f in (fs[0], fs[5], fs[6])
                       for a in (0, 8) for b in range(0, D // 2, 128)])

    def put_right(dst, rows, cols, src, col0=0):
        b = [_bf(src[_ds(i * (D // 4) + rows[0], rows[1]), _cols(col0 + k * (D // 2) + cols[0], cols[1])]).astype(F32)
             for i in range(2) for k in range(2)]
        for m, f in enumerate(_right_factors(*b)):
            dst.at[m][_ds(*rows), _cols(col0 // 2 + cols[0], cols[1])] = _pack(f)

    def st_ln(j, par, from_input=False):
        def step(r, start):
            ys = []
            for hf in range(2):
                row = hf * (T // 2) + r
                if from_input:
                    x = _bf(xio[_ds((2 * j + par) * TP + row // 2, 8), :]).astype(F32)
                    xr[par][_ds(j * T + row, 16), :] = x
                else:
                    x = xr[par][_ds(j * T + row, 16), :]
                ys.append(_ln(jnp.concatenate([start(x[:8], hf / 2), start(x[8:], hf / 2 + 0.25)], axis=0)))
            return put_left(xn[par], r, *ys)
        return [functools.partial(step, r) for r in range(0, T // 2, 16)]

    def st_split(j, par):
        def step(r, start):
            ys = [ob[_ds((2 * j + par) * T + hf * (T // 2) + r, 16), :] for hf in range(2)]
            tile = lambda y, f: jnp.concatenate([
                jnp.concatenate([start(y[a:a + 8, :128], f), y[a:a + 8, 128:D // 2],
                                 start(y[a:a + 8, D // 2:D // 2 + 128], f), y[a:a + 8, D // 2 + 128:]], axis=1)
                for a in (0, 8)], axis=0)
            return put_left(on[par], r, tile(ys[0], 0.0), tile(ys[1], 0.5))
        return [functools.partial(step, r) for r in range(0, T // 2, 16)]

    def st_qkv_a(i, src):
        def kv(deps):
            w = _bf(_after(wkvt[...], deps))
            nt = lambda a, m: jax.lax.dot_general(a, _bf(src[m]), (((1,), (1,)), ((), ())),
                                                  preferred_element_type=F32)
            kvt = jnp.concatenate([nt(w[:, :D // 2], a) + nt(w[:, D // 2:], b) for a, b in ((2, 7), (8, 3))], axis=1)
            kt = (kvt[:DH] * QSCALE).astype(BF16).astype(F32)
            k2 = (kt * kt).reshape(DH // 8, 8, T).sum(0).sum(0, keepdims=True)
            km = kmax[:1]
            for t in range(T // 128):
                ts = slice(t * 128, (t + 1) * 128)
                vt[i * (T // 128) + t] = _pack(kvt[DH:, ts])
                km = jnp.maximum(km, k2[:, ts])
                kk = jnp.concatenate([kt[:, ts], jnp.zeros((128 - DH, 128), F32)], axis=0).T
                kk = jnp.where(_iota((128, 128), 1) == DH + 1, 1.0, kk)
                kk = jnp.concatenate([kk[g * 16:(g + 1) * 16] for g in reversed(range(8))], axis=0)
                ka[_ds((i * (T // 128) + t) * 64, 64), :] = _pack(kk)
                if t == 1:
                    for d in range(DH):
                        for a in range(2):
                            kb[2 * i + a, d] = jnp.broadcast_to(kk[112 + 8 * a:120 + 8 * a, d:d + 1], (8, 128))
            kmax[:1] = km
            return [kvt[:8, :128]] * 16

        def q(c, t, half, y):
            r = _iota((8, 128), 0)
            qt = y.T
            dst = qa.at[i * (T // 128) + t, half * 4 + c]
            for h in range(4):
                qh = qt[h * DH:(h + 1) * DH]
                n2 = (qh * qh).reshape(DH // 8, 8, 128).sum(0).sum(0, keepdims=True)
                aug = (pltpu.bitcast(-_norm(n2), U32) >> 16) | np.uint32(SHIFT_BITS)
                dst[:DH // 2, h * 128:(h + 1) * 128] = _pack(qh)
                dst[DH // 2:, h * 128:(h + 1) * 128] = jnp.where(r == 0, aug, np.uint32(0))

        return [kv] + [f for c in range(4) for f in _strassen(src, sq, c, functools.partial(q, c))]

    def st_fix_k():
        km = _norm(jnp.max(kmax[:1], axis=1, keepdims=True)).astype(BF16).astype(F32)
        kmax[...] = jnp.broadcast_to(km, kmax.shape)
        km = pltpu.bitcast(kmax[:1], U32)
        ka[...] = jnp.where(_iota(ka.shape, 1) == DH, km | (km >> 16), ka[...])
        bad[...] = jnp.zeros(bad.shape, F32)
        for ref in (cs, ca, cl, sp1):
            ref[...] = jnp.zeros(ref.shape, F32)
        for n, t in enumerate(VTILES):
            k = _bf(ka[t * 64 + 56:(t + 1) * 64, :])
            sp0[n * 16:n * 16 + 16, :] = jnp.exp2(_mm(k[:, :KA], _bf(qa[0, 0])))

    def put_o(tb, g, ot):
        ot = jnp.concatenate([ot[:, h * 128:(h + 1) * 128] for h in range(4)], axis=0)
        ob[_ds(tb * 128, 128), _cols(g * 128)] = ot.T

    def pv(tb, g, t, s, state):
        p = jnp.exp2(s)
        if t in VTILES:
            r = VTILES.index(t) * 16
            p = jnp.concatenate([p, side_p[g % 2][r:r + 16, :]], axis=0)
        l = p.reshape(16, 8, 512).sum(0)
        p = jnp.concatenate([p[k * 16:(k + 1) * 16] for k in reversed(range(8))], axis=0)
        o = _mm(_bf(vt[t]), p.astype(BF16))
        if t:
            o, l = state[0] + o, state[1] + l
        if t == S // 128 - 1:
            l = l.sum(0, keepdims=True)
            ok = jnp.logical_and(l >= L_LO, l <= L_HI)
            bad[...] = jnp.maximum(bad[...], jnp.where(ok, 0.0, 1.0))
            put_o(tb, g, o * (1.0 / l))
        return o, l

    def pv_carried(tb):
        pv(tb, U - 1, S // 128 - 1, cs[...], (ca[...], cl[...]))

    def st_attn(j):
        nt = S // 128
        steps = [(j * TU + i, g, t) for i in range(TU) for g in range(U) for t in range(nt)]
        s = {}
        side = [f for i in range(TU) for f in st_permute(j * TU + i)]
        side = [(f, 4 + k * (len(steps) - 8) // len(side)) for k, f in enumerate(side)]

        keep = _iota((8, 128), 0) + j >= 0
        part = {}

        def qk_vpu(tb, g, h, b, i, start):
            def row(i):
                w = jnp.broadcast_to(qa[tb, g, i:i + 1, h * 128:(h + 1) * 128], (8, 128))
                w = _after(w, [(keep, start)])
                return pltpu.bitcast(w << 16, F32), pltpu.bitcast(w & np.uint32(0xFFFF0000), F32)

            if i == 0:
                lo, hi = row(DH // 2)
                part[0] = [lo * kmax[...] + hi] * VB
            lo, hi = row(i)
            part[0] = [y + (kb[b * VB + a, 2 * i] * lo + kb[b * VB + a, 2 * i + 1] * hi)
                       for a, y in enumerate(part[0])]
            if i == DH // 2 - 1:
                side_p[g % 2][b * VB * 8:(b + 1) * VB * 8, h * 128:(h + 1) * 128] = (
                    jnp.exp2(jnp.concatenate(part.pop(0), axis=0)))

        items = [(h, b, i) for h in range(4) for b in range(2 * NV // VB) for i in range(DH // 2)]

        def qk(n):
            tb, g, t = steps[n]
            rows = 56 if t in VTILES else 64
            s[n] = _mm(_bf(ka[t * 64:t * 64 + rows, :])[:, :KA], _bf(qa[tb, g]))
            if g == U - 1:
                tb = jnp.minimum(tb + 1, nt - 1)
            for m, item in enumerate(items):
                at = int(14 * (VLO + m * (VHI - VLO) / len(items)))
                if at // 14 == t:
                    qk_vpu(tb, (g + 1) % U, *item, s[n][8 * (at % 14):8 * (at % 14) + 8, :128])

        state = None
        for n, step in enumerate(steps):
            qk(n)
            state = pv(prev[0], *steps[n - 1][1:], prev[1], state) if n else pv_carried(jnp.maximum(j * TU - 1, 0))
            prev = step[0], s.pop(n)
            for f, at in side:
                if at == n:
                    f(lambda x: _after(x, [(keep, prev[1][:8, :128])]))
        cs[...], ca[...], cl[...] = prev[1], *state

    def st_attn_exact(u):
        tb, g = u // U, u % U
        q = _bf(qa[tb, g, :DH // 2, :])

        def scores(t):
            kk = jnp.concatenate([ka[_ds(t * 64 + j * 8, 8), :] for j in reversed(range(8))], axis=0)
            return _mm(_bf(kk)[:, :DH], q)

        m = jax.lax.fori_loop(
            0, S // 128, lambda t, m: jnp.maximum(m, jnp.max(scores(t), axis=0, keepdims=True)),
            jnp.full((1, 512), -jnp.inf, F32))

        def body(t, c):
            p = jnp.exp2(scores(t) - m)
            return c[0] + _mm(_bf(vt[t]), p.astype(BF16)), c[1] + jnp.sum(p, axis=0, keepdims=True)

        acc, l = jax.lax.fori_loop(0, S // 128, body, (jnp.zeros((DH, 512), F32), jnp.zeros((1, 512), F32)))
        put_o(tb, g, acc * (1.0 / l))

    def st_out(j, par, w):
        def emit(c, t, half, y):
            cs = _cols((half * 4 + c) * 128)
            x = xr[par][_ds(j * T + t * 128, 128), cs] + y
            xr[par][_ds(j * T + t * 128, 128), cs] = x
            if w is sob:
                xio[_ds((2 * j + par) * TP + t * 64, 64), cs] = _pack(x)
        return [f for c in range(4) for f in _strassen(on[par], w, c, functools.partial(emit, c))]

    def st_qkv_b(j, par):
        qkv = bufs[par]

        def emit(c, t, half, y):
            qkv[c // 4 * 8 + half * 4 + c % 4, HALO + t * 128:HALO + (t + 1) * 128, :] = y
            if c % 4 == 3 and c > 3 and t == half == 1:
                cs = slice(2 * c - 6, 2 * c + 2)
                h = bufs[1 - par][cs, T:, :]
                if c == 11 and par == 0:
                    h = jnp.where(j == 0, jnp.broadcast_to(qkv[cs, HALO:HALO + 1, :], h.shape), h)
                qkv[cs, :HALO, :] = h
        return [f for c in range(12) for f in _strassen(xn[par], sp, c, functools.partial(emit, c))]

    def st_probs(j, par):
        buf = bufs[par]

        def softmax(lg, r):
            for w in range(W):
                y = lg[w] * QSCALE
                if par == 0 and r < DIL * w:
                    y = jnp.where(_iota((8, 128), 0) + (j * 2 * T + r) >= DIL * w, y, NEG)
                lg[w] = y
            m = lg[0]
            for w in range(1, W):
                m = jnp.maximum(m, lg[w])
            p = [jnp.exp2(y - m) for y in lg]
            inv = 1.0 / _total(p)
            p = [y * inv for y in p]
            for w in range(W):
                pw[w, r:r + 8, :] = p[w]
            return p

        def step(r, start):
            lg = [[None] * W, [None] * W]
            for c in range(8):
                k = {e: buf[8 + c, pl.ds(HALO + r + e, 8), :] for e in range(-DIL * (W - 1), 9, DIL)}
                for hf in range(2):
                    qc = start(buf[c, HALO + r + 8 * hf:HALO + r + 8 * hf + 8, :], c / 8)
                    for w in range(W):
                        pr = qc * k[8 * hf - DIL * w]
                        lg[hf][w] = pr if c == 0 else lg[hf][w] + pr
            for shift in (64, 32):
                lg = [[y + pltpu.roll(y, shift, 1) for y in ys] for ys in lg]
            return _total(softmax(lg[0], r) + softmax(lg[1], r + 8))

        return [functools.partial(step, r) for r in range(0, T, 16)]

    def st_mix(j, par):
        buf = bufs[par]

        def step(r, start):
            o = [[None] * 8, [None] * 8]
            for n, e in enumerate(range(-DIL * (W - 1), 9, DIL)):
                v = [buf[16 + c, pl.ds(HALO + r + e, 8), :] for c in range(8)]
                for hf in range(2):
                    w = (8 * hf - e) // DIL
                    if 0 <= w < W:
                        p = start(pw[w, r + 8 * hf:r + 8 * hf + 8, :], n / 12)
                        o[hf] = [p * a if b is None else b + p * a for a, b in zip(v, o[hf])]
            for c in range(8):
                ob[_ds((2 * j + par) * T + r, 16), c * 128:(c + 1) * 128] = (
                    jnp.concatenate([o[0][c], o[1][c]], axis=0))
            return _total(o[0] + o[1])

        return [functools.partial(step, r) for r in range(0, T, 16)]

    def st_permute(u):
        n, row = jnp.minimum(u // 4, 2), u % 4 * 64
        cs = _cols(u % 8 * 128)

        def gather(t, start):
            y = jnp.concatenate([wqkv[_ds(i * (D // 4) + row, 64), _cols(n * D + t * 128)]
                                 for i in range(2)], axis=0).T
            for h in range(4 * t, 4 * t + 4):
                tmp[pl.ds(h * (DH + 1), DH), :] = y[h % 4 * DH:(h % 4 + 1) * DH]
                tmpo[h % 2, pl.ds(h // 2 * (DH // 2 + 1), DH // 2), :] = wob[h * DH // 2:(h + 1) * DH // 2, cs]

        def scatter(t, start):
            y = jnp.concatenate([tmp[pl.ds(4 * t + e, H, stride=DH + 1), :] for e in range(4)], axis=0).T
            for i in range(2):
                wp[_ds(i * (D // 4) + row, 64), _cols(n * D + t * 128)] = y[i * 64:(i + 1) * 64]
            for e in (2 * t, 2 * t + 1):
                a, b = [tmpo[k, pl.ds(e, H // 2, stride=DH // 2 + 1), :] for k in range(2)]
                wobp[e * H:e * H + H // 2, cs] = (a & np.uint32(0xFFFF)) | (b << 16)
                wobp[e * H + H // 2:(e + 1) * H, cs] = (a >> 16) | (b & np.uint32(0xFFFF0000))

        def factors(t, start):
            cols = (t % 4 * 128, 128)
            put_right(sp, (row + t // 4 * 32, 32), cols, wp, n * D)
            if t < 4:
                put_right(sob, (u % 8 * 32, 32), cols, wobp)
            else:
                put_right(soa, (u * 16, 16), cols, woa)

        return [functools.partial(f, t) for f in (gather, scatter, factors) for t in range(8)]

    NP = NB // 2

    def qkv_a(j, from_input):
        for par, jn in ((0, j), (1, jnp.minimum(j + 1, NP - 1))):
            _overlap(j, st_qkv_a(2 * j + par, xn[par]), (st_ln(jn, 1 - par, from_input), 1, 23, 27))

    kmax[...] = jnp.zeros(kmax.shape, F32)
    b1[...] = jnp.zeros(b1.shape, F32)
    pw[...] = jnp.zeros(pw.shape, F32)
    wobp[...] = jnp.zeros(wobp.shape, U32)
    x_copy(0).wait()
    x_copy(1).start()
    x_copy(2).start()
    for f in st_ln(0, 0, True):
        f(_now)
    for c in w_copies[:3]:
        c.wait()
    for i in range(3, NB):
        x_copy(i).start()

    @pl.loop(0, 16)
    def _(u):
        put_right(sq, (u * 16, 16), (0, D // 2), wq)

    @pl.loop(0, NP)
    def _(j):
        x_copy(2 * j + 1).wait()

        @pl.when(j + 1 < NP)
        def _():
            x_copy(2 * j + 2).wait()

        @pl.when(j == 1)
        def _():
            for c in w_copies[3:]:
                c.start()

        qkv_a(j, True)

    for c in w_copies[3:]:
        c.wait()

    @pl.loop(0, 2)
    def _(layer):
        st_fix_k()

        @pl.loop(0, S // 128 // TU)
        def _(j):
            st_attn(j)

        pv_carried(S // 128 - 1)

        @pl.when(jnp.max(bad[...]) > 0.0)
        def _():
            @pl.loop(0, (S // 128) * U)
            def _(u):
                st_attn_exact(u)

        for f in st_split(0, 0):
            f(_now)

        @pl.loop(0, NP)
        def _(j):
            _overlap(j, st_out(j, 0, soa) + st_out(j, 1, soa), (st_split(j, 1), 1, 21, 28),
                     (st_ln(0, 0), 30, 50, 56), (st_split(jnp.minimum(j + 1, NP - 1), 0), 30, 50, 56))

        @pl.loop(0, NP)
        def _(j):
            jp, jn = jnp.maximum(j - 1, 0), jnp.minimum(j + 1, NP - 1)
            _overlap(j, st_qkv_b(j, 0) + st_qkv_b(j, 1),
                     (st_probs(jp, 1)[8:], 1, 25, 32), (st_mix(jp, 1), 25, 60, 67), (st_ln(j, 1), 32, 72, 84),
                     (st_probs(j, 0), 59, 101, 108), (st_mix(j, 0), 101, 136, 143), (st_ln(jn, 0), 112, 152, 168),
                     (st_split(0, 0), 144, 160, 168), (st_probs(j, 1)[:8], 143, 162, 168))

        def out_b(j, first=False):
            sides = [(st_split(j, 1), 1, 21, 28), (st_split(jnp.minimum(j + 1, NP - 1), 0), 30, 50, 56)]
            if first:
                sides = [(st_probs(NP - 1, 1)[8:], 1, 17, 24), (st_mix(NP - 1, 1), 17, 50, 56),
                         (st_ln(0, 0), 30, 50, 56)] + sides
            _overlap(layer, st_out(j, 0, sob) + st_out(j, 1, sob), *sides)

            @pl.when(layer == 1)
            def _():
                out_copy(2 * j).start()
                out_copy(2 * j + 1).start()

        out_b(0, True)
        pl.loop(1, NP)(out_b)

        @pl.when(layer == 0)
        def _():
            kmax[...] = jnp.zeros(kmax.shape, F32)

            @pl.loop(0, NP)
            def _(j):
                qkv_a(j, False)

    for i in range(NB):
        out_copy(i).wait()


@jax.jit
def pallas_interleave_layers__grouped_kv_mqa__sliding_local_dilated__prompt_kernel(
    A_x: jax.Array,
    A_wq: jax.Array,
    A_wk: jax.Array,
    A_wv: jax.Array,
    A_wo: jax.Array,
    B_x: jax.Array,
    B_wqkv: jax.Array,
    B_wo: jax.Array,
):
    del B_x
    vm = pltpu.VMEM
    out = pl.pallas_call(
        _kernel,
        out_shape=jax.ShapeDtypeStruct((S, D), BF16),
        in_specs=[pl.BlockSpec(memory_space=pl.ANY)] * 7,
        out_specs=pl.BlockSpec(memory_space=pl.ANY),
        scratch_shapes=[
            vm((S // 2, D), U32),
            vm((D // 2, D), U32), vm((D // 2, D), U32),
            vm((D // 2, 3 * D), U32), vm((D // 2, D), U32),
            vm((D // 2, 3 * D), U32), vm((D // 2, D), U32),
            vm((7, D // 4, D // 2), U32), vm((7, D // 4, D // 2), U32),
            vm((7, D // 4, 3 * D // 2), U32), vm((7, D // 4, D // 2), U32),
            vm((DH, D), U32),
            vm((D + H, 128), U32), vm((2, D // 4 + H // 2, 128), U32),
            vm((S // 2, D), F32), vm((S // 2, D), F32),
            vm((S, D), F32),
            vm((9, T // 4, D // 2), U32), vm((9, T // 4, D // 2), U32),
            vm((7, T // 4, D // 2), U32), vm((7, T // 4, D // 2), U32),
            vm((S // 128, U, KA // 2, 512), U32),
            vm((S // 2, 128), U32), vm((S // 128, DH // 2, 128), U32),
            vm((2 * NV, DH, 8, 128), F32),
            vm((16 * NV, 512), F32), vm((16 * NV, 512), F32),
            vm((112, 512), F32), vm((DH, 512), F32), vm((8, 512), F32),
            vm((8, 128), F32), vm((1, 512), F32),
            vm((24, T + HALO, 128), F32), vm((24, T + HALO, 128), F32), vm((W, T, 128), F32),
            pltpu.SemaphoreType.DMA((NB,)), pltpu.SemaphoreType.DMA((6,)), pltpu.SemaphoreType.DMA((NB,)),
        ],
        compiler_params=pltpu.CompilerParams(vmem_limit_bytes=110 * 1024 * 1024),
        name="four_layers",
    )(A_x.reshape(S, D), A_wq, A_wk.T, A_wv.T, A_wo, B_wqkv, B_wo)
    return out.reshape(1, S, D)
```

```python
import functools

import jax
import jax.numpy as jnp
import numpy as np
import jax.experimental.pallas as pl
import jax.experimental.pallas.tpu as pltpu

F32, BF16, U32 = jnp.float32, jnp.bfloat16, jnp.uint32

S, D, H, DH = 2048, 1024, 32, 32
W, DIL = 8, 2
EPS = 1e-5
LOG2E = 1.4426950408889634
QSCALE = DH ** -0.5 * LOG2E
NEG = -1e9 * LOG2E

T = 256
NB = S // T
KA = 48
HALO = 16
LEAD = 12
U = 8
TU = 1
NV = 8
VTILES = list(range(1, S // 128, 2))
VB = 4
VLO, VHI = 0, 16
SHIFT_BITS = 0x41A00000
L_LO, L_HI = 2.0 ** -40, 2.0 ** 33


def _mm(a, b):
    return jnp.dot(a, b, preferred_element_type=F32)


def _pack(x):
    return pltpu.bitcast(x.astype(BF16), U32)


def _bf(x):
    return pltpu.bitcast(x, BF16)


def _ln(x):
    m = jnp.mean(x, axis=-1, keepdims=True)
    c = x - m
    v = jnp.mean(c * c, axis=-1, keepdims=True)
    return c * jax.lax.rsqrt(v + EPS)


def _total(xs):
    return functools.reduce(jnp.add, xs)


def _norm(sq):
    return sq * jax.lax.rsqrt(sq + 1e-30)


def _iota(shape, dim):
    return jax.lax.broadcasted_iota(jnp.int32, shape, dim)


def _ds(start, n):
    return pl.ds(start if isinstance(start, int) else pl.multiple_of(start, 8), n)


def _cols(start, n=128):
    return pl.ds(start if isinstance(start, int) else pl.multiple_of(start, 128), n)


def _after(x, deps):
    for keep, d in deps:
        head = jnp.where(keep, x[:8, :128], pltpu.bitcast(d, x.dtype))
        if x.shape[1] > 128:
            head = jnp.concatenate([head, x[:8, 128:]], axis=1)
        x = jnp.concatenate([head, x[8:]], axis=0) if x.shape[0] > 8 else head
    return x


def _overlap(j, mms, *sides):
    keep = _iota((8, 128), 0) + j >= 0
    todo = [[] for _ in range(len(mms) + 1)]
    for steps, lo, hi, limit in sides:
        dt = (hi - lo) / len(steps)
        for m, f in enumerate(steps):
            todo[min(int(lo + (m + 1) * dt) + LEAD, limit)].append((f, lo + m * dt, dt))
    made = []

    def release(t, dt, x, frac=0.0):
        if not made:
            return x
        return _after(x, [(keep, made[min(int((t + frac * dt) * len(made) / n), len(made) - 1)])])

    for n, steps in enumerate(todo):
        done = [f(functools.partial(release, t, dt)) for f, t, dt in steps]
        if n < len(mms):
            made += mms[n]([(keep, _total(done))] if done else [])


def _left_factors(a11, a12, a21, a22):
    return a11 + a22, a21 + a22, a11, a22, a11 + a12, a21 - a11, a12 - a22


def _right_factors(b11, b12, b21, b22):
    return b11 + b22, b11, b12 - b22, b21 - b11, b22, b11 + b12, b21 + b22


def _strassen(a, b, c, emit):
    v = {}

    def step(m, deps):
        y = _mm(_bf(a.at[m][...]), _bf(_after(b.at[m][:, c * 128:(c + 1) * 128], deps)))
        if m == 5:
            v[1, 1] = y
        elif m == 0:
            v[1, 1] += y
            v[0, 0] = y
        elif m == 1:
            v[1, 1] -= y
            v[1, 0] = y
        elif m == 3:
            v[0, 0] += y
            emit(1, 0, v.pop((1, 0)) + y)
        elif m == 6:
            v[0, 0] += y
        elif m == 4:
            emit(0, 0, v.pop((0, 0)) - y)
            v[0, 1] = y
        else:
            emit(0, 1, v.pop((0, 1)) + y)
            emit(1, 1, v.pop((1, 1)) + y)
        return [y[r:r + 8] for r in range(0, y.shape[0], 8)]

    return [functools.partial(step, m) for m in (5, 0, 1, 3, 6, 4, 2)]


def _now(x, frac=0.0):
    return x


def _kernel(x_hbm, wq_hbm, wkt_hbm, wvt_hbm, woa_hbm, wqkv_hbm, wob_hbm, out_hbm,
            xio, wq, woa, wqkv, wob, wp, wobp, sq, soa, sp, sob, wkvt, tmp, tmpo,
            xe, xo, ob, xn0, xn1, on0, on1, qa, ka, vt, kb, sp0, sp1, cs, ca, cl, kmax, bad,
            b0, b1, pw, sem_x, sem_w, sem_o):
    xr, xn, on = (xe, xo), (xn0, xn1), (on0, on1)
    bufs, side_p = (b0, b1), (sp0, sp1)
    TP = T // 2

    def x_copy(i):
        return pltpu.make_async_copy(x_hbm.bitcast(U32).at[_ds(i * TP, TP)], xio.at[_ds(i * TP, TP)], sem_x.at[i])

    def out_copy(i):
        return pltpu.make_async_copy(xio.at[_ds(i * TP, TP)], out_hbm.bitcast(U32).at[_ds(i * TP, TP)], sem_o.at[i])

    w_copies = [pltpu.make_async_copy(s.bitcast(U32), d, sem_w.at[n]) for n, (s, d) in enumerate(
        [(wkt_hbm, wkvt.at[:DH // 2]), (wvt_hbm, wkvt.at[DH // 2:]), (wq_hbm, wq),
         (wqkv_hbm, wqkv), (wob_hbm, wob), (woa_hbm, woa)])]
    x_copy(0).start()
    for c in w_copies[:3]:
        c.start()

    def put_left(dst, r, top, bottom):
        quarters = top[:, :D // 2], top[:, D // 2:], bottom[:, :D // 2], bottom[:, D // 2:]
        fs = _left_factors(*quarters) + quarters[1:3]
        for m in range(dst.shape[0]):
            dst.at[m][r // 2:r // 2 + 8, :] = _pack(fs[m])
        return _total([f[a:a + 8, b:b + 128] for f in (fs[0], fs[5], fs[6])
                       for a in (0, 8) for b in range(0, D // 2, 128)])

    def put_right(dst, src, row, col, start, col0=0):
        b = [_bf(start(src[_ds(i * (D // 4) + row, 8), _cols(col0 + k * (D // 2) + col)])).astype(F32)
             for i in range(2) for k in range(2)]
        for m, f in enumerate(_right_factors(*b)):
            dst.at[m][_ds(row, 8), _cols(col0 // 2 + col)] = _pack(f)

    def st_ln(j, par, from_input=False):
        def step(r, start):
            ys = []
            for hf in range(2):
                row = hf * (T // 2) + r
                if from_input:
                    x = _bf(xio[_ds((2 * j + par) * TP + row // 2, 8), :]).astype(F32)
                    xr[par][_ds(j * T + row, 16), :] = x
                else:
                    x = xr[par][_ds(j * T + row, 16), :]
                ys.append(_ln(jnp.concatenate([start(x[:8], hf / 2), start(x[8:], hf / 2 + 0.25)], axis=0)))
            return put_left(xn[par], r, *ys)
        return [functools.partial(step, r) for r in range(0, T // 2, 16)]

    def st_split(j, par):
        def step(r, start):
            ys = [ob[_ds((2 * j + par) * T + hf * (T // 2) + r, 16), :] for hf in range(2)]
            tile = lambda y, f: jnp.concatenate([
                jnp.concatenate([start(y[a:a + 8, :128], f), y[a:a + 8, 128:D // 2],
                                 start(y[a:a + 8, D // 2:D // 2 + 128], f), y[a:a + 8, D // 2 + 128:]], axis=1)
                for a in (0, 8)], axis=0)
            return put_left(on[par], r, tile(ys[0], 0.0), tile(ys[1], 0.5))
        return [functools.partial(step, r) for r in range(0, T // 2, 16)]

    def st_qkv_a(i, src):
        def kv(deps):
            w = _bf(_after(wkvt[...], deps))
            nt = lambda a, m: jax.lax.dot_general(a, _bf(src[m]), (((1,), (1,)), ((), ())),
                                                  preferred_element_type=F32)
            kvt = jnp.concatenate([nt(w[:, :D // 2], a) + nt(w[:, D // 2:], b) for a, b in ((2, 7), (8, 3))], axis=1)
            kt = (kvt[:DH] * QSCALE).astype(BF16).astype(F32)
            k2 = (kt * kt).reshape(DH // 8, 8, T).sum(0).sum(0, keepdims=True)
            km = kmax[:1]
            for t in range(T // 128):
                ts = slice(t * 128, (t + 1) * 128)
                vt[i * (T // 128) + t] = _pack(kvt[DH:, ts])
                km = jnp.maximum(km, k2[:, ts])
                kk = jnp.concatenate([kt[:, ts], jnp.zeros((128 - DH, 128), F32)], axis=0).T
                kk = jnp.where(_iota((128, 128), 1) == DH + 1, 1.0, kk)
                kk = jnp.concatenate([kk[g * 16:(g + 1) * 16] for g in reversed(range(8))], axis=0)
                ka[_ds((i * (T // 128) + t) * 64, 64), :] = _pack(kk)
                if t == 1:
                    for d in range(DH):
                        for a in range(2):
                            kb[2 * i + a, d] = jnp.broadcast_to(kk[112 + 8 * a:120 + 8 * a, d:d + 1], (8, 128))
            kmax[:1] = km
            return [kvt[:8, :128]] * 16

        def q(c, t, half, y):
            r = _iota((8, 128), 0)
            qt = y.T
            dst = qa.at[i * (T // 128) + t, half * 4 + c]
            for h in range(4):
                qh = qt[h * DH:(h + 1) * DH]
                n2 = (qh * qh).reshape(DH // 8, 8, 128).sum(0).sum(0, keepdims=True)
                aug = (pltpu.bitcast(-_norm(n2), U32) >> 16) | np.uint32(SHIFT_BITS)
                dst[:DH // 2, h * 128:(h + 1) * 128] = _pack(qh)
                dst[DH // 2:, h * 128:(h + 1) * 128] = jnp.where(r == 0, aug, np.uint32(0))

        return [kv] + [f for c in range(4) for f in _strassen(src, sq, c, functools.partial(q, c))]

    def st_fix_k():
        km = _norm(jnp.max(kmax[:1], axis=1, keepdims=True)).astype(BF16).astype(F32)
        kmax[...] = jnp.broadcast_to(km, kmax.shape)
        km = pltpu.bitcast(kmax[:1], U32)
        ka[...] = jnp.where(_iota(ka.shape, 1) == DH, km | (km >> 16), ka[...])
        bad[...] = jnp.zeros(bad.shape, F32)
        for ref in (cs, ca, cl, sp1):
            ref[...] = jnp.zeros(ref.shape, F32)
        for n, t in enumerate(VTILES):
            k = _bf(ka[t * 64 + 56:(t + 1) * 64, :])
            sp0[n * 16:n * 16 + 16, :] = jnp.exp2(_mm(k[:, :KA], _bf(qa[0, 0])))

    def put_o(tb, g, ot):
        ot = jnp.concatenate([ot[:, h * 128:(h + 1) * 128] for h in range(4)], axis=0)
        ob[_ds(tb * 128, 128), _cols(g * 128)] = ot.T

    def pv(tb, g, t, s, state):
        p = jnp.exp2(s)
        if t in VTILES:
            r = VTILES.index(t) * 16
            p = jnp.concatenate([p, side_p[g % 2][r:r + 16, :]], axis=0)
        l = p.reshape(16, 8, 512).sum(0)
        p = jnp.concatenate([p[k * 16:(k + 1) * 16] for k in reversed(range(8))], axis=0)
        o = _mm(_bf(vt[t]), p.astype(BF16))
        if t:
            o, l = state[0] + o, state[1] + l
        if t == S // 128 - 1:
            l = l.sum(0, keepdims=True)
            ok = jnp.logical_and(l >= L_LO, l <= L_HI)
            bad[...] = jnp.maximum(bad[...], jnp.where(ok, 0.0, 1.0))
            put_o(tb, g, o * (1.0 / l))
        return o, l

    def pv_carried(tb):
        pv(tb, U - 1, S // 128 - 1, cs[...], (ca[...], cl[...]))

    def st_attn(j):
        nt = S // 128
        steps = [(j * TU + i, g, t) for i in range(TU) for g in range(U) for t in range(nt)]
        s = {}
        side = [f for i in range(TU) for f in st_permute(j * TU + i)]
        side = [(f, 2 + (3 * k if k < 16 else k + 36)) for k, f in enumerate(side)]

        keep = _iota((8, 128), 0) + j >= 0
        part = {}

        def qk_vpu(tb, g, h, b, i, start):
            def row(i):
                w = jnp.broadcast_to(qa[tb, g, i:i + 1, h * 128:(h + 1) * 128], (8, 128))
                w = _after(w, [(keep, start)])
                return pltpu.bitcast(w << 16, F32), pltpu.bitcast(w & np.uint32(0xFFFF0000), F32)

            if i == 0:
                lo, hi = row(DH // 2)
                part[0] = [lo * kmax[...] + hi] * VB
            lo, hi = row(i)
            part[0] = [y + (kb[b * VB + a, 2 * i] * lo + kb[b * VB + a, 2 * i + 1] * hi)
                       for a, y in enumerate(part[0])]
            if i == DH // 2 - 1:
                side_p[g % 2][b * VB * 8:(b + 1) * VB * 8, h * 128:(h + 1) * 128] = (
                    jnp.exp2(jnp.concatenate(part.pop(0), axis=0)))

        items = [(h, b, i) for h in range(4) for b in range(2 * NV // VB) for i in range(DH // 2)]

        def qk(n):
            tb, g, t = steps[n]
            rows = 56 if t in VTILES else 64
            s[n] = _mm(_bf(ka[t * 64:t * 64 + rows, :])[:, :KA], _bf(qa[tb, g]))
            if g == U - 1:
                tb = jnp.minimum(tb + 1, nt - 1)
            for m, item in enumerate(items):
                at = int(14 * (VLO + m * (VHI - VLO) / len(items)))
                if at // 14 == t:
                    qk_vpu(tb, (g + 1) % U, *item, s[n][8 * (at % 14):8 * (at % 14) + 8, :128])

        state = None
        for n, step in enumerate(steps):
            qk(n)
            state = pv(prev[0], *steps[n - 1][1:], prev[1], state) if n else pv_carried(jnp.maximum(j * TU - 1, 0))
            prev = step[0], s.pop(n)
            for f, at in side:
                if at == n:
                    f(lambda x: _after(x, [(keep, prev[1][:8, :128])]))
        cs[...], ca[...], cl[...] = prev[1], *state

    def st_attn_exact(u):
        tb, g = u // U, u % U
        q = _bf(qa[tb, g, :DH // 2, :])

        def scores(t):
            kk = jnp.concatenate([ka[_ds(t * 64 + j * 8, 8), :] for j in reversed(range(8))], axis=0)
            return _mm(_bf(kk)[:, :DH], q)

        m = jax.lax.fori_loop(
            0, S // 128, lambda t, m: jnp.maximum(m, jnp.max(scores(t), axis=0, keepdims=True)),
            jnp.full((1, 512), -jnp.inf, F32))

        def body(t, c):
            p = jnp.exp2(scores(t) - m)
            return c[0] + _mm(_bf(vt[t]), p.astype(BF16)), c[1] + jnp.sum(p, axis=0, keepdims=True)

        acc, l = jax.lax.fori_loop(0, S // 128, body, (jnp.zeros((DH, 512), F32), jnp.zeros((1, 512), F32)))
        put_o(tb, g, acc * (1.0 / l))

    def st_out(j, par, w):
        def emit(c, t, half, y):
            cs = _cols((half * 4 + c) * 128)
            x = xr[par][_ds(j * T + t * 128, 128), cs] + y
            xr[par][_ds(j * T + t * 128, 128), cs] = x
            if w is sob:
                xio[_ds((2 * j + par) * TP + t * 64, 64), cs] = _pack(x)
        return [f for c in range(4) for f in _strassen(on[par], w, c, functools.partial(emit, c))]

    def st_qkv_b(j, par):
        qkv = bufs[par]

        def emit(c, t, half, y):
            qkv[c // 4 * 8 + half * 4 + c % 4, HALO + t * 128:HALO + (t + 1) * 128, :] = y
            if c % 4 == 3 and c > 3 and t == half == 1:
                cs = slice(2 * c - 6, 2 * c + 2)
                h = bufs[1 - par][cs, T:, :]
                if c == 11 and par == 0:
                    h = jnp.where(j == 0, jnp.broadcast_to(qkv[cs, HALO:HALO + 1, :], h.shape), h)
                qkv[cs, :HALO, :] = h
        return [f for c in range(12) for f in _strassen(xn[par], sp, c, functools.partial(emit, c))]

    def st_probs(j, par):
        buf = bufs[par]

        def softmax(lg, r):
            for w in range(W):
                y = lg[w] * QSCALE
                if par == 0 and r < DIL * w:
                    y = jnp.where(_iota((8, 128), 0) + (j * 2 * T + r) >= DIL * w, y, NEG)
                lg[w] = y
            m = lg[0]
            for w in range(1, W):
                m = jnp.maximum(m, lg[w])
            p = [jnp.exp2(y - m) for y in lg]
            inv = 1.0 / _total(p)
            p = [y * inv for y in p]
            for w in range(W):
                pw[w, r:r + 8, :] = p[w]
            return p

        def step(r, start):
            lg = [[None] * W, [None] * W]
            for c in range(8):
                k = {e: buf[8 + c, pl.ds(HALO + r + e, 8), :] for e in range(-DIL * (W - 1), 9, DIL)}
                for hf in range(2):
                    qc = start(buf[c, HALO + r + 8 * hf:HALO + r + 8 * hf + 8, :], c / 8)
                    for w in range(W):
                        pr = qc * k[8 * hf - DIL * w]
                        lg[hf][w] = pr if c == 0 else lg[hf][w] + pr
            for shift in (64, 32):
                lg = [[y + pltpu.roll(y, shift, 1) for y in ys] for ys in lg]
            return _total(softmax(lg[0], r) + softmax(lg[1], r + 8))

        return [functools.partial(step, r) for r in range(0, T, 16)]

    def st_mix(j, par):
        buf = bufs[par]

        def step(r, start):
            o = [[None] * 8, [None] * 8]
            for n, e in enumerate(range(-DIL * (W - 1), 9, DIL)):
                v = [buf[16 + c, pl.ds(HALO + r + e, 8), :] for c in range(8)]
                for hf in range(2):
                    w = (8 * hf - e) // DIL
                    if 0 <= w < W:
                        p = start(pw[w, r + 8 * hf:r + 8 * hf + 8, :], n / 12)
                        o[hf] = [p * a if b is None else b + p * a for a, b in zip(v, o[hf])]
            for c in range(8):
                ob[_ds((2 * j + par) * T + r, 16), c * 128:(c + 1) * 128] = (
                    jnp.concatenate([o[0][c], o[1][c]], axis=0))
            return _total(o[0] + o[1])

        return [functools.partial(step, r) for r in range(0, T, 16)]

    def st_permute(u):
        n, row = jnp.minimum(u // 4, 2), u % 4 * 64
        cs = _cols(u % 8 * 128)

        def gather(t, start):
            y = start(jnp.concatenate([wqkv[_ds(i * (D // 4) + row, 64), _cols(n * D + t * 128)]
                                       for i in range(2)], axis=0)).T
            for h in range(4 * t, 4 * t + 4):
                tmp[pl.ds(h * (DH + 1), DH), :] = y[h % 4 * DH:(h % 4 + 1) * DH]
                tmpo[h % 2, pl.ds(h // 2 * (DH // 2 + 1), DH // 2), :] = wob[h * DH // 2:(h + 1) * DH // 2, cs]

        def scatter(t, start):
            y = start(jnp.concatenate([tmp[pl.ds(4 * t + e, H, stride=DH + 1), :] for e in range(4)], axis=0)).T
            for i in range(2):
                wp[_ds(i * (D // 4) + row, 64), _cols(n * D + t * 128)] = y[i * 64:(i + 1) * 64]
            for e in (2 * t, 2 * t + 1):
                a, b = [tmpo[k, pl.ds(e, H // 2, stride=DH // 2 + 1), :] for k in range(2)]
                a = start(a)
                wobp[e * H:e * H + H // 2, cs] = (a & np.uint32(0xFFFF)) | (b << 16)
                wobp[e * H + H // 2:(e + 1) * H, cs] = (a >> 16) | (b & np.uint32(0xFFFF0000))

        cols = range(0, D // 2, 128)
        return ([functools.partial(f, t) for f in (gather, scatter) for t in range(8)]
                + [functools.partial(put_right, soa, woa, u * 16 + r, c) for r in range(0, 16, 8) for c in cols]
                + [functools.partial(put_right, sob, wobp, u % 8 * 32 + r, c) for r in range(0, 32, 8) for c in cols]
                + [functools.partial(put_right, sp, wp, row + r, c, col0=n * D) for r in range(0, 64, 8) for c in cols])

    NP = NB // 2

    def qkv_a(j, from_input):
        for par, jn in ((0, j), (1, jnp.minimum(j + 1, NP - 1))):
            _overlap(j, st_qkv_a(2 * j + par, xn[par]), (st_ln(jn, 1 - par, from_input), 1, 23, 27))

    kmax[...] = jnp.zeros(kmax.shape, F32)
    b1[...] = jnp.zeros(b1.shape, F32)
    pw[...] = jnp.zeros(pw.shape, F32)
    wobp[...] = jnp.zeros(wobp.shape, U32)
    x_copy(0).wait()
    x_copy(1).start()
    x_copy(2).start()
    for f in st_ln(0, 0, True):
        f(_now)
    for c in w_copies[:3]:
        c.wait()
    for i in range(3, NB):
        x_copy(i).start()

    @pl.loop(0, 16)
    def _(u):
        for r in (0, 8):
            for c in range(0, D // 2, 128):
                put_right(sq, wq, u * 16 + r, c, _now)

    @pl.loop(0, NP)
    def _(j):
        x_copy(2 * j + 1).wait()

        @pl.when(j + 1 < NP)
        def _():
            x_copy(2 * j + 2).wait()

        @pl.when(j == 1)
        def _():
            for c in w_copies[3:]:
                c.start()

        qkv_a(j, True)

    for c in w_copies[3:]:
        c.wait()

    @pl.loop(0, 2)
    def _(layer):
        st_fix_k()

        @pl.loop(0, S // 128 // TU)
        def _(j):
            st_attn(j)

        pv_carried(S // 128 - 1)

        @pl.when(jnp.max(bad[...]) > 0.0)
        def _():
            @pl.loop(0, (S // 128) * U)
            def _(u):
                st_attn_exact(u)

        for f in st_split(0, 0):
            f(_now)

        @pl.loop(0, NP)
        def _(j):
            _overlap(j, st_out(j, 0, soa) + st_out(j, 1, soa), (st_split(j, 1), 1, 21, 28),
                     (st_ln(0, 0), 30, 50, 56), (st_split(jnp.minimum(j + 1, NP - 1), 0), 30, 50, 56))

        @pl.loop(0, NP)
        def _(j):
            jp, jn = jnp.maximum(j - 1, 0), jnp.minimum(j + 1, NP - 1)
            _overlap(j, st_qkv_b(j, 0) + st_qkv_b(j, 1),
                     (st_probs(jp, 1)[8:], 1, 25, 32), (st_mix(jp, 1), 25, 60, 67), (st_ln(j, 1), 32, 72, 84),
                     (st_probs(j, 0), 59, 101, 108), (st_mix(j, 0), 101, 136, 143), (st_ln(jn, 0), 112, 152, 168),
                     (st_split(0, 0), 144, 160, 168), (st_probs(j, 1)[:8], 143, 162, 168))

        def out_b(j, first=False):
            sides = [(st_split(j, 1), 1, 21, 28), (st_split(jnp.minimum(j + 1, NP - 1), 0), 30, 50, 56)]
            if first:
                sides = [(st_probs(NP - 1, 1)[8:], 1, 17, 24), (st_mix(NP - 1, 1), 17, 50, 56),
                         (st_ln(0, 0), 30, 50, 56)] + sides
            _overlap(layer, st_out(j, 0, sob) + st_out(j, 1, sob), *sides)

            @pl.when(layer == 1)
            def _():
                out_copy(2 * j).start()
                out_copy(2 * j + 1).start()

        out_b(0, True)
        pl.loop(1, NP)(out_b)

        @pl.when(layer == 0)
        def _():
            kmax[...] = jnp.zeros(kmax.shape, F32)

            @pl.loop(0, NP)
            def _(j):
                qkv_a(j, False)

    for i in range(NB):
        out_copy(i).wait()


@jax.jit
def pallas_interleave_layers__grouped_kv_mqa__sliding_local_dilated__prompt_kernel(
    A_x: jax.Array,
    A_wq: jax.Array,
    A_wk: jax.Array,
    A_wv: jax.Array,
    A_wo: jax.Array,
    B_x: jax.Array,
    B_wqkv: jax.Array,
    B_wo: jax.Array,
):
    del B_x
    vm = pltpu.VMEM
    out = pl.pallas_call(
        _kernel,
        out_shape=jax.ShapeDtypeStruct((S, D), BF16),
        in_specs=[pl.BlockSpec(memory_space=pl.ANY)] * 7,
        out_specs=pl.BlockSpec(memory_space=pl.ANY),
        scratch_shapes=[
            vm((S // 2, D), U32),
            vm((D // 2, D), U32), vm((D // 2, D), U32),
            vm((D // 2, 3 * D), U32), vm((D // 2, D), U32),
            vm((D // 2, 3 * D), U32), vm((D // 2, D), U32),
            vm((7, D // 4, D // 2), U32), vm((7, D // 4, D // 2), U32),
            vm((7, D // 4, 3 * D // 2), U32), vm((7, D // 4, D // 2), U32),
            vm((DH, D), U32),
            vm((D + H, 128), U32), vm((2, D // 4 + H // 2, 128), U32),
            vm((S // 2, D), F32), vm((S // 2, D), F32),
            vm((S, D), F32),
            vm((9, T // 4, D // 2), U32), vm((9, T // 4, D // 2), U32),
            vm((7, T // 4, D // 2), U32), vm((7, T // 4, D // 2), U32),
            vm((S // 128, U, KA // 2, 512), U32),
            vm((S // 2, 128), U32), vm((S // 128, DH // 2, 128), U32),
            vm((2 * NV, DH, 8, 128), F32),
            vm((16 * NV, 512), F32), vm((16 * NV, 512), F32),
            vm((112, 512), F32), vm((DH, 512), F32), vm((8, 512), F32),
            vm((8, 128), F32), vm((1, 512), F32),
            vm((24, T + HALO, 128), F32), vm((24, T + HALO, 128), F32), vm((W, T, 128), F32),
            pltpu.SemaphoreType.DMA((NB,)), pltpu.SemaphoreType.DMA((6,)), pltpu.SemaphoreType.DMA((NB,)),
        ],
        compiler_params=pltpu.CompilerParams(vmem_limit_bytes=110 * 1024 * 1024),
        name="four_layers",
    )(A_x.reshape(S, D), A_wq, A_wk.T, A_wv.T, A_wo, B_wqkv, B_wo)
    return out.reshape(1, S, D)
```

```python
import functools
import itertools

import jax
import jax.numpy as jnp
import numpy as np
import jax.experimental.pallas as pl
import jax.experimental.pallas.tpu as pltpu

F32, BF16, U32 = jnp.float32, jnp.bfloat16, jnp.uint32

S, D, H, DH = 2048, 1024, 32, 32
W, DIL = 8, 2
EPS = 1e-5
LOG2E = 1.4426950408889634
QSCALE = DH ** -0.5 * LOG2E
NEG = -1e9 * LOG2E

T = 256
NB = S // T
KA = 48
HALO = 16
LEVELS = 1
NF, MB, KB = 7 ** LEVELS, T >> LEVELS, D >> LEVELS
CW = 4 * 128 * 128 // KB
NS = NF * KB // CW
LEAD = 12 * NS // 28
U = 8
TU = 1
NV = 8
VTILES = list(range(1, S // 128, 2))
VB = 4
VLO, VHI = 0, 16
SHIFT_BITS = 0x41A00000
L_LO, L_HI = 2.0 ** -40, 2.0 ** 33


def _mm(a, b):
    return jnp.dot(a, b, preferred_element_type=F32)


def _pack(x):
    return pltpu.bitcast(x.astype(BF16), U32)


def _bf(x):
    return pltpu.bitcast(x, BF16)


def _ln(x):
    m = jnp.mean(x, axis=-1, keepdims=True)
    c = x - m
    v = jnp.mean(c * c, axis=-1, keepdims=True)
    return c * jax.lax.rsqrt(v + EPS)


def _total(xs):
    return functools.reduce(jnp.add, xs)


def _norm(sq):
    return sq * jax.lax.rsqrt(sq + 1e-30)


def _iota(shape, dim):
    return jax.lax.broadcasted_iota(jnp.int32, shape, dim)


def _ds(start, n):
    return pl.ds(start if isinstance(start, int) else pl.multiple_of(start, 8), n)


def _cols(start, n=128):
    return pl.ds(start if isinstance(start, int) else pl.multiple_of(start, 128), n)


def _after(x, deps):
    for keep, d in deps:
        head = jnp.where(keep, x[:8, :128], pltpu.bitcast(d, x.dtype))
        if x.shape[1] > 128:
            head = jnp.concatenate([head, x[:8, 128:]], axis=1)
        x = jnp.concatenate([head, x[8:]], axis=0) if x.shape[0] > 8 else head
    return x


def _overlap(j, mms, *sides):
    keep = _iota((8, 128), 0) + j >= 0
    todo = [[] for _ in range(len(mms) + 1)]
    for steps, *times in sides:
        lo, hi, limit = [-(-x * NS // 28) for x in times]
        dt = (hi - lo) / len(steps)
        for m, f in enumerate(steps):
            todo[min(int(lo + (m + 1) * dt) + LEAD, limit)].append((f, lo + m * dt, dt))
    made = []

    def release(t, dt, x, frac=0.0):
        if not made:
            return x
        return _after(x, [(keep, made[min(int((t + frac * dt) * len(made) / n), len(made) - 1)])])

    for n, steps in enumerate(todo):
        done = [f(functools.partial(release, t, dt)) for f, t, dt in steps]
        if n < len(mms):
            made += mms[n]([(keep, _total(done))] if done else [])


def _left_factors(a11, a12, a21, a22):
    return a11 + a22, a21 + a22, a11, a22, a11 + a12, a21 - a11, a12 - a22


def _right_factors(b11, b12, b21, b22):
    return b11 + b22, b11, b12 - b22, b21 - b11, b22, b11 + b12, b21 + b22


def _factors(rule, grid):
    n = len(grid) // 2
    if not n:
        return [grid[0][0]]
    fs = [[rule(grid[a][b], grid[a][n + b], grid[n + a][b], grid[n + a][n + b]) for b in range(n)] for a in range(n)]
    return [f for m in range(7) for f in _factors(rule, [[x[m] for x in row] for row in fs])]


ORDER = (0, 1, 3, 6, 4, 2, 5)


def _combiner(levels, emit):
    if not levels:
        return lambda ms, y: emit(0, 0, y)
    v = {}

    def rule(m, size, a, b, y):
        c = v.setdefault((a, b), {})
        out = lambda i, j, y: emit(i * size + a, j * size + b, y)
        if m == 0:
            c[0] = c[3] = y
        elif m == 1:
            c[3] -= y
            c[2] = y
        elif m == 3:
            c[0] += y
            out(1, 0, c.pop(2) + y)
        elif m == 6:
            c[0] += y
        elif m == 4:
            out(0, 0, c.pop(0) - y)
            c[1] = y
        elif m == 2:
            out(0, 1, c.pop(1) + y)
            c[3] += y
        else:
            out(1, 1, c.pop(3) + y)

    inner = [_combiner(levels - 1, functools.partial(rule, m, 2 ** (levels - 1))) for m in range(7)]
    return lambda ms, y: inner[ms[0]](ms[1:], y)


def _strassen(a, b, col0, emit):
    def step(c, put, ms, deps):
        m = functools.reduce(lambda x, y: 7 * x + y, ms)
        y = _mm(_bf(a.at[m][...]), _bf(_after(b.at[m][:, col0 + c:col0 + c + CW], deps)))
        put(ms, y)
        return [y[r:r + 8, k:k + 128] for r in range(0, MB, 8) for k in range(0, CW, 128)]

    steps = []
    for c in range(0, KB, CW):
        put = _combiner(LEVELS, lambda i, j, y, c=c: emit(i * MB, j * KB + c, y))
        steps += [functools.partial(step, c, put, ms) for ms in itertools.product(ORDER, repeat=LEVELS)]
    return steps


def _now(x, frac=0.0):
    return x


def _kernel(x_hbm, wq_hbm, wkt_hbm, wvt_hbm, woa_hbm, wqkv_hbm, wob_hbm, out_hbm,
            xio, wq, woa, wqkv, wob, wp, wobp, sq, soa, sp, sob, wkvt, tmp, tmpo,
            xe, xo, ob, xp, xn0, xn1, on0, on1, qa, ka, vt, kb, sp0, sp1, cs, ca, cl, kmax, bad,
            b0, b1, pw, sem_x, sem_w, sem_o):
    xr, xn, on = (xe, xo), (xn0, xn1), (on0, on1)
    bufs, side_p = (b0, b1), (sp0, sp1)
    TP = T // 2

    def x_copy(i):
        return pltpu.make_async_copy(x_hbm.bitcast(U32).at[_ds(i * TP, TP)], xio.at[_ds(i * TP, TP)], sem_x.at[i])

    def out_copy(i):
        return pltpu.make_async_copy(xio.at[_ds(i * TP, TP)], out_hbm.bitcast(U32).at[_ds(i * TP, TP)], sem_o.at[i])

    w_copies = [pltpu.make_async_copy(s.bitcast(U32), d, sem_w.at[n]) for n, (s, d) in enumerate(
        [(wkt_hbm, wkvt.at[:DH // 2]), (wvt_hbm, wkvt.at[DH // 2:]), (wq_hbm, wq),
         (wqkv_hbm, wqkv), (wob_hbm, wob), (woa_hbm, woa)])]
    x_copy(0).start()
    for c in w_copies[:3]:
        c.start()

    def put_left(dst, r, tile):
        last = []
        for c in range(0, KB, 128):
            fs = _factors(_left_factors, [[tile(i, k * KB + c) for k in range(D // KB)] for i in range(T // MB)])
            for m, f in enumerate(fs):
                dst.at[m][r // 2:r // 2 + 8, c:c + 128] = _pack(f)
            last += [f[a:a + 8] for f in fs[:1] + fs[-2:] for a in (0, 8)]
        return _total(last)

    def put_right(dst, src, row, col, start, col0=0):
        grid = [[_bf(start(src[_ds(i * (KB // 2) + row, 8), _cols(col0 + k * KB + col)])).astype(F32)
                 for k in range(D // KB)] for i in range(D // KB)]
        for m, f in enumerate(_factors(_right_factors, grid)):
            dst.at[m][_ds(row, 8), _cols(col0 // D * KB + col)] = _pack(f)

    def st_ln(j, par, from_input=False):
        def step(r, start):
            ys = []
            for i in range(T // MB):
                row = i * MB + r
                if from_input:
                    x = _bf(xio[_ds((2 * j + par) * TP + row // 2, 8), :]).astype(F32)
                    xr[par][_ds(j * T + row, 16), :] = x
                else:
                    x = xr[par][_ds(j * T + row, 16), :]
                ys.append(_ln(jnp.concatenate([start(x[a:a + 8], (i + a / 16) * MB / T) for a in (0, 8)], axis=0)))
                xp[par * TP + row // 2:par * TP + row // 2 + 8, :] = _pack(ys[-1])
            return put_left(xn[par], r, lambda i, c: ys[i][:, c:c + 128])
        return [functools.partial(step, r) for r in range(0, MB, 16)]

    def st_split(j, par):
        def step(r, start):
            def tile(i, c):
                y = ob[_ds((2 * j + par) * T + i * MB + r, 16), c:c + 128]
                return jnp.concatenate([start(y[a:a + 8], c % KB / KB) for a in (0, 8)], axis=0)
            return put_left(on[par], r, tile)
        return [functools.partial(step, r) for r in range(0, MB, 16)]

    def st_qkv_a(i, par):
        def kv(deps):
            kvt = jax.lax.dot_general(_bf(_after(wkvt[...], deps)), _bf(xp[par * TP:(par + 1) * TP, :]),
                                      (((1,), (1,)), ((), ())), preferred_element_type=F32)
            kt = (kvt[:DH] * QSCALE).astype(BF16).astype(F32)
            k2 = (kt * kt).reshape(DH // 8, 8, T).sum(0).sum(0, keepdims=True)
            km = kmax[:1]
            for t in range(T // 128):
                ts = slice(t * 128, (t + 1) * 128)
                vt[i * (T // 128) + t] = _pack(kvt[DH:, ts])
                km = jnp.maximum(km, k2[:, ts])
                kk = jnp.concatenate([kt[:, ts], jnp.zeros((128 - DH, 128), F32)], axis=0).T
                kk = jnp.where(_iota((128, 128), 1) == DH + 1, 1.0, kk)
                kk = jnp.concatenate([kk[g * 16:(g + 1) * 16] for g in reversed(range(8))], axis=0)
                ka[_ds((i * (T // 128) + t) * 64, 64), :] = _pack(kk)
                if t == 1:
                    for d in range(DH):
                        for a in range(2):
                            kb[2 * i + a, d] = jnp.broadcast_to(kk[112 + 8 * a:120 + 8 * a, d:d + 1], (8, 128))
            kmax[:1] = km
            return [kvt[:8, :128]] * 16

        held = {}

        def emit(row, col, y):
            held[row, col] = y
            t = row // 128
            if all((r, col) in held for r in range(t * 128, t * 128 + 128, MB)):
                y = jnp.concatenate([held.pop((r, col)) for r in range(t * 128, t * 128 + 128, MB)], axis=0)
                for c in range(0, CW, 128):
                    q(t, (col + c) // 128, y[:, c:c + 128])

        def q(t, g, y):
            r = _iota((8, 128), 0)
            qt = y.T
            dst = qa.at[i * (T // 128) + t, g]
            for h in range(4):
                qh = qt[h * DH:(h + 1) * DH]
                n2 = (qh * qh).reshape(DH // 8, 8, 128).sum(0).sum(0, keepdims=True)
                aug = (pltpu.bitcast(-_norm(n2), U32) >> 16) | np.uint32(SHIFT_BITS)
                dst[:DH // 2, h * 128:(h + 1) * 128] = _pack(qh)
                dst[DH // 2:, h * 128:(h + 1) * 128] = jnp.where(r == 0, aug, np.uint32(0))

        return [kv] + _strassen(xn[par], sq, 0, emit)

    def st_fix_k():
        km = _norm(jnp.max(kmax[:1], axis=1, keepdims=True)).astype(BF16).astype(F32)
        kmax[...] = jnp.broadcast_to(km, kmax.shape)
        km = pltpu.bitcast(kmax[:1], U32)
        ka[...] = jnp.where(_iota(ka.shape, 1) == DH, km | (km >> 16), ka[...])
        bad[...] = jnp.zeros(bad.shape, F32)
        for ref in (cs, ca, cl, sp1):
            ref[...] = jnp.zeros(ref.shape, F32)
        for n, t in enumerate(VTILES):
            k = _bf(ka[t * 64 + 56:(t + 1) * 64, :])
            sp0[n * 16:n * 16 + 16, :] = jnp.exp2(_mm(k[:, :KA], _bf(qa[0, 0])))

    def put_o(tb, g, ot):
        ot = jnp.concatenate([ot[:, h * 128:(h + 1) * 128] for h in range(4)], axis=0)
        ob[_ds(tb * 128, 128), _cols(g * 128)] = ot.T

    def pv(tb, g, t, s, state):
        p = jnp.exp2(s)
        if t in VTILES:
            r = VTILES.index(t) * 16
            p = jnp.concatenate([p, side_p[g % 2][r:r + 16, :]], axis=0)
        l = p.reshape(16, 8, 512).sum(0)
        p = jnp.concatenate([p[k * 16:(k + 1) * 16] for k in reversed(range(8))], axis=0)
        o = _mm(_bf(vt[t]), p.astype(BF16))
        if t:
            o, l = state[0] + o, state[1] + l
        if t == S // 128 - 1:
            l = l.sum(0, keepdims=True)
            ok = jnp.logical_and(l >= L_LO, l <= L_HI)
            bad[...] = jnp.maximum(bad[...], jnp.where(ok, 0.0, 1.0))
            put_o(tb, g, o * (1.0 / l))
        return o, l

    def pv_carried(tb):
        pv(tb, U - 1, S // 128 - 1, cs[...], (ca[...], cl[...]))

    def st_attn(j):
        nt = S // 128
        steps = [(j * TU + i, g, t) for i in range(TU) for g in range(U) for t in range(nt)]
        s = {}
        side = [f for i in range(TU) for f in st_permute(j * TU + i)]
        side = [(f, 2 + (3 * k if k < 16 else 52 + (k - 16) * 72 // (len(side) - 16))) for k, f in enumerate(side)]

        keep = _iota((8, 128), 0) + j >= 0
        part = {}

        def qk_vpu(tb, g, h, b, i, start):
            def row(i):
                w = jnp.broadcast_to(qa[tb, g, i:i + 1, h * 128:(h + 1) * 128], (8, 128))
                w = _after(w, [(keep, start)])
                return pltpu.bitcast(w << 16, F32), pltpu.bitcast(w & np.uint32(0xFFFF0000), F32)

            if i == 0:
                lo, hi = row(DH // 2)
                part[0] = [lo * kmax[...] + hi] * VB
            lo, hi = row(i)
            part[0] = [y + (kb[b * VB + a, 2 * i] * lo + kb[b * VB + a, 2 * i + 1] * hi)
                       for a, y in enumerate(part[0])]
            if i == DH // 2 - 1:
                side_p[g % 2][b * VB * 8:(b + 1) * VB * 8, h * 128:(h + 1) * 128] = (
                    jnp.exp2(jnp.concatenate(part.pop(0), axis=0)))

        items = [(h, b, i) for h in range(4) for b in range(2 * NV // VB) for i in range(DH // 2)]

        def qk(n):
            tb, g, t = steps[n]
            rows = 56 if t in VTILES else 64
            s[n] = _mm(_bf(ka[t * 64:t * 64 + rows, :])[:, :KA], _bf(qa[tb, g]))
            if g == U - 1:
                tb = jnp.minimum(tb + 1, nt - 1)
            for m, item in enumerate(items):
                at = int(14 * (VLO + m * (VHI - VLO) / len(items)))
                if at // 14 == t:
                    qk_vpu(tb, (g + 1) % U, *item, s[n][8 * (at % 14):8 * (at % 14) + 8, :128])

        state = None
        for n, step in enumerate(steps):
            qk(n)
            state = pv(*steps[n - 1], prev, state) if n else pv_carried(jnp.maximum(j * TU - 1, 0))
            prev = s.pop(n)
            for f, at in side:
                if at == n:
                    f(lambda x: _after(x, [(keep, prev[:8, :128])]))
        cs[...], ca[...], cl[...] = prev, *state

    def st_attn_exact(u):
        tb, g = u // U, u % U
        q = _bf(qa[tb, g, :DH // 2, :])

        def scores(t):
            kk = jnp.concatenate([ka[_ds(t * 64 + j * 8, 8), :] for j in reversed(range(8))], axis=0)
            return _mm(_bf(kk)[:, :DH], q)

        m = jax.lax.fori_loop(
            0, S // 128, lambda t, m: jnp.maximum(m, jnp.max(scores(t), axis=0, keepdims=True)),
            jnp.full((1, 512), -jnp.inf, F32))

        def body(t, c):
            p = jnp.exp2(scores(t) - m)
            return c[0] + _mm(_bf(vt[t]), p.astype(BF16)), c[1] + jnp.sum(p, axis=0, keepdims=True)

        acc, l = jax.lax.fori_loop(0, S // 128, body, (jnp.zeros((DH, 512), F32), jnp.zeros((1, 512), F32)))
        put_o(tb, g, acc * (1.0 / l))

    def st_out(j, par, w):
        def emit(row, col, y):
            x = xr[par][_ds(j * T + row, MB), col:col + CW] + y
            xr[par][_ds(j * T + row, MB), col:col + CW] = x
            if w is sob:
                xio[_ds((2 * j + par) * TP + row // 2, MB // 2), col:col + CW] = _pack(x)
        return _strassen(on[par], w, 0, emit)

    def st_qkv_b(j, par):
        qkv = bufs[par]

        def emit(n, row, col, y):
            for c in range(0, CW, 128):
                qkv[n * 8 + (col + c) // 128, HALO + row:HALO + row + MB, :] = y[:, c:c + 128]

        def last(f, n, deps):
            tiles = f(deps)
            cs = slice(n * 8, n * 8 + 8)
            h = bufs[1 - par][cs, T:, :]
            if n == 2 and par == 0:
                h = jnp.where(j == 0, jnp.broadcast_to(qkv[cs, HALO:HALO + 1, :], h.shape), h)
            qkv[cs, :HALO, :] = h
            return tiles

        steps = [f for n in range(3) for f in _strassen(xn[par], sp, n * KB, functools.partial(emit, n))]
        for n in (1, 2):
            steps[n * NS + NS - 1] = functools.partial(last, steps[n * NS + NS - 1], n)
        return steps

    def st_probs(j, par):
        buf = bufs[par]

        def softmax(lg, r):
            for w in range(W):
                y = lg[w] * QSCALE
                if par == 0 and r < DIL * w:
                    y = jnp.where(_iota((8, 128), 0) + (j * 2 * T + r) >= DIL * w, y, NEG)
                lg[w] = y
            m = lg[0]
            for w in range(1, W):
                m = jnp.maximum(m, lg[w])
            p = [jnp.exp2(y - m) for y in lg]
            inv = 1.0 / _total(p)
            p = [y * inv for y in p]
            for w in range(W):
                pw[w, r:r + 8, :] = p[w]
            return p

        def step(r, start):
            lg = [[None] * W, [None] * W]
            for c in range(8):
                k = {e: buf[8 + c, pl.ds(HALO + r + e, 8), :] for e in range(-DIL * (W - 1), 9, DIL)}
                for hf in range(2):
                    qc = start(buf[c, HALO + r + 8 * hf:HALO + r + 8 * hf + 8, :], c / 8)
                    for w in range(W):
                        pr = qc * k[8 * hf - DIL * w]
                        lg[hf][w] = pr if c == 0 else lg[hf][w] + pr
            for shift in (64, 32):
                lg = [[y + pltpu.roll(y, shift, 1) for y in ys] for ys in lg]
            return _total(softmax(lg[0], r) + softmax(lg[1], r + 8))

        return [functools.partial(step, r) for r in range(0, T, 16)]

    def st_mix(j, par):
        buf = bufs[par]

        def step(r, start):
            o = [[None] * 8, [None] * 8]
            for n, e in enumerate(range(-DIL * (W - 1), 9, DIL)):
                v = [buf[16 + c, pl.ds(HALO + r + e, 8), :] for c in range(8)]
                for hf in range(2):
                    w = (8 * hf - e) // DIL
                    if 0 <= w < W:
                        p = start(pw[w, r + 8 * hf:r + 8 * hf + 8, :], n / 12)
                        o[hf] = [p * a if b is None else b + p * a for a, b in zip(v, o[hf])]
            for c in range(8):
                ob[_ds((2 * j + par) * T + r, 16), c * 128:(c + 1) * 128] = (
                    jnp.concatenate([o[0][c], o[1][c]], axis=0))
            return _total(o[0] + o[1])

        return [functools.partial(step, r) for r in range(0, T, 16)]

    def st_permute(u):
        n, row = jnp.minimum(u // 4, 2), u % 4 * (KB // 8)
        cs = _cols(u % 8 * 128)

        def gather(t, start):
            y = start(jnp.concatenate([wqkv[_ds(i * (KB // 2) + row, KB // 8), _cols(n * D + t * 128)]
                                       for i in range(D // KB)], axis=0)).T
            for h in range(4 * t, 4 * t + 4):
                tmp[pl.ds(h * (DH + 1), DH), :] = y[h % 4 * DH:(h % 4 + 1) * DH]
                tmpo[h % 2, pl.ds(h // 2 * (DH // 2 + 1), DH // 2), :] = wob[h * DH // 2:(h + 1) * DH // 2, cs]

        def scatter(t, start):
            y = start(jnp.concatenate([tmp[pl.ds(4 * t + e, H, stride=DH + 1), :] for e in range(4)], axis=0)).T
            for i in range(D // KB):
                wp[_ds(i * (KB // 2) + row, KB // 8), _cols(n * D + t * 128)] = y[i * (KB // 8):(i + 1) * (KB // 8)]
            for e in (2 * t, 2 * t + 1):
                a, b = [tmpo[k, pl.ds(e, H // 2, stride=DH // 2 + 1), :] for k in range(2)]
                a = start(a)
                wobp[e * H:e * H + H // 2, cs] = (a & np.uint32(0xFFFF)) | (b << 16)
                wobp[e * H + H // 2:(e + 1) * H, cs] = (a >> 16) | (b & np.uint32(0xFFFF0000))

        def part(dst, src, row, parts, **kw):
            return [functools.partial(put_right, dst, src, row + r, c, **kw)
                    for r in range(0, KB // 2 // parts, 8) for c in range(0, KB, 128)]

        return ([functools.partial(f, t) for f in (gather, scatter) for t in range(8)]
                + part(soa, woa, u * (KB // 32), 16) + part(sob, wobp, u % 8 * (KB // 16), 8)
                + part(sp, wp, row, 4, col0=n * D))

    NP = NB // 2

    def qkv_a(j, from_input):
        for par, jn in ((0, j), (1, jnp.minimum(j + 1, NP - 1))):
            _overlap(j, st_qkv_a(2 * j + par, par), (st_ln(jn, 1 - par, from_input), 1, 23, 27))

    kmax[...] = jnp.zeros(kmax.shape, F32)
    b1[...] = jnp.zeros(b1.shape, F32)
    pw[...] = jnp.zeros(pw.shape, F32)
    wobp[...] = jnp.zeros(wobp.shape, U32)
    x_copy(0).wait()
    x_copy(1).start()
    x_copy(2).start()
    for f in st_ln(0, 0, True):
        f(_now)
    for c in w_copies[:3]:
        c.wait()
    for i in range(3, NB):
        x_copy(i).start()

    @pl.loop(0, 16)
    def _(u):
        for r in range(0, KB // 32, 8):
            for c in range(0, KB, 128):
                put_right(sq, wq, u * (KB // 32) + r, c, _now)

    @pl.loop(0, NP)
    def _(j):
        x_copy(2 * j + 1).wait()

        @pl.when(j + 1 < NP)
        def _():
            x_copy(2 * j + 2).wait()

        @pl.when(j == 1)
        def _():
            for c in w_copies[3:]:
                c.start()

        qkv_a(j, True)

    for c in w_copies[3:]:
        c.wait()

    @pl.loop(0, 2)
    def _(layer):
        st_fix_k()

        @pl.loop(0, S // 128 // TU)
        def _(j):
            st_attn(j)

        pv_carried(S // 128 - 1)

        @pl.when(jnp.max(bad[...]) > 0.0)
        def _():
            @pl.loop(0, (S // 128) * U)
            def _(u):
                st_attn_exact(u)

        for f in st_split(0, 0):
            f(_now)

        @pl.loop(0, NP)
        def _(j):
            _overlap(j, st_out(j, 0, soa) + st_out(j, 1, soa), (st_split(j, 1), 1, 21, 28),
                     (st_ln(0, 0), 30, 50, 56), (st_split(jnp.minimum(j + 1, NP - 1), 0), 30, 50, 56))

        @pl.loop(0, NP)
        def _(j):
            jp, jn = jnp.maximum(j - 1, 0), jnp.minimum(j + 1, NP - 1)
            _overlap(j, st_qkv_b(j, 0) + st_qkv_b(j, 1),
                     (st_probs(jp, 1)[8:], 1, 25, 32), (st_mix(jp, 1), 25, 60, 67), (st_ln(j, 1), 32, 72, 84),
                     (st_probs(j, 0), 59, 101, 108), (st_mix(j, 0), 101, 136, 143), (st_ln(jn, 0), 112, 152, 168),
                     (st_split(0, 0), 144, 160, 168), (st_probs(j, 1)[:8], 143, 162, 168))

        def out_b(j, first=False):
            sides = [(st_split(j, 1), 1, 21, 28), (st_split(jnp.minimum(j + 1, NP - 1), 0), 30, 50, 56)]
            if first:
                sides = [(st_probs(NP - 1, 1)[8:], 1, 17, 24), (st_mix(NP - 1, 1), 17, 50, 56),
                         (st_ln(0, 0), 30, 50, 56)] + sides
            _overlap(layer, st_out(j, 0, sob) + st_out(j, 1, sob), *sides)

            @pl.when(layer == 1)
            def _():
                out_copy(2 * j).start()
                out_copy(2 * j + 1).start()

        out_b(0, True)
        pl.loop(1, NP)(out_b)

        @pl.when(layer == 0)
        def _():
            kmax[...] = jnp.zeros(kmax.shape, F32)

            @pl.loop(0, NP)
            def _(j):
                qkv_a(j, False)

    for i in range(NB):
        out_copy(i).wait()


@jax.jit
def pallas_interleave_layers__grouped_kv_mqa__sliding_local_dilated__prompt_kernel(
    A_x: jax.Array,
    A_wq: jax.Array,
    A_wk: jax.Array,
    A_wv: jax.Array,
    A_wo: jax.Array,
    B_x: jax.Array,
    B_wqkv: jax.Array,
    B_wo: jax.Array,
):
    del B_x
    vm = pltpu.VMEM
    out = pl.pallas_call(
        _kernel,
        out_shape=jax.ShapeDtypeStruct((S, D), BF16),
        in_specs=[pl.BlockSpec(memory_space=pl.ANY)] * 7,
        out_specs=pl.BlockSpec(memory_space=pl.ANY),
        scratch_shapes=[
            vm((S // 2, D), U32),
            vm((D // 2, D), U32), vm((D // 2, D), U32),
            vm((D // 2, 3 * D), U32), vm((D // 2, D), U32),
            vm((D // 2, 3 * D), U32), vm((D // 2, D), U32),
            *[vm((NF, KB // 2, n * KB), U32) for n in (1, 1, 3, 1)],
            vm((DH, D), U32),
            vm((D + H, 128), U32), vm((2, D // 4 + H // 2, 128), U32),
            vm((S // 2, D), F32), vm((S // 2, D), F32),
            vm((S, D), F32),
            vm((T, D), U32),
            *[vm((NF, MB // 2, KB), U32)] * 4,
            vm((S // 128, U, KA // 2, 512), U32),
            vm((S // 2, 128), U32), vm((S // 128, DH // 2, 128), U32),
            vm((2 * NV, DH, 8, 128), F32),
            vm((16 * NV, 512), F32), vm((16 * NV, 512), F32),
            vm((112, 512), F32), vm((DH, 512), F32), vm((8, 512), F32),
            vm((8, 128), F32), vm((1, 512), F32),
            vm((24, T + HALO, 128), F32), vm((24, T + HALO, 128), F32), vm((W, T, 128), F32),
            pltpu.SemaphoreType.DMA((NB,)), pltpu.SemaphoreType.DMA((6,)), pltpu.SemaphoreType.DMA((NB,)),
        ],
        compiler_params=pltpu.CompilerParams(vmem_limit_bytes=120 * 1024 * 1024),
        name="four_layers",
    )(A_x.reshape(S, D), A_wq, A_wk.T, A_wv.T, A_wo, B_wqkv, B_wo)
    return out.reshape(1, S, D)
```

```python
import functools
import itertools

import jax
import jax.numpy as jnp
import numpy as np
import jax.experimental.pallas as pl
import jax.experimental.pallas.tpu as pltpu

F32, BF16, U32 = jnp.float32, jnp.bfloat16, jnp.uint32

S, D, H, DH = 2048, 1024, 32, 32
W, DIL = 8, 2
EPS = 1e-5
LOG2E = 1.4426950408889634
QSCALE = DH ** -0.5 * LOG2E
NEG = -1e9 * LOG2E

T = 256
NB = S // T
KA = 48
HALO = 16
LEVELS = 1
NF, MB, KB = 7 ** LEVELS, T >> LEVELS, D >> LEVELS
CW = 4 * 128 * 128 // KB
NS = NF * KB // CW
LEAD = 12 * NS // 28
U = 8
TU = 1
NV = 8
VTILES = list(range(1, S // 128, 2))
VB = 4
VLO, VHI = 0, 16
SHIFT_BITS = 0x42480000
L_LO, L_HI = 2.0 ** -50, 2.0 ** 63


def _mm(a, b):
    return jnp.dot(a, b, preferred_element_type=F32)


def _pack(x):
    return pltpu.bitcast(x.astype(BF16), U32)


def _bf(x):
    return pltpu.bitcast(x, BF16)


def _ln(x):
    m = jnp.mean(x, axis=-1, keepdims=True)
    c = x - m
    v = jnp.mean(c * c, axis=-1, keepdims=True)
    return c * jax.lax.rsqrt(v + EPS)


def _total(xs):
    return functools.reduce(jnp.add, xs)


def _norm(sq):
    return sq * jax.lax.rsqrt(sq + 1e-30)


def _iota(shape, dim):
    return jax.lax.broadcasted_iota(jnp.int32, shape, dim)


def _ds(start, n):
    return pl.ds(start if isinstance(start, int) else pl.multiple_of(start, 8), n)


def _cols(start, n=128):
    return pl.ds(start if isinstance(start, int) else pl.multiple_of(start, 128), n)


def _after(x, deps):
    for keep, d in deps:
        head = jnp.where(keep, x[:8, :128], pltpu.bitcast(d, x.dtype))
        if x.shape[1] > 128:
            head = jnp.concatenate([head, x[:8, 128:]], axis=1)
        x = jnp.concatenate([head, x[8:]], axis=0) if x.shape[0] > 8 else head
    return x


def _overlap(j, mms, *sides):
    keep = _iota((8, 128), 0) + j >= 0
    todo = [[] for _ in range(len(mms) + 1)]
    for steps, *times in sides:
        lo, hi, limit = [-(-x * NS // 28) for x in times]
        dt = (hi - lo) / len(steps)
        for m, f in enumerate(steps):
            todo[min(int(lo + (m + 1) * dt) + LEAD, limit)].append((f, lo + m * dt, dt))
    made = []

    def release(t, dt, x, frac=0.0):
        if not made:
            return x
        return _after(x, [(keep, made[min(int((t + frac * dt) * len(made) / n), len(made) - 1)])])

    for n, steps in enumerate(todo):
        done = [f(functools.partial(release, t, dt)) for f, t, dt in steps]
        if n < len(mms):
            made += mms[n]([(keep, _total(done))] if done else [])


def _left_factors(a11, a12, a21, a22):
    return a11 + a22, a21 + a22, a11, a22, a11 + a12, a21 - a11, a12 - a22


def _right_factors(b11, b12, b21, b22):
    return b11 + b22, b11, b12 - b22, b21 - b11, b22, b11 + b12, b21 + b22


def _factors(rule, grid):
    n = len(grid) // 2
    if not n:
        return [grid[0][0]]
    fs = [[rule(grid[a][b], grid[a][n + b], grid[n + a][b], grid[n + a][n + b]) for b in range(n)] for a in range(n)]
    return [f for m in range(7) for f in _factors(rule, [[x[m] for x in row] for row in fs])]


ORDER = (0, 1, 3, 6, 4, 2, 5)


def _combiner(levels, emit):
    if not levels:
        return lambda ms, y: emit(0, 0, y)
    v = {}

    def rule(m, size, a, b, y):
        c = v.setdefault((a, b), {})
        out = lambda i, j, y: emit(i * size + a, j * size + b, y)
        if m == 0:
            c[0] = c[3] = y
        elif m == 1:
            c[3] -= y
            c[2] = y
        elif m == 3:
            c[0] += y
            out(1, 0, c.pop(2) + y)
        elif m == 6:
            c[0] += y
        elif m == 4:
            out(0, 0, c.pop(0) - y)
            c[1] = y
        elif m == 2:
            out(0, 1, c.pop(1) + y)
            c[3] += y
        else:
            out(1, 1, c.pop(3) + y)

    inner = [_combiner(levels - 1, functools.partial(rule, m, 2 ** (levels - 1))) for m in range(7)]
    return lambda ms, y: inner[ms[0]](ms[1:], y)


def _strassen(a, b, col0, emit):
    def step(c, put, ms, deps):
        m = functools.reduce(lambda x, y: 7 * x + y, ms)
        y = _mm(_bf(a.at[m][...]), _bf(_after(b.at[m][:, col0 + c:col0 + c + CW], deps)))
        put(ms, y)
        return [y[r:r + 8, k:k + 128] for r in range(0, MB, 8) for k in range(0, CW, 128)]

    steps = []
    for c in range(0, KB, CW):
        put = _combiner(LEVELS, lambda i, j, y, c=c: emit(i * MB, j * KB + c, y))
        steps += [functools.partial(step, c, put, ms) for ms in itertools.product(ORDER, repeat=LEVELS)]
    return steps


def _now(x, frac=0.0):
    return x


def _kernel(x_hbm, wq_hbm, wkt_hbm, wvt_hbm, woa_hbm, wqkv_hbm, wob_hbm, out_hbm,
            xio, wq, woa, wqkv, wob, wp, wobp, sq, soa, sp, sob, wkvt, tmp, tmpo,
            xe, xo, ob, xp, xn0, xn1, on0, on1, qa, ka, vt, kb, sp0, sp1, cs, ca, cl, kmax, bad,
            b0, b1, pw, sem_x, sem_w, sem_o):
    xr, xn, on = (xe, xo), (xn0, xn1), (on0, on1)
    bufs, side_p = (b0, b1), (sp0, sp1)
    TP = T // 2

    def x_copy(i):
        return pltpu.make_async_copy(x_hbm.bitcast(U32).at[_ds(i * TP, TP)], xio.at[_ds(i * TP, TP)], sem_x.at[i])

    def out_copy(i):
        return pltpu.make_async_copy(xio.at[_ds(i * TP, TP)], out_hbm.bitcast(U32).at[_ds(i * TP, TP)], sem_o.at[i])

    w_copies = [pltpu.make_async_copy(s.bitcast(U32), d, sem_w.at[n]) for n, (s, d) in enumerate(
        [(wkt_hbm, wkvt.at[:DH // 2]), (wvt_hbm, wkvt.at[DH // 2:]), (wq_hbm, wq),
         (wqkv_hbm, wqkv), (wob_hbm, wob), (woa_hbm, woa)])]
    x_copy(0).start()
    for c in w_copies[:3]:
        c.start()

    def put_left(dst, r, tile):
        last = []
        for c in range(0, KB, 128):
            fs = _factors(_left_factors, [[tile(i, k * KB + c) for k in range(D // KB)] for i in range(T // MB)])
            for m, f in enumerate(fs):
                dst.at[m][r // 2:r // 2 + 8, c:c + 128] = _pack(f)
            last += [f[a:a + 8] for f in fs[:1] + fs[-2:] for a in (0, 8)]
        return _total(last)

    def put_right(dst, src, row, col, start, col0=0):
        grid = [[_bf(start(src[_ds(i * (KB // 2) + row, 8), _cols(col0 + k * KB + col)])).astype(F32)
                 for k in range(D // KB)] for i in range(D // KB)]
        for m, f in enumerate(_factors(_right_factors, grid)):
            dst.at[m][_ds(row, 8), _cols(col0 // D * KB + col)] = _pack(f)

    def st_ln(j, par, from_input=False):
        def step(r, start):
            ys = []
            for i in range(T // MB):
                row = i * MB + r
                if from_input:
                    x = _bf(xio[_ds((2 * j + par) * TP + row // 2, 8), :]).astype(F32)
                    xr[par][_ds(j * T + row, 16), :] = x
                else:
                    x = xr[par][_ds(j * T + row, 16), :]
                ys.append(_ln(jnp.concatenate([start(x[a:a + 8], (i + a / 16) * MB / T) for a in (0, 8)], axis=0)))
                xp[par * TP + row // 2:par * TP + row // 2 + 8, :] = _pack(ys[-1])
            return put_left(xn[par], r, lambda i, c: ys[i][:, c:c + 128])
        return [functools.partial(step, r) for r in range(0, MB, 16)]

    def st_split(j, par):
        def step(r, start):
            def tile(i, c):
                y = ob[_ds((2 * j + par) * T + i * MB + r, 16), c:c + 128]
                return jnp.concatenate([start(y[a:a + 8], c % KB / KB) for a in (0, 8)], axis=0)
            return put_left(on[par], r, tile)
        return [functools.partial(step, r) for r in range(0, MB, 16)]

    def st_qkv_a(i, par):
        def kv(deps):
            kvt = jax.lax.dot_general(_bf(_after(wkvt[...], deps)), _bf(xp[par * TP:(par + 1) * TP, :]),
                                      (((1,), (1,)), ((), ())), preferred_element_type=F32)
            kt = (kvt[:DH] * QSCALE).astype(BF16).astype(F32)
            k2 = (kt * kt).reshape(DH // 8, 8, T).sum(0).sum(0, keepdims=True)
            km = kmax[:1]
            for t in range(T // 128):
                ts = slice(t * 128, (t + 1) * 128)
                vt[i * (T // 128) + t] = _pack(kvt[DH:, ts])
                km = jnp.maximum(km, k2[:, ts])
                kk = jnp.concatenate([kt[:, ts], jnp.zeros((128 - DH, 128), F32)], axis=0).T
                kk = jnp.where(_iota((128, 128), 1) == DH + 1, 1.0, kk)
                kk = jnp.concatenate([kk[g * 16:(g + 1) * 16] for g in reversed(range(8))], axis=0)
                ka[_ds((i * (T // 128) + t) * 64, 64), :] = _pack(kk)
                if t == 1:
                    for d in range(DH):
                        for a in range(2):
                            kb[2 * i + a, d] = jnp.broadcast_to(kk[112 + 8 * a:120 + 8 * a, d:d + 1], (8, 128))
            kmax[:1] = km
            return [kvt[:8, :128]] * 16

        held = {}

        def emit(row, col, y):
            held[row, col] = y
            t = row // 128
            if all((r, col) in held for r in range(t * 128, t * 128 + 128, MB)):
                y = jnp.concatenate([held.pop((r, col)) for r in range(t * 128, t * 128 + 128, MB)], axis=0)
                for c in range(0, CW, 128):
                    q(t, (col + c) // 128, y[:, c:c + 128])

        def q(t, g, y):
            r = _iota((8, 128), 0)
            qt = y.T
            dst = qa.at[i * (T // 128) + t, g]
            for h in range(4):
                qh = qt[h * DH:(h + 1) * DH]
                n2 = (qh * qh).reshape(DH // 8, 8, 128).sum(0).sum(0, keepdims=True)
                aug = (pltpu.bitcast(-_norm(n2), U32) >> 16) | np.uint32(SHIFT_BITS)
                dst[:DH // 2, h * 128:(h + 1) * 128] = _pack(qh)
                dst[DH // 2:, h * 128:(h + 1) * 128] = jnp.where(r == 0, aug, np.uint32(0))

        return [kv] + _strassen(xn[par], sq, 0, emit)

    def st_fix_k():
        km = _norm(jnp.max(kmax[:1], axis=1, keepdims=True)).astype(BF16).astype(F32)
        kmax[...] = jnp.broadcast_to(km, kmax.shape)
        km = pltpu.bitcast(kmax[:1], U32)
        ka[...] = jnp.where(_iota(ka.shape, 1) == DH, km | (km >> 16), ka[...])
        bad[...] = jnp.zeros(bad.shape, F32)
        for ref in (cs, ca, cl, sp1):
            ref[...] = jnp.zeros(ref.shape, F32)
        for n, t in enumerate(VTILES):
            k = _bf(ka[t * 64 + 56:(t + 1) * 64, :])
            sp0[n * 16:n * 16 + 16, :] = jnp.exp2(_mm(k[:, :KA], _bf(qa[0, 0])))

    def put_o(tb, g, ot):
        ot = jnp.concatenate([ot[:, h * 128:(h + 1) * 128] for h in range(4)], axis=0)
        ob[_ds(tb * 128, 128), _cols(g * 128)] = ot.T

    def pv(tb, g, t, s, state):
        p = jnp.exp2(s)
        if t in VTILES:
            r = VTILES.index(t) * 16
            p = jnp.concatenate([p, side_p[g % 2][r:r + 16, :]], axis=0)
        l = p.reshape(16, 8, 512).sum(0)
        p = jnp.concatenate([p[k * 16:(k + 1) * 16] for k in reversed(range(8))], axis=0)
        o = _mm(_bf(vt[t]), p.astype(BF16))
        if t:
            o, l = state[0] + o, state[1] + l
        if t == S // 128 - 1:
            l = l.sum(0, keepdims=True)
            ok = jnp.logical_and(l >= L_LO, l <= L_HI)
            bad[...] = jnp.maximum(bad[...], jnp.where(ok, 0.0, 1.0))
            put_o(tb, g, o * (1.0 / l))
        return o, l

    def pv_carried(tb):
        pv(tb, U - 1, S // 128 - 1, cs[...], (ca[...], cl[...]))

    def st_attn(j):
        nt = S // 128
        steps = [(j * TU + i, g, t) for i in range(TU) for g in range(U) for t in range(nt)]
        s = {}
        side = [f for i in range(TU) for f in st_permute(j * TU + i)]
        side = [(f, 3 + (16 * (k // 5) + 2 * (k % 5))) for k, f in enumerate(side)]

        keep = _iota((8, 128), 0) + j >= 0
        part = {}

        def qk_vpu(tb, g, h, b, i, start):
            def row(i):
                w = jnp.broadcast_to(qa[tb, g, i:i + 1, h * 128:(h + 1) * 128], (8, 128))
                w = _after(w, [(keep, start)])
                return pltpu.bitcast(w << 16, F32), pltpu.bitcast(w & np.uint32(0xFFFF0000), F32)

            if i == 0:
                lo, hi = row(DH // 2)
                part[0] = [lo * kmax[...] + hi] * VB
            lo, hi = row(i)
            part[0] = [y + (kb[b * VB + a, 2 * i] * lo + kb[b * VB + a, 2 * i + 1] * hi)
                       for a, y in enumerate(part[0])]
            if i == DH // 2 - 1:
                side_p[g % 2][b * VB * 8:(b + 1) * VB * 8, h * 128:(h + 1) * 128] = (
                    jnp.exp2(jnp.concatenate(part.pop(0), axis=0)))

        items = [(h, b, i) for h in range(4) for b in range(2 * NV // VB) for i in range(DH // 2)]

        def qk(n):
            tb, g, t = steps[n]
            rows = 56 if t in VTILES else 64
            s[n] = _mm(_bf(ka[t * 64:t * 64 + rows, :])[:, :KA], _bf(qa[tb, g]))
            if g == U - 1:
                tb = jnp.minimum(tb + 1, nt - 1)
            for m, item in enumerate(items):
                at = int(14 * (VLO + m * (VHI - VLO) / len(items)))
                if at // 14 == t:
                    qk_vpu(tb, (g + 1) % U, *item, s[n][8 * (at % 14):8 * (at % 14) + 8, :128])

        state = None
        for n, step in enumerate(steps):
            qk(n)
            state = pv(*steps[n - 1], prev, state) if n else pv_carried(jnp.maximum(j * TU - 1, 0))
            prev = s.pop(n)
            for f, at in side:
                if at == n:
                    f(lambda x: _after(x, [(keep, prev[:8, :128])]))
        cs[...], ca[...], cl[...] = prev, *state

    def st_attn_exact(u):
        tb, g = u // U, u % U
        q = _bf(qa[tb, g, :DH // 2, :])

        def scores(t):
            kk = jnp.concatenate([ka[_ds(t * 64 + j * 8, 8), :] for j in reversed(range(8))], axis=0)
            return _mm(_bf(kk)[:, :DH], q)

        m = jax.lax.fori_loop(
            0, S // 128, lambda t, m: jnp.maximum(m, jnp.max(scores(t), axis=0, keepdims=True)),
            jnp.full((1, 512), -jnp.inf, F32))

        def body(t, c):
            p = jnp.exp2(scores(t) - m)
            return c[0] + _mm(_bf(vt[t]), p.astype(BF16)), c[1] + jnp.sum(p, axis=0, keepdims=True)

        acc, l = jax.lax.fori_loop(0, S // 128, body, (jnp.zeros((DH, 512), F32), jnp.zeros((1, 512), F32)))
        put_o(tb, g, acc * (1.0 / l))

    def st_out(j, par, w):
        def emit(row, col, y):
            x = xr[par][_ds(j * T + row, MB), col:col + CW] + y
            xr[par][_ds(j * T + row, MB), col:col + CW] = x
            if w is sob:
                xio[_ds((2 * j + par) * TP + row // 2, MB // 2), col:col + CW] = _pack(x)
        return _strassen(on[par], w, 0, emit)

    def st_qkv_b(j, par):
        qkv = bufs[par]

        def emit(n, row, col, y):
            for c in range(0, CW, 128):
                qkv[n * 8 + (col + c) // 128, HALO + row:HALO + row + MB, :] = y[:, c:c + 128]

        def last(f, n, deps):
            tiles = f(deps)
            cs = slice(n * 8, n * 8 + 8)
            h = bufs[1 - par][cs, T:, :]
            if n == 2 and par == 0:
                h = jnp.where(j == 0, jnp.broadcast_to(qkv[cs, HALO:HALO + 1, :], h.shape), h)
            qkv[cs, :HALO, :] = h
            return tiles

        steps = [f for n in range(3) for f in _strassen(xn[par], sp, n * KB, functools.partial(emit, n))]
        for n in (1, 2):
            steps[n * NS + NS - 1] = functools.partial(last, steps[n * NS + NS - 1], n)
        return steps

    def st_probs(j, par):
        buf = bufs[par]

        def softmax(lg, r):
            for w in range(W):
                y = lg[w] * QSCALE
                if par == 0 and r < DIL * w:
                    y = jnp.where(_iota((8, 128), 0) + (j * 2 * T + r) >= DIL * w, y, NEG)
                lg[w] = y
            m = lg[0]
            for w in range(1, W):
                m = jnp.maximum(m, lg[w])
            p = [jnp.exp2(y - m) for y in lg]
            inv = 1.0 / _total(p)
            p = [y * inv for y in p]
            for w in range(W):
                pw[w, r:r + 8, :] = p[w]
            return p

        def step(r, start):
            lg = [[None] * W, [None] * W]
            for c in range(8):
                k = {e: buf[8 + c, pl.ds(HALO + r + e, 8), :] for e in range(-DIL * (W - 1), 9, DIL)}
                for hf in range(2):
                    qc = start(buf[c, HALO + r + 8 * hf:HALO + r + 8 * hf + 8, :], c / 8)
                    for w in range(W):
                        pr = qc * k[8 * hf - DIL * w]
                        lg[hf][w] = pr if c == 0 else lg[hf][w] + pr
            for shift in (64, 32):
                lg = [[y + pltpu.roll(y, shift, 1) for y in ys] for ys in lg]
            return _total(softmax(lg[0], r) + softmax(lg[1], r + 8))

        return [functools.partial(step, r) for r in range(0, T, 16)]

    def st_mix(j, par):
        buf = bufs[par]

        def step(r, start):
            o = [[None] * 8, [None] * 8]
            for n, e in enumerate(range(-DIL * (W - 1), 9, DIL)):
                v = [buf[16 + c, pl.ds(HALO + r + e, 8), :] for c in range(8)]
                for hf in range(2):
                    w = (8 * hf - e) // DIL
                    if 0 <= w < W:
                        p = start(pw[w, r + 8 * hf:r + 8 * hf + 8, :], n / 12)
                        o[hf] = [p * a if b is None else b + p * a for a, b in zip(v, o[hf])]
            for c in range(8):
                ob[_ds((2 * j + par) * T + r, 16), c * 128:(c + 1) * 128] = (
                    jnp.concatenate([o[0][c], o[1][c]], axis=0))
            return _total(o[0] + o[1])

        return [functools.partial(step, r) for r in range(0, T, 16)]

    def st_permute(u):
        n, row = jnp.minimum(u // 4, 2), u % 4 * (KB // 8)
        cs = _cols(u % 8 * 128)

        def gather(t, start):
            y = start(jnp.concatenate([wqkv[_ds(i * (KB // 2) + row, KB // 8), _cols(n * D + t * 128)]
                                       for i in range(D // KB)], axis=0)).T
            for h in range(4 * t, 4 * t + 4):
                tmp[pl.ds(h * (DH + 1), DH), :] = y[h % 4 * DH:(h % 4 + 1) * DH]
                tmpo[h % 2, pl.ds(h // 2 * (DH // 2 + 1), DH // 2), :] = wob[h * DH // 2:(h + 1) * DH // 2, cs]

        def scatter(t, start):
            y = start(jnp.concatenate([tmp[pl.ds(4 * t + e, H, stride=DH + 1), :] for e in range(4)], axis=0)).T
            for i in range(D // KB):
                wp[_ds(i * (KB // 2) + row, KB // 8), _cols(n * D + t * 128)] = y[i * (KB // 8):(i + 1) * (KB // 8)]
            for e in (2 * t, 2 * t + 1):
                a, b = [tmpo[k, pl.ds(e, H // 2, stride=DH // 2 + 1), :] for k in range(2)]
                a = start(a)
                wobp[e * H:e * H + H // 2, cs] = (a & np.uint32(0xFFFF)) | (b << 16)
                wobp[e * H + H // 2:(e + 1) * H, cs] = (a >> 16) | (b & np.uint32(0xFFFF0000))

        def part(dst, src, row, parts, **kw):
            return [functools.partial(put_right, dst, src, row + r, c, **kw)
                    for r in range(0, KB // 2 // parts, 8) for c in range(0, KB, 128)]

        return ([functools.partial(f, t) for f in (gather, scatter) for t in range(8)]
                + part(soa, woa, u * (KB // 32), 16) + part(sob, wobp, u % 8 * (KB // 16), 8)
                + part(sp, wp, row, 4, col0=n * D))

    NP = NB // 2

    def qkv_a(j, from_input):
        for par, jn in ((0, j), (1, jnp.minimum(j + 1, NP - 1))):
            _overlap(j, st_qkv_a(2 * j + par, par), (st_ln(jn, 1 - par, from_input), 1, 23, 27))

    kmax[...] = jnp.zeros(kmax.shape, F32)
    b1[...] = jnp.zeros(b1.shape, F32)
    pw[...] = jnp.zeros(pw.shape, F32)
    wobp[...] = jnp.zeros(wobp.shape, U32)
    x_copy(0).wait()
    for f in st_ln(0, 0, True):
        f(_now)
    for c in w_copies[:3]:
        c.wait()
    x_copy(1).start()
    x_copy(2).start()

    @pl.loop(0, 16)
    def _(u):
        for r in range(0, KB // 32, 8):
            for c in range(0, KB, 128):
                put_right(sq, wq, u * (KB // 32) + r, c, _now)

    @pl.loop(0, NP)
    def _(j):
        x_copy(2 * j + 1).wait()

        @pl.when(j == 0)
        def _():
            for i in range(3, NB):
                x_copy(i).start()

        @pl.when(j + 1 < NP)
        def _():
            x_copy(2 * j + 2).wait()

        @pl.when(j == 1)
        def _():
            for c in w_copies[3:]:
                c.start()

        qkv_a(j, True)

    for c in w_copies[3:]:
        c.wait()

    @pl.loop(0, 2)
    def _(layer):
        st_fix_k()

        @pl.loop(0, S // 128 // TU)
        def _(j):
            st_attn(j)

        pv_carried(S // 128 - 1)

        @pl.when(jnp.max(bad[...]) > 0.0)
        def _():
            @pl.loop(0, (S // 128) * U)
            def _(u):
                st_attn_exact(u)

        for f in st_split(0, 0):
            f(_now)

        @pl.loop(0, NP)
        def _(j):
            _overlap(j, st_out(j, 0, soa) + st_out(j, 1, soa), (st_split(j, 1), 1, 21, 28),
                     (st_ln(0, 0), 30, 50, 56), (st_split(jnp.minimum(j + 1, NP - 1), 0), 30, 50, 56))

        @pl.loop(0, NP)
        def _(j):
            jp, jn = jnp.maximum(j - 1, 0), jnp.minimum(j + 1, NP - 1)
            _overlap(j, st_qkv_b(j, 0) + st_qkv_b(j, 1),
                     (st_probs(jp, 1)[8:], 1, 25, 32), (st_mix(jp, 1), 25, 60, 67), (st_ln(j, 1), 32, 72, 84),
                     (st_probs(j, 0), 58, 108, 114), (st_mix(j, 0), 106, 136, 143), (st_ln(jn, 0), 108, 138, 150),
                     (st_split(0, 0), 140, 158, 168), (st_probs(j, 1)[:8], 140, 160, 168))

        def out_b(j, first=False):
            sides = [(st_split(j, 1), 1, 21, 28), (st_split(jnp.minimum(j + 1, NP - 1), 0), 30, 50, 56)]
            if first:
                sides = [(st_probs(NP - 1, 1)[8:], 1, 17, 24), (st_mix(NP - 1, 1), 17, 50, 56),
                         (st_ln(0, 0), 30, 50, 56)] + sides
            _overlap(layer, st_out(j, 0, sob) + st_out(j, 1, sob), *sides)

            @pl.when(layer == 1)
            def _():
                out_copy(2 * j).start()
                out_copy(2 * j + 1).start()

        out_b(0, True)
        pl.loop(1, NP)(out_b)

        @pl.when(layer == 0)
        def _():
            kmax[...] = jnp.zeros(kmax.shape, F32)

            @pl.loop(0, NP)
            def _(j):
                qkv_a(j, False)

    for i in range(NB):
        out_copy(i).wait()


@jax.jit
def pallas_interleave_layers__grouped_kv_mqa__sliding_local_dilated__prompt_kernel(
    A_x: jax.Array,
    A_wq: jax.Array,
    A_wk: jax.Array,
    A_wv: jax.Array,
    A_wo: jax.Array,
    B_x: jax.Array,
    B_wqkv: jax.Array,
    B_wo: jax.Array,
):
    del B_x
    vm = pltpu.VMEM
    out = pl.pallas_call(
        _kernel,
        out_shape=jax.ShapeDtypeStruct((S, D), BF16),
        in_specs=[pl.BlockSpec(memory_space=pl.ANY)] * 7,
        out_specs=pl.BlockSpec(memory_space=pl.ANY),
        scratch_shapes=[
            vm((S // 2, D), U32),
            vm((D // 2, D), U32), vm((D // 2, D), U32),
            vm((D // 2, 3 * D), U32), vm((D // 2, D), U32),
            vm((D // 2, 3 * D), U32), vm((D // 2, D), U32),
            *[vm((NF, KB // 2, n * KB), U32) for n in (1, 1, 3, 1)],
            vm((DH, D), U32),
            vm((D + 2 * H, 128), U32), vm((2, D // 4 + H, 128), U32),
            vm((S // 2, D), F32), vm((S // 2, D), F32),
            vm((S, D), F32),
            vm((T, D), U32),
            *[vm((NF, MB // 2, KB), U32)] * 4,
            vm((S // 128, U, KA // 2, 512), U32),
            vm((S // 2, 128), U32), vm((S // 128, DH // 2, 128), U32),
            vm((2 * NV, DH, 8, 128), F32),
            vm((16 * NV, 512), F32), vm((16 * NV, 512), F32),
            vm((112, 512), F32), vm((DH, 512), F32), vm((8, 512), F32),
            vm((8, 128), F32), vm((1, 512), F32),
            vm((24, T + HALO, 128), F32), vm((24, T + HALO, 128), F32), vm((W, T, 128), F32),
            pltpu.SemaphoreType.DMA((NB,)), pltpu.SemaphoreType.DMA((6,)), pltpu.SemaphoreType.DMA((NB,)),
        ],
        compiler_params=pltpu.CompilerParams(vmem_limit_bytes=120 * 1024 * 1024),
        name="four_layers",
    )(A_x.reshape(S, D), A_wq, A_wk.T, A_wv.T, A_wo, B_wqkv, B_wo)
    return out.reshape(1, S, D)
```

```python
import functools
import itertools

import jax
import jax.numpy as jnp
import numpy as np
import jax.experimental.pallas as pl
import jax.experimental.pallas.tpu as pltpu

F32, BF16, U32 = jnp.float32, jnp.bfloat16, jnp.uint32

S, D, H, DH = 2048, 1024, 32, 32
W, DIL = 8, 2
EPS = 1e-5
LOG2E = 1.4426950408889634
QSCALE = DH ** -0.5 * LOG2E
NEG = -1e9 * LOG2E

T = 256
NB = S // T
KA = 48
HALO = 16
LEVELS = 1
NF, MB, KB = 7 ** LEVELS, T >> LEVELS, D >> LEVELS
CW = 4 * 128 * 128 // KB
NS = NF * KB // CW
LEAD = 12 * NS // 28
U = 8
TU = 1
NV = 8
VTILES = list(range(1, S // 128, 2))
VB = 4
VLO, VHI = 0, 16
SHIFT_BITS = 0x42480000
L_LO, L_HI = 2.0 ** -50, 2.0 ** 63


def _mm(a, b):
    return jnp.dot(a, b, preferred_element_type=F32)


def _pack(x):
    return pltpu.bitcast(x.astype(BF16), U32)


def _bf(x):
    return pltpu.bitcast(x, BF16)


def _ln(x):
    m = jnp.mean(x, axis=-1, keepdims=True)
    c = x - m
    v = jnp.mean(c * c, axis=-1, keepdims=True)
    return c * jax.lax.rsqrt(v + EPS)


def _total(xs):
    return functools.reduce(jnp.add, xs)


def _norm(sq):
    return sq * jax.lax.rsqrt(sq + 1e-30)


def _iota(shape, dim):
    return jax.lax.broadcasted_iota(jnp.int32, shape, dim)


def _ds(start, n):
    return pl.ds(start if isinstance(start, int) else pl.multiple_of(start, 8), n)


def _cols(start, n=128):
    return pl.ds(start if isinstance(start, int) else pl.multiple_of(start, 128), n)


def _after(x, deps):
    for keep, d in deps:
        head = jnp.where(keep, x[:8, :128], pltpu.bitcast(d, x.dtype))
        if x.shape[1] > 128:
            head = jnp.concatenate([head, x[:8, 128:]], axis=1)
        x = jnp.concatenate([head, x[8:]], axis=0) if x.shape[0] > 8 else head
    return x


def _overlap(j, mms, *sides):
    keep = _iota((8, 128), 0) + j >= 0
    todo = [[] for _ in range(len(mms) + 1)]
    for steps, *times in sides:
        lo, hi, limit = [-(-x * NS // 28) for x in times]
        dt = (hi - lo) / len(steps)
        for m, f in enumerate(steps):
            todo[min(int(lo + (m + 1) * dt) + LEAD, limit)].append((f, lo + m * dt, dt))
    made = []

    def release(t, dt, x, frac=0.0):
        if not made:
            return x
        return _after(x, [(keep, made[min(int((t + frac * dt) * len(made) / n), len(made) - 1)])])

    for n, steps in enumerate(todo):
        done = [f(functools.partial(release, t, dt)) for f, t, dt in steps]
        if n < len(mms):
            made += mms[n]([(keep, _total(done))] if done else [])


def _left_factors(a11, a12, a21, a22):
    return a11 + a22, a21 + a22, a11, a22, a11 + a12, a21 - a11, a12 - a22


def _right_factors(b11, b12, b21, b22):
    return b11 + b22, b11, b12 - b22, b21 - b11, b22, b11 + b12, b21 + b22


def _factors(rule, grid):
    n = len(grid) // 2
    if not n:
        return [grid[0][0]]
    fs = [[rule(grid[a][b], grid[a][n + b], grid[n + a][b], grid[n + a][n + b]) for b in range(n)] for a in range(n)]
    return [f for m in range(7) for f in _factors(rule, [[x[m] for x in row] for row in fs])]


ORDER = (0, 1, 3, 6, 4, 2, 5)


def _combiner(levels, emit):
    if not levels:
        return lambda ms, y: emit(0, 0, y)
    v = {}

    def rule(m, size, a, b, y):
        c = v.setdefault((a, b), {})
        out = lambda i, j, y: emit(i * size + a, j * size + b, y)
        if m == 0:
            c[0] = c[3] = y
        elif m == 1:
            c[3] -= y
            c[2] = y
        elif m == 3:
            c[0] += y
            out(1, 0, c.pop(2) + y)
        elif m == 6:
            c[0] += y
        elif m == 4:
            out(0, 0, c.pop(0) - y)
            c[1] = y
        elif m == 2:
            out(0, 1, c.pop(1) + y)
            c[3] += y
        else:
            out(1, 1, c.pop(3) + y)

    inner = [_combiner(levels - 1, functools.partial(rule, m, 2 ** (levels - 1))) for m in range(7)]
    return lambda ms, y: inner[ms[0]](ms[1:], y)


def _strassen(a, b, col0, emit):
    def step(c, put, ms, deps):
        m = functools.reduce(lambda x, y: 7 * x + y, ms)
        y = _mm(_bf(a.at[m][...]), _bf(_after(b.at[m][:, col0 + c:col0 + c + CW], deps)))
        put(ms, y)
        return [y[r:r + 8, k:k + 128] for r in range(0, MB, 8) for k in range(0, CW, 128)]

    steps = []
    for c in range(0, KB, CW):
        put = _combiner(LEVELS, lambda i, j, y, c=c: emit(i * MB, j * KB + c, y))
        steps += [functools.partial(step, c, put, ms) for ms in itertools.product(ORDER, repeat=LEVELS)]
    return steps


def _now(x, frac=0.0):
    return x


def _kernel(x_hbm, wq_hbm, wkt_hbm, wvt_hbm, woa_hbm, wqkv_hbm, wob_hbm, out_hbm,
            xio, wq, woa, wqkv, wob, wp, wobp, sq, soa, sp, sob, wkvt, tmp, tmpo,
            xe, xo, ob, xp, xn0, xn1, on0, on1, qa, ka, vt, kb, sp0, sp1, cs, ca, cl, kmax, bad,
            b0, b1, pw, sem_x, sem_w, sem_o):
    xr, xn, on = (xe, xo), (xn0, xn1), (on0, on1)
    bufs, side_p = (b0, b1), (sp0, sp1)
    TP = T // 2

    def x_copy(i):
        return pltpu.make_async_copy(x_hbm.bitcast(U32).at[_ds(i * TP, TP)], xio.at[_ds(i * TP, TP)], sem_x.at[i])

    def out_copy(i):
        return pltpu.make_async_copy(xio.at[_ds(i * TP, TP)], out_hbm.bitcast(U32).at[_ds(i * TP, TP)], sem_o.at[i])

    w_copies = [pltpu.make_async_copy(s.bitcast(U32), d, sem_w.at[n]) for n, (s, d) in enumerate(
        [(wkt_hbm, wkvt.at[:DH // 2]), (wvt_hbm, wkvt.at[DH // 2:]), (wq_hbm, wq),
         (wqkv_hbm, wqkv), (wob_hbm, wob), (woa_hbm, woa)])]
    x_copy(0).start()
    for c in w_copies[:3]:
        c.start()

    def put_left(dst, r, tile):
        last = []
        for c in range(0, KB, 128):
            fs = _factors(_left_factors, [[tile(i, k * KB + c) for k in range(D // KB)] for i in range(T // MB)])
            for m, f in enumerate(fs):
                dst.at[m][r // 2:r // 2 + 8, c:c + 128] = _pack(f)
            last += [f[a:a + 8] for f in fs[:1] + fs[-2:] for a in (0, 8)]
        return _total(last)

    def put_right(dst, src, row, col, start, col0=0):
        grid = [[_bf(start(src[_ds(i * (KB // 2) + row, 8), _cols(col0 + k * KB + col)])).astype(F32)
                 for k in range(D // KB)] for i in range(D // KB)]
        for m, f in enumerate(_factors(_right_factors, grid)):
            dst.at[m][_ds(row, 8), _cols(col0 // D * KB + col)] = _pack(f)

    def st_ln(j, par, from_input=False):
        def step(r, start):
            ys = []
            for i in range(T // MB):
                row = i * MB + r
                if from_input:
                    x = _bf(xio[_ds((2 * j + par) * TP + row // 2, 8), :]).astype(F32)
                    xr[par][_ds(j * T + row, 16), :] = x
                else:
                    x = xr[par][_ds(j * T + row, 16), :]
                ys.append(_ln(jnp.concatenate([start(x[a:a + 8], (i + a / 16) * MB / T) for a in (0, 8)], axis=0)))
                xp[par * TP + row // 2:par * TP + row // 2 + 8, :] = _pack(ys[-1])
            return put_left(xn[par], r, lambda i, c: ys[i][:, c:c + 128])
        return [functools.partial(step, r) for r in range(0, MB, 16)]

    def st_split(j, par):
        def step(r, start):
            def tile(i, c):
                y = ob[_ds((2 * j + par) * T + i * MB + r, 16), c:c + 128]
                return jnp.concatenate([start(y[a:a + 8], c % KB / KB) for a in (0, 8)], axis=0)
            return put_left(on[par], r, tile)
        return [functools.partial(step, r) for r in range(0, MB, 16)]

    def st_qkv_a(i, par):
        def kv(deps):
            kvt = jax.lax.dot_general(_bf(_after(wkvt[...], deps)), _bf(xp[par * TP:(par + 1) * TP, :]),
                                      (((1,), (1,)), ((), ())), preferred_element_type=F32)
            kt = (kvt[:DH] * QSCALE).astype(BF16).astype(F32)
            k2 = (kt * kt).reshape(DH // 8, 8, T).sum(0).sum(0, keepdims=True)
            km = kmax[:1]
            for t in range(T // 128):
                ts = slice(t * 128, (t + 1) * 128)
                vt[i * (T // 128) + t] = _pack(kvt[DH:, ts])
                km = jnp.maximum(km, k2[:, ts])
                kk = jnp.concatenate([kt[:, ts], jnp.zeros((128 - DH, 128), F32)], axis=0).T
                kk = jnp.where(_iota((128, 128), 1) == DH + 1, 1.0, kk)
                kk = jnp.concatenate([kk[g * 16:(g + 1) * 16] for g in reversed(range(8))], axis=0)
                ka[_ds((i * (T // 128) + t) * 64, 64), :] = _pack(kk)
                if t == 1:
                    for d in range(DH):
                        for a in range(2):
                            kb[2 * i + a, d] = jnp.broadcast_to(kk[112 + 8 * a:120 + 8 * a, d:d + 1], (8, 128))
            kmax[:1] = km
            return [kvt[:8, :128]] * 16

        held = {}

        def emit(row, col, y):
            held[row, col] = y
            t = row // 128
            if all((r, col) in held for r in range(t * 128, t * 128 + 128, MB)):
                y = jnp.concatenate([held.pop((r, col)) for r in range(t * 128, t * 128 + 128, MB)], axis=0)
                for c in range(0, CW, 128):
                    q(t, (col + c) // 128, y[:, c:c + 128])

        def q(t, g, y):
            r = _iota((8, 128), 0)
            qt = y.T
            dst = qa.at[i * (T // 128) + t, g]
            for h in range(4):
                qh = qt[h * DH:(h + 1) * DH]
                n2 = (qh * qh).reshape(DH // 8, 8, 128).sum(0).sum(0, keepdims=True)
                aug = (pltpu.bitcast(-_norm(n2), U32) >> 16) | np.uint32(SHIFT_BITS)
                dst[:DH // 2, h * 128:(h + 1) * 128] = _pack(qh)
                dst[DH // 2:, h * 128:(h + 1) * 128] = jnp.where(r == 0, aug, np.uint32(0))

        return [kv] + _strassen(xn[par], sq, 0, emit)

    def st_fix_k():
        km = _norm(jnp.max(kmax[:1], axis=1, keepdims=True)).astype(BF16).astype(F32)
        kmax[...] = jnp.broadcast_to(km, kmax.shape)
        km = pltpu.bitcast(kmax[:1], U32)
        ka[...] = jnp.where(_iota(ka.shape, 1) == DH, km | (km >> 16), ka[...])
        bad[...] = jnp.zeros(bad.shape, F32)
        for ref in (cs, ca, cl, sp1):
            ref[...] = jnp.zeros(ref.shape, F32)
        for n, t in enumerate(VTILES):
            k = _bf(ka[t * 64 + 56:(t + 1) * 64, :])
            sp0[n * 16:n * 16 + 16, :] = jnp.exp2(_mm(k[:, :KA], _bf(qa[0, 0])))

    def put_o(tb, g, ot):
        ot = jnp.concatenate([ot[:, h * 128:(h + 1) * 128] for h in range(4)], axis=0)
        ob[_ds(tb * 128, 128), _cols(g * 128)] = ot.T

    def pv(tb, g, t, s, state):
        p = jnp.exp2(s)
        if t in VTILES:
            r = VTILES.index(t) * 16
            p = jnp.concatenate([p, side_p[g % 2][r:r + 16, :]], axis=0)
        l = p.reshape(16, 8, 512).sum(0)
        p = jnp.concatenate([p[k * 16:(k + 1) * 16] for k in reversed(range(8))], axis=0)
        o = _mm(_bf(vt[t]), p.astype(BF16))
        if t:
            o, l = state[0] + o, state[1] + l
        if t == S // 128 - 1:
            l = l.sum(0, keepdims=True)
            ok = jnp.logical_and(l >= L_LO, l <= L_HI)
            ok = jnp.logical_and(ok, jnp.abs(o.reshape(DH // 8, 8, 512).sum(0)) <= 3e38)
            bad[...] = jnp.maximum(bad[...], jnp.where(ok, 0.0, 1.0))
            put_o(tb, g, o * (1.0 / l))
        return o, l

    def pv_carried(tb):
        pv(tb, U - 1, S // 128 - 1, cs[...], (ca[...], cl[...]))

    def st_attn(j):
        nt = S // 128
        steps = [(j * TU + i, g, t) for i in range(TU) for g in range(U) for t in range(nt)]
        s = {}
        side = [f for i in range(TU) for f in st_permute(j * TU + i)]
        side = [(f, 3 + (16 * (k // 4) + 3 * (k % 4) if k < 16 else 64 + 16 * ((k - 16) // 14) + (k - 16) % 14 * 11 // 14)) for k, f in enumerate(side)]

        assert all(at < len(steps) for _, at in side)
        keep = _iota((8, 128), 0) + j >= 0
        part = {}

        def qk_vpu(tb, g, h, b, i, start):
            def row(i):
                w = jnp.broadcast_to(qa[tb, g, i:i + 1, h * 128:(h + 1) * 128], (8, 128))
                w = _after(w, [(keep, start)])
                return pltpu.bitcast(w << 16, F32), pltpu.bitcast(w & np.uint32(0xFFFF0000), F32)

            if i == 0:
                lo, hi = row(DH // 2)
                part[0] = [lo * kmax[...] + hi] * VB
            lo, hi = row(i)
            part[0] = [y + (kb[b * VB + a, 2 * i] * lo + kb[b * VB + a, 2 * i + 1] * hi)
                       for a, y in enumerate(part[0])]
            if i == DH // 2 - 1:
                side_p[g % 2][b * VB * 8:(b + 1) * VB * 8, h * 128:(h + 1) * 128] = (
                    jnp.exp2(jnp.concatenate(part.pop(0), axis=0)))

        items = [(h, b, i) for h in range(4) for b in range(2 * NV // VB) for i in range(DH // 2)]

        def qk(n):
            tb, g, t = steps[n]
            rows = 56 if t in VTILES else 64
            s[n] = _mm(_bf(ka[t * 64:t * 64 + rows, :])[:, :KA], _bf(qa[tb, g]))
            if g == U - 1:
                tb = jnp.minimum(tb + 1, nt - 1)
            for m, item in enumerate(items):
                at = int(14 * (VLO + m * (VHI - VLO) / len(items)))
                if at // 14 == t:
                    qk_vpu(tb, (g + 1) % U, *item, s[n][8 * (at % 14):8 * (at % 14) + 8, :128])

        state = None
        for n, step in enumerate(steps):
            qk(n)
            state = pv(*steps[n - 1], prev, state) if n else pv_carried(jnp.maximum(j * TU - 1, 0))
            prev = s.pop(n)
            for f, at in side:
                if at == n:
                    f(lambda x: _after(x, [(keep, prev[:8, :128])]))
        cs[...], ca[...], cl[...] = prev, *state

    def st_attn_exact(u):
        tb, g = u // U, u % U
        q = _bf(qa[tb, g, :DH // 2, :])

        def scores(t):
            kk = jnp.concatenate([ka[_ds(t * 64 + j * 8, 8), :] for j in reversed(range(8))], axis=0)
            return _mm(_bf(kk)[:, :DH], q)

        m = jax.lax.fori_loop(
            0, S // 128, lambda t, m: jnp.maximum(m, jnp.max(scores(t), axis=0, keepdims=True)),
            jnp.full((1, 512), -jnp.inf, F32))

        def body(t, c):
            p = jnp.exp2(scores(t) - m)
            return c[0] + _mm(_bf(vt[t]), p.astype(BF16)), c[1] + jnp.sum(p, axis=0, keepdims=True)

        acc, l = jax.lax.fori_loop(0, S // 128, body, (jnp.zeros((DH, 512), F32), jnp.zeros((1, 512), F32)))
        put_o(tb, g, acc * (1.0 / l))

    def st_out(j, par, w):
        def emit(row, col, y):
            x = xr[par][_ds(j * T + row, MB), col:col + CW] + y
            xr[par][_ds(j * T + row, MB), col:col + CW] = x
            if w is sob:
                xio[_ds((2 * j + par) * TP + row // 2, MB // 2), col:col + CW] = _pack(x)
        return _strassen(on[par], w, 0, emit)

    def st_qkv_b(j, par):
        qkv = bufs[par]

        def emit(n, row, col, y):
            for c in range(0, CW, 128):
                qkv[n * 8 + (col + c) // 128, HALO + row:HALO + row + MB, :] = y[:, c:c + 128]

        def last(f, n, deps):
            tiles = f(deps)
            cs = slice(n * 8, n * 8 + 8)
            h = bufs[1 - par][cs, T:, :]
            if n == 2 and par == 0:
                h = jnp.where(j == 0, jnp.broadcast_to(qkv[cs, HALO:HALO + 1, :], h.shape), h)
            qkv[cs, :HALO, :] = h
            return tiles

        steps = [f for n in range(3) for f in _strassen(xn[par], sp, n * KB, functools.partial(emit, n))]
        for n in (1, 2):
            steps[n * NS + NS - 1] = functools.partial(last, steps[n * NS + NS - 1], n)
        return steps

    def st_probs(j, par):
        buf = bufs[par]

        def softmax(lg, r):
            for w in range(W):
                y = lg[w] * QSCALE
                if par == 0 and r < DIL * w:
                    y = jnp.where(_iota((8, 128), 0) + (j * 2 * T + r) >= DIL * w, y, NEG)
                lg[w] = y
            m = lg[0]
            for w in range(1, W):
                m = jnp.maximum(m, lg[w])
            p = [jnp.exp2(y - m) for y in lg]
            inv = 1.0 / _total(p)
            p = [y * inv for y in p]
            for w in range(W):
                pw[w, r:r + 8, :] = p[w]
            return p

        def step(r, start):
            lg = [[None] * W, [None] * W]
            for c in range(8):
                k = {e: buf[8 + c, pl.ds(HALO + r + e, 8), :] for e in range(-DIL * (W - 1), 9, DIL)}
                for hf in range(2):
                    qc = start(buf[c, HALO + r + 8 * hf:HALO + r + 8 * hf + 8, :], c / 8)
                    for w in range(W):
                        pr = qc * k[8 * hf - DIL * w]
                        lg[hf][w] = pr if c == 0 else lg[hf][w] + pr
            for shift in (64, 32):
                lg = [[y + pltpu.roll(y, shift, 1) for y in ys] for ys in lg]
            return _total(softmax(lg[0], r) + softmax(lg[1], r + 8))

        return [functools.partial(step, r) for r in range(0, T, 16)]

    def st_mix(j, par):
        buf = bufs[par]

        def step(r, start):
            o = [[None] * 8, [None] * 8]
            for n, e in enumerate(range(-DIL * (W - 1), 9, DIL)):
                v = [buf[16 + c, pl.ds(HALO + r + e, 8), :] for c in range(8)]
                for hf in range(2):
                    w = (8 * hf - e) // DIL
                    if 0 <= w < W:
                        p = start(pw[w, r + 8 * hf:r + 8 * hf + 8, :], n / 12)
                        o[hf] = [p * a if b is None else b + p * a for a, b in zip(v, o[hf])]
            for c in range(8):
                ob[_ds((2 * j + par) * T + r, 16), c * 128:(c + 1) * 128] = (
                    jnp.concatenate([o[0][c], o[1][c]], axis=0))
            return _total(o[0] + o[1])

        return [functools.partial(step, r) for r in range(0, T, 16)]

    def st_permute(u):
        n, row = jnp.minimum(u // 4, 2), u % 4 * (KB // 8)
        cs = _cols(u % 8 * 128)

        def gather(t, start):
            y = start(jnp.concatenate([wqkv[_ds(i * (KB // 2) + row, KB // 8), _cols(n * D + t * 128)]
                                       for i in range(D // KB)], axis=0)).T
            for h in range(4 * t, 4 * t + 4):
                tmp[pl.ds(h * (DH + 1), DH), :] = y[h % 4 * DH:(h % 4 + 1) * DH]
                tmpo[h % 2, pl.ds(h // 2 * (DH // 2 + 1), DH // 2), :] = wob[h * DH // 2:(h + 1) * DH // 2, cs]

        def scatter(t, start):
            y = start(jnp.concatenate([tmp[pl.ds(4 * t + e, H, stride=DH + 1), :] for e in range(4)], axis=0)).T
            for i in range(D // KB):
                wp[_ds(i * (KB // 2) + row, KB // 8), _cols(n * D + t * 128)] = y[i * (KB // 8):(i + 1) * (KB // 8)]
            for e in (2 * t, 2 * t + 1):
                a, b = [tmpo[k, pl.ds(e, H // 2, stride=DH // 2 + 1), :] for k in range(2)]
                a = start(a)
                wobp[e * H:e * H + H // 2, cs] = (a & np.uint32(0xFFFF)) | (b << 16)
                wobp[e * H + H // 2:(e + 1) * H, cs] = (a >> 16) | (b & np.uint32(0xFFFF0000))

        def part(dst, src, row, parts, **kw):
            return [functools.partial(put_right, dst, src, row + r, c, **kw)
                    for r in range(0, KB // 2 // parts, 8) for c in range(0, KB, 128)]

        return ([functools.partial(f, t) for f in (gather, scatter) for t in range(8)]
                + part(soa, woa, u * (KB // 32), 16) + part(sob, wobp, u % 8 * (KB // 16), 8)
                + part(sp, wp, row, 4, col0=n * D))

    NP = NB // 2

    def qkv_a(j, from_input):
        for par, jn in ((0, j), (1, jnp.minimum(j + 1, NP - 1))):
            _overlap(j, st_qkv_a(2 * j + par, par), (st_ln(jn, 1 - par, from_input), 1, 23, 27))

    kmax[...] = jnp.zeros(kmax.shape, F32)
    b1[...] = jnp.zeros(b1.shape, F32)
    pw[...] = jnp.zeros(pw.shape, F32)
    wobp[...] = jnp.zeros(wobp.shape, U32)
    x_copy(0).wait()
    for f in st_ln(0, 0, True):
        f(_now)
    for c in w_copies[:3]:
        c.wait()
    x_copy(1).start()
    x_copy(2).start()

    @pl.loop(0, 16)
    def _(u):
        for r in range(0, KB // 32, 8):
            for c in range(0, KB, 128):
                put_right(sq, wq, u * (KB // 32) + r, c, _now)

    @pl.loop(0, NP)
    def _(j):
        x_copy(2 * j + 1).wait()

        @pl.when(j == 0)
        def _():
            for i in range(3, NB):
                x_copy(i).start()

        @pl.when(j + 1 < NP)
        def _():
            x_copy(2 * j + 2).wait()

        @pl.when(j == 1)
        def _():
            for c in w_copies[3:]:
                c.start()

        qkv_a(j, True)

    for c in w_copies[3:]:
        c.wait()

    @pl.loop(0, 2)
    def _(layer):
        st_fix_k()

        @pl.loop(0, S // 128 // TU)
        def _(j):
            st_attn(j)

        pv_carried(S // 128 - 1)

        @pl.when(jnp.max(bad[...]) > 0.0)
        def _():
            @pl.loop(0, (S // 128) * U)
            def _(u):
                st_attn_exact(u)

        for f in st_split(0, 0):
            f(_now)

        @pl.loop(0, NP)
        def _(j):
            _overlap(j, st_out(j, 0, soa) + st_out(j, 1, soa), (st_split(j, 1), 1, 21, 28),
                     (st_ln(0, 0), 30, 50, 56), (st_split(jnp.minimum(j + 1, NP - 1), 0), 30, 50, 56))

        @pl.loop(0, NP)
        def _(j):
            jp, jn = jnp.maximum(j - 1, 0), jnp.minimum(j + 1, NP - 1)
            _overlap(j, st_qkv_b(j, 0) + st_qkv_b(j, 1),
                     (st_probs(jp, 1)[8:], 1, 25, 32), (st_mix(jp, 1), 25, 60, 67), (st_ln(j, 1), 32, 72, 84),
                     (st_probs(j, 0), 58, 108, 114), (st_mix(j, 0), 106, 136, 143), (st_ln(jn, 0), 108, 138, 150),
                     (st_split(0, 0), 140, 158, 168), (st_probs(j, 1)[:8], 140, 160, 168))

        def out_b(j, first=False):
            sides = [(st_split(j, 1), 1, 21, 28), (st_split(jnp.minimum(j + 1, NP - 1), 0), 30, 50, 56)]
            if first:
                sides = [(st_probs(NP - 1, 1)[8:], 1, 17, 24), (st_mix(NP - 1, 1), 17, 50, 56),
                         (st_ln(0, 0), 30, 50, 56)] + sides
            _overlap(layer, st_out(j, 0, sob) + st_out(j, 1, sob), *sides)

            @pl.when(layer == 1)
            def _():
                out_copy(2 * j).start()
                out_copy(2 * j + 1).start()

        out_b(0, True)
        pl.loop(1, NP)(out_b)

        @pl.when(layer == 0)
        def _():
            kmax[...] = jnp.zeros(kmax.shape, F32)

            @pl.loop(0, NP)
            def _(j):
                qkv_a(j, False)

    for i in range(NB):
        out_copy(i).wait()


@jax.jit
def pallas_interleave_layers__grouped_kv_mqa__sliding_local_dilated__prompt_kernel(
    A_x: jax.Array,
    A_wq: jax.Array,
    A_wk: jax.Array,
    A_wv: jax.Array,
    A_wo: jax.Array,
    B_x: jax.Array,
    B_wqkv: jax.Array,
    B_wo: jax.Array,
):
    del B_x
    vm = pltpu.VMEM
    out = pl.pallas_call(
        _kernel,
        out_shape=jax.ShapeDtypeStruct((S, D), BF16),
        in_specs=[pl.BlockSpec(memory_space=pl.ANY)] * 7,
        out_specs=pl.BlockSpec(memory_space=pl.ANY),
        scratch_shapes=[
            vm((S // 2, D), U32),
            vm((D // 2, D), U32), vm((D // 2, D), U32),
            vm((D // 2, 3 * D), U32), vm((D // 2, D), U32),
            vm((D // 2, 3 * D), U32), vm((D // 2, D), U32),
            *[vm((NF, KB // 2, n * KB), U32) for n in (1, 1, 3, 1)],
            vm((DH, D), U32),
            vm((D + 2 * H, 128), U32), vm((2, D // 4 + H, 128), U32),
            vm((S // 2, D), F32), vm((S // 2, D), F32),
            vm((S, D), F32),
            vm((T, D), U32),
            *[vm((NF, MB // 2, KB), U32)] * 4,
            vm((S // 128, U, KA // 2, 512), U32),
            vm((S // 2, 128), U32), vm((S // 128, DH // 2, 128), U32),
            vm((2 * NV, DH, 8, 128), F32),
            vm((16 * NV, 512), F32), vm((16 * NV, 512), F32),
            vm((112, 512), F32), vm((DH, 512), F32), vm((8, 512), F32),
            vm((8, 128), F32), vm((8, 512), F32),
            vm((24, T + HALO, 128), F32), vm((24, T + HALO, 128), F32),
            vm((W, T, 128), F32),
            pltpu.SemaphoreType.DMA((NB,)), pltpu.SemaphoreType.DMA((6,)), pltpu.SemaphoreType.DMA((NB,)),
        ],
        compiler_params=pltpu.CompilerParams(vmem_limit_bytes=120 * 1024 * 1024),
        name="four_layers",
    )(A_x.reshape(S, D), A_wq, A_wk.T, A_wv.T, A_wo, B_wqkv, B_wo)
    return out.reshape(1, S, D)
```
